```python
import jax
import jax.numpy as jnp

def _softmax(x, axis=-1):
    return jax.nn.softmax(x, axis=axis)

def _gelu(x):
    return jax.nn.gelu(x, approximate=True)

def _silu(x):
    return jax.nn.silu(x)

def _sigmoid(x):
    return jax.nn.sigmoid(x)

def _layernorm(x, axis=-1, eps=1e-05):
    m = jnp.mean(x, axis=axis, keepdims=True)
    v = jnp.var(x, axis=axis, keepdims=True)
    return (x - m) / jnp.sqrt(v + eps)

def _scatter_add(tgt, idx, src, axis=0):
    return tgt.at[idx].add(src)

def _segment_sum(src, seg, n):
    return jax.ops.segment_sum(src, seg, n)

class _Rng:

    def __init__(self, key):
        self._k = key

    def _next(self):
        self._k, sub = jax.random.split(self._k)
        return sub

    def normal(self, shape):
        return jax.random.normal(self._next(), shape, dtype=jnp.bfloat16)

    def randint(self, lo, hi, shape):
        return jax.random.randint(self._next(), shape, lo, hi, dtype=jnp.int32)

    def uniform(self, shape, lo=0.0, hi=1.0):
        return jax.random.uniform(self._next(), shape, jnp.bfloat16, lo, hi)

    def permutation(self, n):
        return jax.random.permutation(self._next(), n)
kernel_name = 'adaLN_cond__sliding_local_dilated__swiglu_ffn__prompt'

def setup_inputs():
    _rng = _Rng(jax.random.key(int.from_bytes(__import__("os").urandom(4), "little")))
    _w = lambda a: (lambda t: t.astype(jnp.bfloat16) if jnp.issubdtype(t.dtype, jnp.floating) else t)(jnp.asarray(a))

    def _A_setup():
        B, S, D = (1, 2048, 1024)
        return {'x': _w((lambda *s: _rng.normal(s) * 0.05)(B, S, D)), 'wqkv': _w((lambda *s: _rng.normal(s) * 0.05)(D, 3 * D)), 'wo': _w((lambda *s: _rng.normal(s) * 0.05)(D, D))}
    _A_in = _A_setup()

    def _B_setup():
        B, S, D, F = (1, 2048, 1024, 3584)
        return {'x': _w((lambda *s: _rng.normal(s) * 0.05)(B, S, D)), 'w_gate': _w((lambda *s: _rng.normal(s) * 0.05)(D, F)), 'w_up': _w((lambda *s: _rng.normal(s) * 0.05)(D, F)), 'w_down': _w((lambda *s: _rng.normal(s) * 0.05)(F, D))}
    _B_in = _B_setup()
    return {'A_x': _A_in['x'], 'A_wqkv': _A_in['wqkv'], 'A_wo': _A_in['wo'], 'B_x': _B_in['x'], 'B_w_gate': _B_in['w_gate'], 'B_w_up': _B_in['w_up'], 'B_w_down': _B_in['w_down'], 'c': _w((lambda *s: _rng.normal(s) * 0.05)(1, 1024)), 'w_mod': _w((lambda *s: _rng.normal(s) * 0.05)(1024, 6 * 1024) * 1024 ** (-0.5))}

def reference(A_x, A_wqkv, A_wo, B_x, B_w_gate, B_w_up, B_w_down, c, w_mod):

    def _A_ref(x, wqkv, wo):
        B, S, D = x.shape
        H = 32
        Dh = D // H
        W, dil = (8, 2)
        qkv = (lambda x, *d: x.transpose(*d))((x @ wqkv).reshape(B, S, 3, H, Dh), 2, 0, 3, 1, 4)
        q, k, v = (qkv[0], qkv[1], qkv[2])
        scale = Dh ** (-0.5)
        pos = jnp.arange(S)
        off = jnp.arange(W) * dil
        idx = pos[:, None] - off[None, :]
        mask = idx >= 0
        idx_c = jnp.where(mask, idx, 0).reshape(-1)
        kg = k[:, :, idx_c, :].reshape(B, H, S, W, Dh)
        vg = v[:, :, idx_c, :].reshape(B, H, S, W, Dh)
        logits = jnp.einsum('bhsd,bhswd->bhsw', q, kg) * scale
        logits = jnp.where(mask[None, None, :, :], logits, -1000000000.0)
        attn = _softmax(logits, axis=-1)
        o = jnp.einsum('bhsw,bhswd->bhsd', attn, vg)
        return (lambda x, *d: x.transpose(*d))(o, 0, 2, 1, 3).reshape(B, S, D) @ wo

    def _B_ref(x, w_gate, w_up, w_down):
        g = _silu(x @ w_gate)
        u = x @ w_up
        return g * u @ w_down
    x = A_x
    mod = (_silu(c) @ w_mod).reshape(c.shape[0], 6, 1, -1)
    sa, ca, ga, sb, cb, gb = (mod[:, 0].copy(), mod[:, 1].copy(), mod[:, 2].copy(), mod[:, 3].copy(), mod[:, 4].copy(), mod[:, 5].copy())
    h = _layernorm(x, axis=-1) * (1 + ca) + sa
    x = x + ga * _A_ref(h, A_wqkv, A_wo)
    h = _layernorm(x, axis=-1) * (1 + cb) + sb
    x = x + gb * _B_ref(h, B_w_gate, B_w_up, B_w_down)
    return x
```

```python
import jax
import jax.numpy as jnp
import numpy as np
from jax.experimental import pallas as pl
from jax.experimental.pallas import tpu as pltpu

S, D, F = 2048, 1024, 3584
H, DH, W, DIL = 32, 32, 8, 2
HALO = 16
NG = D // 128
TA = 256
TB = 512
FC = 512
RB = 16
LB = 32
EPS = 1e-5
NA, NB, NF = S // TA, S // TB, F // FC
F32, BF16 = jnp.float32, jnp.bfloat16


def _butterfly(cols, stages):
    lane = jax.lax.broadcasted_iota(jnp.int32, cols[0].shape, 1)
    cols = list(cols)
    for s, d in stages:
        low = (lane & s) == 0
        for a in range(NG):
            if a & d:
                continue
            ca, cb = cols[a], cols[a + d]
            cols[a] = jnp.where(low, ca, pltpu.roll(cb, s, 1))
            cols[a + d] = jnp.where(low, pltpu.roll(ca, 128 - s, 1), cb)
    return cols


_FWD = ((16, 1), (8, 2), (4, 4))
_INV = _FWD[::-1]


def _ln_mod(x, scale1, shift):
    m = jnp.mean(x, axis=-1, keepdims=True)
    xc = x - m
    v = jnp.mean(xc * xc, axis=-1, keepdims=True)
    return xc * jax.lax.rsqrt(v + EPS) * scale1 + shift


def _kernel(x_hbm, wqkv_hbm, wo_hbm, wg_hbm, wu_hbm, wd_hbm, c_ref, wmod_hbm, out_hbm,
            xv, wqkv, wo, wg, wu, wd, wmod, sb, mod, hbuf, qb, kb, vb, tb, ob, x1, h2,
            sem_x, sem_qkv, sem_mod, sem_w, sem_out):
    def cp_x(i):
        return pltpu.make_async_copy(x_hbm.at[pl.ds(i * TA, TA)], xv.at[pl.ds(i * TA, TA)], sem_x.at[i])

    def cp_mod(j):
        return pltpu.make_async_copy(wmod_hbm.at[:, pl.ds(j * D, D)], wmod.at[j], sem_mod.at[j])

    def cp_qkv(j):
        return pltpu.make_async_copy(wqkv_hbm.at[:, pl.ds(j * D, D)], wqkv.at[j], sem_qkv.at[j])

    cp_wo = pltpu.make_async_copy(wo_hbm, wo, sem_w.at[0])
    cp_wg = pltpu.make_async_copy(wg_hbm, wg, sem_w.at[1])
    cp_wu = pltpu.make_async_copy(wu_hbm, wu, sem_w.at[2])
    cp_wd = pltpu.make_async_copy(wd_hbm, wd, sem_w.at[3])

    def cp_out(i):
        return pltpu.make_async_copy(xv.at[pl.ds(i * TB, TB)], out_hbm.at[pl.ds(i * TB, TB)], sem_out.at[i])

    first = [cp_mod(0), cp_mod(1), cp_x(0), cp_qkv(0), cp_qkv(1), cp_qkv(2)]
    for cp in first:
        cp.start()

    cv = c_ref[...].astype(F32)
    sc = (cv * jax.nn.sigmoid(cv)).astype(BF16).astype(F32)
    for j in range(NG):
        row = jnp.broadcast_to(sc[:, j * 128:(j + 1) * 128], (128, 128))
        sb[j * 128:(j + 1) * 128, :] = row.T

    def mod_chunk(j, plus_one):
        for g in range(NG):
            acc = jnp.zeros((16, 128), F32)
            for r in range(0, D, 16):
                acc = acc + wmod[j, r:r + 16, g * 128:(g + 1) * 128].astype(F32) * sb[r:r + 16, :]
            res = jnp.sum(acc, axis=0, keepdims=True)
            if plus_one:
                res = res + 1.0
            mod[j, :, g * 128:(g + 1) * 128] = jnp.broadcast_to(res, (8, 128))

    def permute_w(j):
        def body(r, carry):
            r0 = pl.multiple_of(r * 64, 64)
            cols = [pltpu.bitcast(wqkv[j, pl.ds(r0, 64), g * 128:(g + 1) * 128], jnp.uint32) for g in range(NG)]
            cols = _butterfly(cols, _FWD)
            for g in range(NG):
                wqkv[j, pl.ds(r0, 64), g * 128:(g + 1) * 128] = pltpu.bitcast(cols[g], BF16)
            return carry
        jax.lax.fori_loop(0, D // 64, body, 0)

    cp_mod(0).wait()
    mod_chunk(0, False)
    cp_mod(1).wait()
    rest = [cp_x(i) for i in range(1, NA)] + [cp_wo, cp_mod(2), cp_mod(3), cp_mod(4), cp_mod(5), cp_wg, cp_wu, cp_wd]
    for cp in rest:
        cp.start()
    mod_chunk(1, True)
    cp_x(0).wait()

    def ln1(i):
        for r in range(0, TA, LB):
            r0 = pl.multiple_of(i * TA + r, LB)
            xt = xv[pl.ds(r0, LB), :].astype(F32)
            hbuf[r:r + LB, :] = _ln_mod(xt, mod[1, 0:1, :], mod[0, 0:1, :]).astype(BF16)

    qscale = float(DH ** -0.5 * np.log2(np.e))

    def qkv_part(j, slot):
        res = jnp.dot(hbuf[...], wqkv[j], preferred_element_type=F32)
        for g in range(NG):
            blk = res[:, g * 128:(g + 1) * 128]
            if j == 0:
                qb[slot, g] = blk * qscale
            elif j == 1:
                kb[slot, g, HALO:HALO + TA, :] = blk
            else:
                vb[slot, g, HALO:HALO + TA, :] = blk

    ln1(0)
    for j in range(3):
        cp_qkv(j).wait()
        permute_w(j)
        qkv_part(j, 0)
    kb[0, :, 0:HALO, :] = jnp.zeros((NG, HALO, 128), F32)
    vb[0, :, 0:HALO, :] = jnp.zeros((NG, HALO, 128), F32)

    ri = jax.lax.broadcasted_iota(jnp.int32, (128, 128), 0)
    ci = jax.lax.broadcasted_iota(jnp.int32, (128, 128), 1)
    group_ones = jnp.where((ri >> 2) == (ci >> 2), 1.0, 0.0).astype(BF16)

    def attn_logits(slot):
        for r in range(0, TA, RB):
            acc = [None] * W
            for g in range(NG):
                qv = qb[slot, g, r:r + RB, :]
                for w in range(W):
                    o = HALO + r - DIL * w
                    p = qv * kb[slot, g, o:o + RB, :]
                    acc[w] = p if g == 0 else acc[w] + p
            for w in range(W):
                tb[w * TA + r:w * TA + r + RB, :] = acc[w].astype(BF16)

    def attn_out(i, slot, lg):
        for r in range(0, TA, RB):
            pos = i * TA + r + jax.lax.broadcasted_iota(jnp.int32, (RB, 128), 0)
            l = [lg[w * TA + r:w * TA + r + RB, :] for w in range(W)]
            if r < HALO:
                l = [l[0]] + [jnp.where(pos >= DIL * w, l[w], -1e9) for w in range(1, W)]
            m = l[0]
            for w in range(1, W):
                m = jnp.maximum(m, l[w])
            e = [jnp.exp2(l[w] - m) for w in range(W)]
            den = e[0]
            for w in range(1, W):
                den = den + e[w]
            inv = 1.0 / den
            p = [e[w] * inv for w in range(W)]
            cols = []
            for g in range(NG):
                acc = None
                for w in range(W):
                    o = HALO + r - DIL * w
                    t = p[w] * vb[slot, g, o:o + RB, :]
                    acc = t if w == 0 else acc + t
                cols.append(pltpu.bitcast(acc.astype(BF16), jnp.uint32))
            cols = _butterfly(cols, _INV)
            for g in range(NG):
                ob[r:r + RB, g * 128:(g + 1) * 128] = pltpu.bitcast(cols[g], BF16)

    def attn_tail(i):
        a = jnp.dot(ob[...], wo[...], preferred_element_type=F32)
        for r in range(0, TA, LB):
            r0 = pl.multiple_of(i * TA + r, LB)
            xn = xv[pl.ds(r0, LB), :].astype(F32) + mod[2, 0:1, :] * a[r:r + LB, :]
            x1[pl.ds(r0, LB), :] = xn
            h2[pl.ds(r0, LB), :] = _ln_mod(xn, mod[4, 0:1, :], mod[3, 0:1, :]).astype(BF16)

    def step_a(i, slot, has_next):
        if has_next:
            ln1(i + 1)
        attn_logits(slot)
        if has_next:
            qkv_part(0, 1 - slot)
        lg = jnp.dot(tb[...], group_ones, preferred_element_type=F32)
        if has_next:
            qkv_part(1, 1 - slot)
        attn_out(i, slot, lg)
        if has_next:
            qkv_part(2, 1 - slot)
            kb[1 - slot, :, 0:HALO, :] = kb[slot, :, TA:TA + HALO, :]
            vb[1 - slot, :, 0:HALO, :] = vb[slot, :, TA:TA + HALO, :]
        attn_tail(i)

    cp_wo.wait()
    for j in (2, 3, 4):
        cp_mod(j).wait()
        mod_chunk(j, j == 4)

    def loop_a(i, carry):
        pltpu.make_async_copy(x_hbm.at[pl.ds(0, TA)], xv.at[pl.ds(0, TA)], sem_x.at[i + 1]).wait()
        step_a(i, i & 1, True)
        return carry
    jax.lax.fori_loop(0, NA - 1, loop_a, 0)
    step_a(NA - 1, (NA - 1) & 1, False)

    cp_mod(5).wait()
    mod_chunk(5, False)
    cp_wg.wait()
    cp_wu.wait()
    cp_wd.wait()

    def loop_b(i, carry):
        r0 = pl.multiple_of(i * TB, TB)
        hh = h2[pl.ds(r0, TB), :]
        acc = None
        for f in range(NF):
            g = jnp.dot(hh, wg[:, f * FC:(f + 1) * FC], preferred_element_type=F32)
            u = jnp.dot(hh, wu[:, f * FC:(f + 1) * FC], preferred_element_type=F32)
            a = (g * jax.nn.sigmoid(g) * u).astype(BF16)
            d = jnp.dot(a, wd[f * FC:(f + 1) * FC, :], preferred_element_type=F32)
            acc = d if f == 0 else acc + d
        xv[pl.ds(r0, TB), :] = (x1[pl.ds(r0, TB), :] + mod[5, 0:1, :] * acc).astype(BF16)
        pltpu.make_async_copy(xv.at[pl.ds(r0, TB)], out_hbm.at[pl.ds(r0, TB)], sem_out.at[i]).start()
        return carry
    jax.lax.fori_loop(0, NB, loop_b, 0)
    for i in range(NB):
        cp_out(i).wait()


@jax.jit
def pallas_adaLN_cond__sliding_local_dilated__swiglu_ffn__prompt_kernel(
    A_x: jax.Array,
    A_wqkv: jax.Array,
    A_wo: jax.Array,
    B_x: jax.Array,
    B_w_gate: jax.Array,
    B_w_up: jax.Array,
    B_w_down: jax.Array,
    c: jax.Array,
    w_mod: jax.Array,
):
    del B_x
    hbm = pl.BlockSpec(memory_space=pl.ANY)
    out = pl.pallas_call(
        _kernel,
        out_shape=jax.ShapeDtypeStruct((S, D), BF16),
        in_specs=[hbm, hbm, hbm, hbm, hbm, hbm, pl.BlockSpec(memory_space=pltpu.VMEM), hbm],
        out_specs=hbm,
        scratch_shapes=[
            pltpu.VMEM((S, D), BF16),
            pltpu.VMEM((3, D, D), BF16),
            pltpu.VMEM((D, D), BF16),
            pltpu.VMEM((D, F), BF16),
            pltpu.VMEM((D, F), BF16),
            pltpu.VMEM((F, D), BF16),
            pltpu.VMEM((6, D, D), BF16),
            pltpu.VMEM((D, 128), F32),
            pltpu.VMEM((6, 8, D), F32),
            pltpu.VMEM((TA, D), BF16),
            pltpu.VMEM((2, NG, TA, 128), F32),
            pltpu.VMEM((2, NG, HALO + TA, 128), F32),
            pltpu.VMEM((2, NG, HALO + TA, 128), F32),
            pltpu.VMEM((W * TA, 128), BF16),
            pltpu.VMEM((TA, D), BF16),
            pltpu.VMEM((S, D), F32),
            pltpu.VMEM((S, D), BF16),
            pltpu.SemaphoreType.DMA((NA,)),
            pltpu.SemaphoreType.DMA((3,)),
            pltpu.SemaphoreType.DMA((6,)),
            pltpu.SemaphoreType.DMA((4,)),
            pltpu.SemaphoreType.DMA((NB,)),
        ],
        compiler_params=pltpu.CompilerParams(vmem_limit_bytes=110 * 1024 * 1024),
    )(A_x.reshape(S, D), A_wqkv, A_wo, B_w_gate, B_w_up, B_w_down, c, w_mod)
    return out.reshape(1, S, D)
```

```python
import functools

import jax
import jax.numpy as jnp
import numpy as np
from jax.experimental import pallas as pl
from jax.experimental.pallas import tpu as pltpu

S, D, F = 2048, 1024, 3584
H, DH, W, DIL = 32, 32, 8, 2
HALO = 16
NG = D // 128
T = 256
TB = 512
NC = 512
FC = 512
RB = 16
LB = 32
EPS = 1e-5
NT, NB, NF = S // T, S // TB, F // FC
F32, BF16 = jnp.float32, jnp.bfloat16


def _butterfly(cols, stages):
    lane = jax.lax.broadcasted_iota(jnp.int32, cols[0].shape, 1)
    cols = list(cols)
    for s, d in stages:
        low = (lane & s) == 0
        for a in range(NG):
            if a & d:
                continue
            ca, cb = cols[a], cols[a + d]
            cols[a] = jnp.where(low, ca, pltpu.roll(cb, s, 1))
            cols[a + d] = jnp.where(low, pltpu.roll(ca, 128 - s, 1), cb)
    return cols


_FWD = ((16, 1), (8, 2), (4, 4))
_INV = _FWD[::-1]


def _ln_mod(x, scale1, shift):
    m = jnp.mean(x, axis=-1, keepdims=True)
    xc = x - m
    v = jnp.mean(xc * xc, axis=-1, keepdims=True)
    return xc * jax.lax.rsqrt(v + EPS) * scale1 + shift


def _aligned(v, n):
    return v if isinstance(v, int) else pl.multiple_of(v, n)


def _digest(blocks):
    out = None
    for b in blocks:
        for r in range(0, b.shape[0], 16):
            for c in range(0, b.shape[1], 128):
                v = pltpu.bitcast(b[r:r + 16, c:c + 128], jnp.uint32)
                out = v if out is None else out | v
    return pltpu.bitcast(out, BF16)


def _run(tasks):
    for t in tasks:
        t()


def _kernel(x_hbm, wqkv_hbm, wo_hbm, wg_hbm, wu_hbm, wd_hbm, c_ref, wmod_hbm, out_hbm,
            xv, wqkv, wo, wg, wu, wd, wmod, sb, mod, hbuf, qb, kb, vb, tb, lg, ob, ab, act, x1, h2, flag,
            sem_x, sem_qkv, sem_mod, sem_w, sem_out):
    def cp_x(i):
        return pltpu.make_async_copy(x_hbm.at[pl.ds(_aligned(i * T, T), T)], xv.at[pl.ds(_aligned(i * T, T), T)], sem_x.at[i])

    def cp_mod(j):
        return pltpu.make_async_copy(wmod_hbm.at[:, pl.ds(_aligned(j * D, D), D)], wmod.at[j], sem_mod.at[j])

    def cp_qkv(j):
        return pltpu.make_async_copy(wqkv_hbm.at[:, pl.ds(j * D, D)], wqkv.at[j], sem_qkv.at[j])

    cp_wo = pltpu.make_async_copy(wo_hbm, wo, sem_w.at[0])

    def cp_ffn(f):
        c0 = f * FC
        return (pltpu.make_async_copy(wg_hbm.at[:, c0:c0 + FC], wg.at[f], sem_w.at[1 + 3 * f]),
                pltpu.make_async_copy(wu_hbm.at[:, c0:c0 + FC], wu.at[f], sem_w.at[2 + 3 * f]),
                pltpu.make_async_copy(wd_hbm.at[c0:c0 + FC, :], wd.at[f], sem_w.at[3 + 3 * f]))

    def cp_out(b):
        r0 = _aligned(b * TB, TB)
        return pltpu.make_async_copy(xv.at[pl.ds(r0, TB)], out_hbm.at[pl.ds(r0, TB)], sem_out.at[b])

    cp_qkv(0).start()
    cp_mod(0).start()
    flag[0] = 0
    cv = c_ref[...].astype(F32)
    sc = (cv * jax.nn.sigmoid(cv)).astype(BF16).astype(F32)
    for j in range(NG):
        row = jnp.broadcast_to(sc[:, j * 128:(j + 1) * 128], (128, 128))
        sb[j * 128:(j + 1) * 128, :] = row.T

    def mod_chunk(j):
        def body(r, acc):
            r0 = pl.multiple_of(r * 64, 64)
            s = sb[pl.ds(r0, 64), :]
            out = []
            for g in range(NG):
                t = wmod[j, pl.ds(r0, 64), g * 128:(g + 1) * 128].astype(F32) * s
                t = t[0:32] + t[32:64]
                t = t[0:16] + t[16:32]
                out.append(acc[g] + (t[0:8] + t[8:16]))
            return tuple(out)
        acc = jax.lax.fori_loop(0, D // 64, body, tuple(jnp.zeros((8, 128), F32) for _ in range(NG)))
        one = jnp.where((j == 1) | (j == 4), 1.0, 0.0)
        for g in range(NG):
            res = jnp.sum(acc[g], axis=0, keepdims=True) + one
            mod[j, :, g * 128:(g + 1) * 128] = jnp.broadcast_to(res, (8, 128))

    def permute_piece(j, r):
        cols = [pltpu.bitcast(wqkv[j, pl.ds(r, 32), g * 128:(g + 1) * 128], jnp.uint32) for g in range(NG)]
        cols = _butterfly(cols, _FWD)
        for g in range(NG):
            wqkv[j, pl.ds(r, 32), g * 128:(g + 1) * 128] = pltpu.bitcast(cols[g], BF16)
        return _digest([pltpu.bitcast(c, BF16) for c in cols])

    def ln1_piece(i, slot, r):
        r0 = _aligned(i * T + r, LB)
        xt = xv[pl.ds(r0, LB), :].astype(F32)
        hv = _ln_mod(xt, mod[1, 0:1, :], mod[0, 0:1, :]).astype(BF16)
        hbuf[slot, pl.ds(r, LB), :] = hv
        return _digest([hv])

    qscale = float(DH ** -0.5 * np.log2(np.e))

    def qkv_piece(slot, j, n):
        res = jnp.dot(hbuf[slot], wqkv[j, :, n * NC:(n + 1) * NC], preferred_element_type=F32)
        for gg in range(NC // 128):
            g = n * (NC // 128) + gg
            blk = res[:, gg * 128:(gg + 1) * 128]
            if j == 0:
                qb[slot, g] = blk * qscale
            elif j == 1:
                kb[slot, g, HALO:HALO + T, :] = blk
            else:
                vb[slot, g, HALO:HALO + T, :] = blk

    def halo_copy(slot):
        kb[1 - slot, :, 0:HALO, :] = kb[slot, :, T:T + HALO, :]
        vb[1 - slot, :, 0:HALO, :] = vb[slot, :, T:T + HALO, :]

    def logits_piece(slot, r):
        acc = [None] * W
        for g in range(NG):
            qv = qb[slot, g, r:r + RB, :]
            for w in range(W):
                o = HALO + r - DIL * w
                p = qv * kb[slot, g, o:o + RB, :]
                acc[w] = p if g == 0 else acc[w] + p
        for w in range(W):
            tb[r * W + w * RB:r * W + (w + 1) * RB, :] = acc[w].astype(BF16)
        return _digest([a.astype(BF16) for a in acc])

    def groupsum_piece(r0, r1):
        ri = jax.lax.broadcasted_iota(jnp.int32, (128, 128), 0)
        ci = jax.lax.broadcasted_iota(jnp.int32, (128, 128), 1)
        group_ones = jnp.where((ri >> 2) == (ci >> 2), 1.0, 0.0).astype(BF16)
        lg[r0 * W:r1 * W, :] = jnp.dot(tb[r0 * W:r1 * W, :], group_ones, preferred_element_type=F32)

    def out_piece(i, slot, r):
        l = [lg[r * W + w * RB:r * W + (w + 1) * RB, :] for w in range(W)]
        if r < HALO and not (isinstance(i, int) and i > 0):
            pos = i * T + r + jax.lax.broadcasted_iota(jnp.int32, (RB, 128), 0)
            l = [l[0]] + [jnp.where(pos >= DIL * w, l[w], -1e9) for w in range(1, W)]
        m = l[0]
        for w in range(1, W):
            m = jnp.maximum(m, l[w])
        e = [jnp.exp2(l[w] - m) for w in range(W)]
        den = e[0]
        for w in range(1, W):
            den = den + e[w]
        inv = 1.0 / den
        p = [e[w] * inv for w in range(W)]
        cols = []
        for g in range(NG):
            acc = None
            for w in range(W):
                o = HALO + r - DIL * w
                t = p[w] * vb[slot, g, o:o + RB, :]
                acc = t if w == 0 else acc + t
            cols.append(pltpu.bitcast(acc.astype(BF16), jnp.uint32))
        cols = _butterfly(cols, _INV)
        for g in range(NG):
            ob[r:r + RB, g * 128:(g + 1) * 128] = pltpu.bitcast(cols[g], BF16)
        return _digest([pltpu.bitcast(c, BF16) for c in cols])

    def wo_piece(n):
        ab[:, n * NC:(n + 1) * NC] = jnp.dot(ob[...], wo[:, n * NC:(n + 1) * NC], preferred_element_type=F32)

    def tail_piece(i, r):
        r0 = _aligned(i * T + r, LB)
        xn = xv[pl.ds(r0, LB), :].astype(F32) + mod[2, 0:1, :] * ab[r:r + LB, :]
        x1[pl.ds(r0, LB), :] = xn
        hv = _ln_mod(xn, mod[4, 0:1, :], mod[3, 0:1, :]).astype(BF16)
        h2[pl.ds(r0, LB), :] = hv
        return _digest([hv])

    def anchor(tasks, w_ref, col0, never):
        for n, task in enumerate(tasks):
            col, k = divmod(n * 8 // len(tasks), 2)
            r, c = k * 512, col0 + col * 128
            w_ref[r:r + 16, c:c + 128] = jnp.where(never, task(), w_ref[r:r + 16, c:c + 128])

    def tasks(fn, step, *args):
        return [functools.partial(fn, *args, r) for r in range(0, T, step)]

    def never_mask():
        return jnp.full((16, 128), flag[0], jnp.int32) > 0

    def gate_up(b, f, under_gate=(), between=(), under_up=(), never=None):
        r0 = _aligned(b * TB, TB)
        if under_gate:
            anchor(under_gate, wg.at[f], 0, never)
        g = jnp.dot(h2[pl.ds(r0, TB), :], wg[f], preferred_element_type=F32)
        _run(between)
        if under_up:
            anchor(under_up, wu.at[f], 0, never)
        u = jnp.dot(h2[pl.ds(r0, TB), :], wu[f], preferred_element_type=F32)
        hg = 0.5 * g
        act[...] = ((hg * jnp.tanh(hg) + hg) * u).astype(BF16)

    def down(b, f):
        r0 = _aligned(b * TB, TB)
        d = jnp.dot(act[...], wd[f], preferred_element_type=F32)
        xn = x1[pl.ds(r0, TB), :] + mod[5, 0:1, :] * d
        x1[pl.ds(r0, TB), :] = xn
        xv[pl.ds(r0, TB), :] = xn.astype(BF16)

    gs = [functools.partial(groupsum_piece, r, r + T // 4) for r in range(0, T, T // 4)]

    ab[...] = jnp.zeros((T, D), F32)
    kb[0, :, 0:HALO, :] = jnp.zeros((NG, HALO, 128), F32)
    vb[0, :, 0:HALO, :] = jnp.zeros((NG, HALO, 128), F32)
    cp_qkv(0).wait()
    cp_mod(1).start()
    cp_x(0).start()

    def permute_q(r, carry):
        for u in range(4):
            permute_piece(0, pl.multiple_of(r * 128 + u * 32, 32))
        return carry
    jax.lax.fori_loop(0, D // 128, permute_q, 0)
    cp_qkv(1).start()
    cp_x(1).start()

    def mod_first(j, carry):
        cp_mod(j).wait()
        mod_chunk(j)
        return carry
    jax.lax.fori_loop(0, 2, mod_first, 0)
    cp_qkv(2).start()
    cp_x(0).wait()
    cp_x(1).wait()

    def ln_first(n, carry):
        for u in range(2):
            ln1_piece(n // (T // 64), n // (T // 64), pl.multiple_of((n % (T // 64)) * 64 + u * LB, LB))
        return carry
    jax.lax.fori_loop(0, 2 * T // 64, ln_first, 0)
    for cp in (cp_wo, cp_mod(2), cp_mod(3), cp_mod(4), cp_x(2)):
        cp.start()
    never = never_mask()
    for j in range(3):
        if j < 2:
            cp_qkv(j + 1).wait()
        if j == 1:
            for cp in tuple(cp_x(i) for i in range(3, NT)) + (cp_mod(5),):
                cp.start()
        for n in range(2):
            if j < 2:
                anchor([functools.partial(permute_piece, j + 1, r) for r in range(n * 512, n * 512 + 512, 32)],
                       wqkv.at[j], n * NC, never)
            qkv_piece(0, j, n)
    cp_wo.wait()

    def mod_rest(j, carry):
        cp_mod(j).wait()
        mod_chunk(j)
        return carry
    jax.lax.fori_loop(2, 5, mod_rest, 0)
    for f in range(NF):
        for cp in cp_ffn(f):
            cp.start()

    def step_a(i, carry):
        @pl.when(i + 2 < NT)
        def _():
            cp_x(i + 2).wait()
        slot = i & 1
        never = never_mask()
        lo, ou = tasks(logits_piece, RB, slot), tasks(out_piece, RB, i, slot)
        ta = tasks(tail_piece, LB, jnp.maximum(i - 1, 0))
        l1 = tasks(ln1_piece, LB, jnp.minimum(i + 2, NT - 1), slot)
        under = (lo[:8], lo[8:], ta, ou[:5], ou[5:10], ou[10:])
        for j in range(3):
            for n in range(2):
                anchor(under[2 * j + n], wqkv.at[j], n * NC, never)
                qkv_piece(1 - slot, j, n)
            if j == 0:
                _run(gs)
        halo_copy(slot)
        for n in range(2):
            anchor(l1[4 * n:4 * n + 4], wo, n * NC, never)
            wo_piece(n)
        return carry
    jax.lax.fori_loop(0, NT - 1, step_a, 0)

    for cp in cp_ffn(0)[:2]:
        cp.wait()
    last, never = NT - 1, never_mask()
    gate_up(0, 0, tasks(logits_piece, RB, last & 1), gs,
            tasks(tail_piece, LB, last - 1) + tasks(out_piece, RB, last, last & 1), never)
    for n in range(2):
        wo_piece(n)
    _run(tasks(tail_piece, LB, last))
    mod_rest(5, 0)
    for f in range(NF):
        for cp in cp_ffn(f)[2 if f == 0 else 0:]:
            cp.wait()

    def step_b(n, carry):
        bp, fp = (n - 1) // NF, (n - 1) % NF
        down(bp, fp)
        gate_up(n // NF, n % NF)

        @pl.when(fp == NF - 1)
        def _():
            cp_out(bp).start()
        return carry
    jax.lax.fori_loop(1, NB * NF, step_b, 0)
    down(NB - 1, NF - 1)
    cp_out(NB - 1).start()
    for b in range(NB):
        cp_out(b).wait()


@jax.jit
def pallas_adaLN_cond__sliding_local_dilated__swiglu_ffn__prompt_kernel(
    A_x: jax.Array,
    A_wqkv: jax.Array,
    A_wo: jax.Array,
    B_x: jax.Array,
    B_w_gate: jax.Array,
    B_w_up: jax.Array,
    B_w_down: jax.Array,
    c: jax.Array,
    w_mod: jax.Array,
):
    del B_x
    hbm = pl.BlockSpec(memory_space=pl.ANY)
    out = pl.pallas_call(
        _kernel,
        out_shape=jax.ShapeDtypeStruct((S, D), BF16),
        grid=(1,),
        in_specs=[hbm, hbm, hbm, hbm, hbm, hbm, pl.BlockSpec((1, D), lambda i: (0, 0)), hbm],
        out_specs=hbm,
        scratch_shapes=[
            pltpu.VMEM((S, D), BF16),
            pltpu.VMEM((3, D, D), BF16),
            pltpu.VMEM((D, D), BF16),
            pltpu.VMEM((NF, D, FC), BF16),
            pltpu.VMEM((NF, D, FC), BF16),
            pltpu.VMEM((NF, FC, D), BF16),
            pltpu.VMEM((6, D, D), BF16),
            pltpu.VMEM((D, 128), F32),
            pltpu.VMEM((6, 8, D), F32),
            pltpu.VMEM((2, T, D), BF16),
            pltpu.VMEM((2, NG, T, 128), F32),
            pltpu.VMEM((2, NG, HALO + T, 128), F32),
            pltpu.VMEM((2, NG, HALO + T, 128), F32),
            pltpu.VMEM((W * T, 128), BF16),
            pltpu.VMEM((W * T, 128), F32),
            pltpu.VMEM((T, D), BF16),
            pltpu.VMEM((T, D), F32),
            pltpu.VMEM((TB, FC), BF16),
            pltpu.VMEM((S, D), F32),
            pltpu.VMEM((S, D), BF16),
            pltpu.SMEM((1,), jnp.int32),
            pltpu.SemaphoreType.DMA((NT,)),
            pltpu.SemaphoreType.DMA((3,)),
            pltpu.SemaphoreType.DMA((6,)),
            pltpu.SemaphoreType.DMA((1 + 3 * NF,)),
            pltpu.SemaphoreType.DMA((NB,)),
        ],
        compiler_params=pltpu.CompilerParams(vmem_limit_bytes=110 * 1024 * 1024),
    )(A_x.reshape(S, D), A_wqkv, A_wo, B_w_gate, B_w_up, B_w_down, c, w_mod)
    return out.reshape(1, S, D)
```

```python
import functools

import jax
import jax.numpy as jnp
import numpy as np
from jax.experimental import pallas as pl
from jax.experimental.pallas import tpu as pltpu

S, D, F = 2048, 1024, 3584
H, DH, W, DIL = 32, 32, 8, 2
HALO = 16
NG = D // 128
T = 256
TB = 512
PB = 64
FC = 512
RB = 16
LB = 32
LAG = 2
EPS = 1e-5
NT, NB, NF = S // T, S // TB, F // FC
F32, BF16 = jnp.float32, jnp.bfloat16


def _butterfly(cols, stages):
    lane = jax.lax.broadcasted_iota(jnp.int32, cols[0].shape, 1)
    cols = list(cols)
    for s, d in stages:
        low = (lane & s) == 0
        for a in range(NG):
            if a & d:
                continue
            ca, cb = cols[a], cols[a + d]
            cols[a] = jnp.where(low, ca, pltpu.roll(cb, s, 1))
            cols[a + d] = jnp.where(low, pltpu.roll(ca, 128 - s, 1), cb)
    return cols


_FWD = ((16, 1), (8, 2), (4, 4))
_INV = _FWD[::-1]


def _ln_mod(x, scale1, shift):
    m = jnp.mean(x, axis=-1, keepdims=True)
    xc = x - m
    v = jnp.mean(xc * xc, axis=-1, keepdims=True)
    return xc * jax.lax.rsqrt(v + EPS) * scale1 + shift


def _aligned(v, n):
    return v if isinstance(v, int) else pl.multiple_of(v, n)


def _digest(blocks):
    out = None
    for b in blocks:
        for r in range(0, b.shape[0], 16):
            for c in range(0, b.shape[1], 128):
                v = pltpu.bitcast(b[r:r + 16, c:c + 128], jnp.uint32)
                out = v if out is None else out | v
    return pltpu.bitcast(out, BF16)


def _gated(x, gate):
    if gate is None:
        return x
    never, v = gate
    head = jnp.where(never, pltpu.bitcast(v, x.dtype), x[0:8, 0:128])
    if x.shape[1] > 128:
        head = jnp.concatenate([head, x[0:8, 128:]], axis=1)
    return jnp.concatenate([head, x[8:]], axis=0)


def _run(tasks):
    for t in tasks:
        t()


def _kernel(x_hbm, wqkv_hbm, wo_hbm, wg_hbm, wu_hbm, wd_hbm, c_ref, wmod_hbm, out_hbm,
            xv, wraw, wqkv, wo, wg, wu, wd, wmod, sb, mod, hcur, hnext, qb, kb, vb, tb, lg, ob, ab, act, x1, h2, flag,
            sem_x, sem_qkv, sem_mod, sem_w, sem_out):
    def cp_x(i):
        return pltpu.make_async_copy(x_hbm.at[pl.ds(_aligned(i * T, T), T)], xv.at[pl.ds(_aligned(i * T, T), T)], sem_x.at[i])

    def cp_mod(j):
        return pltpu.make_async_copy(wmod_hbm.at[:, pl.ds(_aligned(j * D, D), D)], wmod.at[j], sem_mod.at[j])

    def cp_qkv(j):
        return pltpu.make_async_copy(wqkv_hbm.at[:, pl.ds(j * D, D)], wraw.at[j], sem_qkv.at[j])

    cp_wo = pltpu.make_async_copy(wo_hbm, wo, sem_w.at[0])

    def cp_ffn(f):
        c0 = f * FC
        return (pltpu.make_async_copy(wg_hbm.at[:, c0:c0 + FC], wg.at[f], sem_w.at[1 + 3 * f]),
                pltpu.make_async_copy(wu_hbm.at[:, c0:c0 + FC], wu.at[f], sem_w.at[2 + 3 * f]),
                pltpu.make_async_copy(wd_hbm.at[c0:c0 + FC, :], wd.at[f], sem_w.at[3 + 3 * f]))

    def cp_out(b):
        r0 = _aligned(b * TB, TB)
        return pltpu.make_async_copy(xv.at[pl.ds(r0, TB)], out_hbm.at[pl.ds(r0, TB)], sem_out.at[b])

    cp_qkv(0).start()
    cp_mod(0).start()
    flag[0] = 0
    cv = c_ref[...].astype(F32)
    sc = (cv * jax.nn.sigmoid(cv)).astype(BF16).astype(F32)
    for j in range(NG):
        row = jnp.broadcast_to(sc[:, j * 128:(j + 1) * 128], (128, 128))
        sb[j * 128:(j + 1) * 128, :] = row.T

    def mod_chunk(j):
        def body(r, acc):
            r0 = pl.multiple_of(r * 64, 64)
            s = sb[pl.ds(r0, 64), :]
            out = []
            for g in range(NG):
                t = wmod[j, pl.ds(r0, 64), g * 128:(g + 1) * 128].astype(F32) * s
                t = t[0:32] + t[32:64]
                t = t[0:16] + t[16:32]
                out.append(acc[g] + (t[0:8] + t[8:16]))
            return tuple(out)
        acc = jax.lax.fori_loop(0, D // 64, body, tuple(jnp.zeros((8, 128), F32) for _ in range(NG)))
        one = jnp.where((j == 1) | (j == 4), 1.0, 0.0)
        for g in range(NG):
            res = jnp.sum(acc[g], axis=0, keepdims=True) + one
            mod[j, :, g * 128:(g + 1) * 128] = jnp.broadcast_to(res, (8, 128))

    def permute_piece(j, r, gate=None):
        cols = [pltpu.bitcast(wraw[j, pl.ds(r, PB), g * 128:(g + 1) * 128], jnp.uint32) for g in range(NG)]
        if gate is not None:
            cols = [_gated(c, gate) for c in cols]
        cols = [pltpu.bitcast(c, BF16) for c in _butterfly(cols, _FWD)]
        for g in range(NG):
            wqkv[j, pl.ds(r, PB), g * 128:(g + 1) * 128] = cols[g]
        return _digest(cols)

    def ln1_piece(i, dst, r, gate=None):
        r0 = _aligned(i * T + r, LB)
        xt = _gated(xv[pl.ds(r0, LB), :].astype(F32), gate)
        hv = _ln_mod(xt, mod[1, 0:1, :], mod[0, 0:1, :]).astype(BF16)
        dst[pl.ds(r, LB), :] = hv
        return _digest([hv])

    qscale = float(DH ** -0.5 * np.log2(np.e))

    def qkv_dot(h, slot, j, g):
        res = jnp.dot(h, wqkv[j, :, g * 128:(g + 1) * 128], preferred_element_type=F32)
        if j == 0:
            qb[slot, g] = res * qscale
        else:
            buf = kb if j == 1 else vb
            buf[slot, g, HALO:HALO + T, :] = res
            buf[1 - slot, g, 0:HALO, :] = res[T - HALO:, :]
        return res

    def logits_piece(slot, r, gate=None):
        acc = [None] * W
        for g in range(NG):
            qv = qb[slot, g, r:r + RB, :]
            if g == 0:
                qv = _gated(qv, gate)
            for w in range(W):
                o = HALO + r - DIL * w
                p = qv * kb[slot, g, o:o + RB, :]
                acc[w] = p if g == 0 else acc[w] + p
        acc = [a.astype(BF16) for a in acc]
        for w in range(W):
            tb[r * W + w * RB:r * W + (w + 1) * RB, :] = acc[w]
        return _digest(acc)

    def groupsum_piece(r0, r1):
        ri = jax.lax.broadcasted_iota(jnp.int32, (128, 128), 0)
        ci = jax.lax.broadcasted_iota(jnp.int32, (128, 128), 1)
        group_ones = jnp.where((ri >> 2) == (ci >> 2), 1.0, 0.0).astype(BF16)
        lg[r0 * W:r1 * W, :] = jnp.dot(tb[r0 * W:r1 * W, :], group_ones, preferred_element_type=F32)

    def out_piece(i, slot, r, gate=None):
        l = [lg[r * W + w * RB:r * W + (w + 1) * RB, :] for w in range(W)]
        if r < HALO and not (isinstance(i, int) and i > 0):
            pos = i * T + r + jax.lax.broadcasted_iota(jnp.int32, (RB, 128), 0)
            l = [l[0]] + [jnp.where(pos >= DIL * w, l[w], -1e9) for w in range(1, W)]
        l[0] = _gated(l[0], gate)
        m = l[0]
        for w in range(1, W):
            m = jnp.maximum(m, l[w])
        e = [jnp.exp2(l[w] - m) for w in range(W)]
        den = e[0]
        for w in range(1, W):
            den = den + e[w]
        inv = 1.0 / den
        p = [e[w] * inv for w in range(W)]
        cols = []
        for g in range(NG):
            acc = None
            for w in range(W):
                o = HALO + r - DIL * w
                t = p[w] * vb[slot, g, o:o + RB, :]
                acc = t if w == 0 else acc + t
            cols.append(pltpu.bitcast(acc.astype(BF16), jnp.uint32))
        cols = _butterfly(cols, _INV)
        for g in range(NG):
            ob[r:r + RB, g * 128:(g + 1) * 128] = pltpu.bitcast(cols[g], BF16)
        return _digest([pltpu.bitcast(c, BF16) for c in cols])

    def wo_dot(st, dst, g):
        if g == 0:
            st['o'] = ob[...]
        res = jnp.dot(st['o'], wo[:, g * 128:(g + 1) * 128], preferred_element_type=F32)
        dst[:, g * 128:(g + 1) * 128] = res
        return res

    def tail_piece(i, r, gate=None):
        src = ab.at[i & 1]
        r0 = _aligned(i * T + r, LB)
        xn = xv[pl.ds(r0, LB), :].astype(F32) + mod[2, 0:1, :] * _gated(src[r:r + LB, :], gate)
        x1[pl.ds(r0, LB), :] = xn
        hv = _ln_mod(xn, mod[4, 0:1, :], mod[3, 0:1, :]).astype(BF16)
        h2[pl.ds(r0, LB), :] = hv
        return _digest([hv])

    def tasks(fn, step, *args):
        return [functools.partial(fn, *args, r) for r in range(0, T, step)]

    def stream(dots, under, after=None):
        never = never_mask()
        prev, out = None, []
        for s, (fn, _, _) in enumerate(dots):
            out.append(fn())
            for task in under[s]:
                dig = task(gate=None if prev is None else (never[0:8], prev))
                if s + LAG < len(dots):
                    _, w_ref, c = dots[s + LAG]
                    w_ref[0:16, c:c + 128] = jnp.where(never, dig, w_ref[0:16, c:c + 128])
            if after is not None and s in after:
                after[s]()
            prev = out[-1][-8:, :]
        return out

    def qkv_dots(slot, src, js):
        h = src[...]
        return [(functools.partial(qkv_dot, h, slot, j, g), wqkv.at[j], g * 128) for j in js for g in range(NG)]

    def wo_dots(i):
        st = {}
        return [(functools.partial(wo_dot, st, ab.at[i & 1], g), wo, g * 128) for g in range(NG)]

    def never_mask():
        return jnp.full((16, 128), flag[0], jnp.int32) > 0

    def swiglu(g, u):
        hg = 0.5 * g
        return ((hg * jnp.tanh(hg) + hg) * u).astype(BF16)

    def gate_up(b, f):
        r0 = _aligned(b * TB, TB)
        h = h2[pl.ds(r0, TB), :]
        g = jnp.dot(h, wg[f], preferred_element_type=F32)
        u = jnp.dot(h, wu[f], preferred_element_type=F32)
        act[...] = swiglu(g, u)

    def down(b, f):
        r0 = _aligned(b * TB, TB)
        d = jnp.dot(act[...], wd[f], preferred_element_type=F32)
        xn = x1[pl.ds(r0, TB), :] + mod[5, 0:1, :] * d
        x1[pl.ds(r0, TB), :] = xn
        xv[pl.ds(r0, TB), :] = xn.astype(BF16)

    gs = [functools.partial(groupsum_piece, r, r + T // 4) for r in range(0, T, T // 4)]

    kb[0, :, 0:HALO, :] = jnp.zeros((NG, HALO, 128), F32)
    vb[0, :, 0:HALO, :] = jnp.zeros((NG, HALO, 128), F32)
    ab[0] = jnp.zeros((T, D), F32)
    cp_qkv(0).wait()
    cp_mod(1).start()
    cp_x(0).start()

    def permute_q(r, carry):
        for u in range(128 // PB):
            permute_piece(0, pl.multiple_of(r * 128 + u * PB, PB))
        return carry
    jax.lax.fori_loop(0, D // 128, permute_q, 0)
    cp_qkv(1).start()
    cp_x(1).start()

    def mod_first(j, carry):
        cp_mod(j).wait()
        mod_chunk(j)
        return carry
    jax.lax.fori_loop(0, 2, mod_first, 0)
    cp_qkv(2).start()
    cp_x(0).wait()
    cp_x(1).wait()

    def ln_first(n, carry):
        for t, dst in enumerate((hcur, hnext)):
            ln1_piece(t, dst, pl.multiple_of(n * LB, LB))
        return carry
    jax.lax.fori_loop(0, T // LB, ln_first, 0)
    for cp in (cp_wo, cp_mod(2), cp_mod(3), cp_mod(4), cp_x(2)):
        cp.start()
    for j in range(2):
        cp_qkv(j + 1).wait()
        pm = [functools.partial(permute_piece, j + 1, r) for r in range(0, D, PB)]
        n = len(pm) // NG
        stream(qkv_dots(0, hcur, (j,)), [pm[g * n:(g + 1) * n] for g in range(NG)])
    for cp in tuple(cp_x(i) for i in range(3, NT)) + (cp_mod(5),):
        cp.start()
    lo = tasks(logits_piece, RB, 0)
    stream(qkv_dots(0, hcur, (2,)), [lo[2 * g:2 * g + 2] for g in range(NG)])
    _run(gs)
    cp_wo.wait()

    def mod_rest(j, carry):
        cp_mod(j).wait()
        mod_chunk(j)
        return carry
    jax.lax.fori_loop(2, 5, mod_rest, 0)
    for f in range(NF):
        for cp in cp_ffn(f):
            cp.start()

    def step_a(i, carry):
        @pl.when(i + 2 < NT)
        def _():
            cp_x(i + 2).wait()
        slot = i & 1
        ou = tasks(out_piece, RB, i, slot)
        l1 = tasks(ln1_piece, LB, jnp.minimum(i + 2, NT - 1), hnext)
        ta = tasks(tail_piece, LB, jnp.maximum(i - 1, 0))
        lo = tasks(logits_piece, RB, 1 - slot)
        under = [[ou[s]] + ([l1[s // 2]] if s & 1 else []) for s in range(16)]
        under += [[ta[k], lo[k]] for k in range(8)]
        under += [lo[8:10], lo[10:12], lo[12:13], lo[13:14], lo[14:15], lo[15:16], [], []]
        stream(qkv_dots(1 - slot, hnext, range(3)) + wo_dots(i), under, {25: gs[0], 27: gs[1], 29: gs[2], 31: gs[3]})
        return carry
    jax.lax.fori_loop(0, NT - 1, step_a, 0)

    for cp in cp_ffn(0)[:2]:
        cp.wait()
    last = NT - 1

    h0 = h2[0:TB, :]

    def ffn_dot(w_ref, g):
        return jnp.dot(h0, w_ref[0, :, g * 128:(g + 1) * 128], preferred_element_type=F32)

    nc = FC // 128
    ou, t6, t7 = tasks(out_piece, RB, last, last & 1), tasks(tail_piece, LB, last - 1), tasks(tail_piece, LB, last)
    gd, ud = [[(functools.partial(ffn_dot, w, g), w.at[0], g * 128) for g in range(nc)] for w in (wg, wu)]
    res = stream(gd + ud[:2] + wo_dots(last) + ud[2:],
                 [ou[3 * k:3 * k + 3] for k in range(6)] + [t6[k:k + 1] for k in range(NG)] + [t7[:4], t7[4:]])
    for g, u in enumerate(res[nc:nc + 2] + res[-2:]):
        act[:, g * 128:(g + 1) * 128] = swiglu(res[g], u)
    mod_rest(5, 0)
    for f in range(NF):
        for cp in cp_ffn(f)[2 if f == 0 else 0:]:
            cp.wait()

    def step_b(n, carry):
        bp, fp = (n - 1) // NF, (n - 1) % NF
        down(bp, fp)
        gate_up(n // NF, n % NF)

        @pl.when(fp == NF - 1)
        def _():
            cp_out(bp).start()
        return carry
    jax.lax.fori_loop(1, NB * NF, step_b, 0)
    down(NB - 1, NF - 1)
    cp_out(NB - 1).start()
    for b in range(NB):
        cp_out(b).wait()


@jax.jit
def pallas_adaLN_cond__sliding_local_dilated__swiglu_ffn__prompt_kernel(
    A_x: jax.Array,
    A_wqkv: jax.Array,
    A_wo: jax.Array,
    B_x: jax.Array,
    B_w_gate: jax.Array,
    B_w_up: jax.Array,
    B_w_down: jax.Array,
    c: jax.Array,
    w_mod: jax.Array,
):
    del B_x
    hbm = pl.BlockSpec(memory_space=pl.ANY)
    out = pl.pallas_call(
        _kernel,
        out_shape=jax.ShapeDtypeStruct((S, D), BF16),
        grid=(1,),
        in_specs=[hbm, hbm, hbm, hbm, hbm, hbm, pl.BlockSpec((1, D), lambda i: (0, 0)), hbm],
        out_specs=hbm,
        scratch_shapes=[
            pltpu.VMEM((S, D), BF16),
            pltpu.VMEM((3, D, D), BF16),
            pltpu.VMEM((3, D, D), BF16),
            pltpu.VMEM((D, D), BF16),
            pltpu.VMEM((NF, D, FC), BF16),
            pltpu.VMEM((NF, D, FC), BF16),
            pltpu.VMEM((NF, FC, D), BF16),
            pltpu.VMEM((6, D, D), BF16),
            pltpu.VMEM((D, 128), F32),
            pltpu.VMEM((6, 8, D), F32),
            pltpu.VMEM((T, D), BF16),
            pltpu.VMEM((T, D), BF16),
            pltpu.VMEM((2, NG, T, 128), F32),
            pltpu.VMEM((2, NG, HALO + T, 128), F32),
            pltpu.VMEM((2, NG, HALO + T, 128), F32),
            pltpu.VMEM((W * T, 128), BF16),
            pltpu.VMEM((W * T, 128), F32),
            pltpu.VMEM((T, D), BF16),
            pltpu.VMEM((2, T, D), F32),
            pltpu.VMEM((TB, FC), BF16),
            pltpu.VMEM((S, D), F32),
            pltpu.VMEM((S, D), BF16),
            pltpu.SMEM((1,), jnp.int32),
            pltpu.SemaphoreType.DMA((NT,)),
            pltpu.SemaphoreType.DMA((3,)),
            pltpu.SemaphoreType.DMA((6,)),
            pltpu.SemaphoreType.DMA((1 + 3 * NF,)),
            pltpu.SemaphoreType.DMA((NB,)),
        ],
        compiler_params=pltpu.CompilerParams(vmem_limit_bytes=110 * 1024 * 1024),
    )(A_x.reshape(S, D), A_wqkv, A_wo, B_w_gate, B_w_up, B_w_down, c, w_mod)
    return out.reshape(1, S, D)
```

```python
import functools

import jax
import jax.numpy as jnp
import numpy as np
from jax.experimental import pallas as pl
from jax.experimental.pallas import tpu as pltpu

S, D, F = 2048, 1024, 3584
H, DH, W, DIL = 32, 32, 8, 2
HALO = 16
NG = D // 128
T = 256
TB = 1024
PB = 64
FC = 512
RB = 16
LB = 32
LAG = 3
KH = 1024
ZB = 256
EPS = 1e-5
NT, NB, NF = S // T, S // TB, F // FC
F32, BF16 = jnp.float32, jnp.bfloat16


def _spread_rows(v):
    sub = jax.lax.broadcasted_iota(jnp.int32, v[0].shape, 0)
    v = list(v)
    for s, d in ((4, 2), (2, 1)):
        low = (sub & s) == 0
        for a in range(4):
            if not a & d:
                va, vb = v[a], v[a + d]
                v[a] = jnp.where(low, va, pltpu.roll(vb, s, 0))
                v[a + d] = jnp.where(low, pltpu.roll(va, 8 - s, 0), vb)
    return v


def _spread_heads(cols):
    sub = (jax.lax.broadcasted_iota(jnp.int32, cols[0].shape, 1) >> 2) & 7
    out = [None] * NG
    for d in range(1 - NG, NG):
        js = [j for j in range(NG) if 0 <= j - d < NG]
        diag = cols[js[0]]
        for j in js[1:]:
            diag = jnp.where(sub == j - d, cols[j], diag)
        if d:
            diag = pltpu.roll(diag, (4 * d) % 128, 1)
        for j in js:
            out[j - d] = diag if out[j - d] is None else jnp.where(sub == j, diag, out[j - d])
    return out


def _ln_mod(x, scale1, shift):
    m = jnp.mean(x, axis=-1, keepdims=True)
    xc = x - m
    v = jnp.mean(xc * xc, axis=-1, keepdims=True)
    return xc * jax.lax.rsqrt(v + EPS) * scale1 + shift


def _aligned(v, n):
    return v if isinstance(v, int) else pl.multiple_of(v, n)


def _digest(blocks):
    out = None
    for b in blocks:
        for r in range(0, b.shape[0], 16):
            for c in range(0, b.shape[1], 128):
                v = pltpu.bitcast(b[r:r + 16, c:c + 128], jnp.uint32)
                out = v if out is None else out | v
    return pltpu.bitcast(out, BF16)


def _gated(x, gate):
    if gate is None:
        return x
    never, v = gate
    head = jnp.where(never, pltpu.bitcast(v, x.dtype), x[0:8, 0:128])
    if x.shape[1] > 128:
        head = jnp.concatenate([head, x[0:8, 128:]], axis=1)
    return jnp.concatenate([head, x[8:]], axis=0)


def _run(tasks):
    for t in tasks:
        t()


def _kernel(x_hbm, wqkv_hbm, wo_hbm, wg_hbm, wu_hbm, wd_hbm, c_ref, wmod_hbm, out_hbm,
            xv, wraw, wqkv, wo, wg, wu, wd, wmod, sb, mod, hcur, hnext, qb, kb, vb, tb, lg, ob, ab, act, x1, h2, flag,
            sem_x, sem_qkv, sem_mod, sem_w, sem_out):
    def cp_x(i):
        return pltpu.make_async_copy(x_hbm.at[pl.ds(_aligned(i * T, T), T)], xv.at[pl.ds(_aligned(i * T, T), T)], sem_x.at[i])

    def cp_mod(j):
        return pltpu.make_async_copy(wmod_hbm.at[:, pl.ds(_aligned(j * D, D), D)], wmod.at[j], sem_mod.at[j])

    def cp_qkv(j):
        return pltpu.make_async_copy(wqkv_hbm.at[:, pl.ds(_aligned(j * D, D), D)], wraw.at[j], sem_qkv.at[j])

    cp_wo = pltpu.make_async_copy(wo_hbm, wraw.at[0], sem_w.at[0])

    def cp_ffn(f):
        c0 = f * FC
        return (pltpu.make_async_copy(wg_hbm.at[:, c0:c0 + FC], wg.at[f], sem_w.at[1 + 3 * f]),
                pltpu.make_async_copy(wu_hbm.at[:, c0:c0 + FC], wu.at[f], sem_w.at[2 + 3 * f]),
                pltpu.make_async_copy(wd_hbm.at[c0:c0 + FC, :], wd.at[f], sem_w.at[3 + 3 * f]))

    def cp_out(row0, rows, k):
        return pltpu.make_async_copy(xv.at[pl.ds(row0, rows)], out_hbm.at[pl.ds(row0, rows)], sem_out.at[k])

    cp_qkv(0).start()
    cp_mod(0).start()
    flag[0] = 0
    cv = c_ref[...].astype(F32)
    sc = (cv * jax.nn.sigmoid(cv)).astype(BF16).astype(F32)
    for j in range(NG):
        row = jnp.broadcast_to(sc[:, j * 128:(j + 1) * 128], (128, 128))
        sb[j * 128:(j + 1) * 128, :] = row.T

    def mod_chunk(j):
        def body(r, acc):
            r0 = pl.multiple_of(r * 64, 64)
            s = sb[pl.ds(r0, 64), :]
            out = []
            for g in range(NG):
                t = wmod[j, pl.ds(r0, 64), g * 128:(g + 1) * 128].astype(F32) * s
                t = t[0:32] + t[32:64]
                t = t[0:16] + t[16:32]
                out.append(acc[g] + (t[0:8] + t[8:16]))
            return tuple(out)
        acc = jax.lax.fori_loop(0, D // 64, body, tuple(jnp.zeros((8, 128), F32) for _ in range(NG)))
        one = jnp.where((j == 1) | (j == 4), 1.0, 0.0)
        for g in range(NG):
            res = jnp.sum(acc[g], axis=0, keepdims=True) + one
            mod[j, :, g * 128:(g + 1) * 128] = jnp.broadcast_to(res, (8, 128))

    def mod_rows(j, rows):
        return jnp.concatenate([mod[j]] * (rows // 8), axis=0)

    def permute_piece(j, r, gate=None):
        cols = [pltpu.bitcast(wraw[j, pl.ds(r, PB), g * 128:(g + 1) * 128], jnp.uint32) for g in range(NG)]
        if gate is not None:
            cols = [_gated(c, gate) for c in cols]
        cols = [pltpu.bitcast(c, BF16) for c in _spread_heads(cols)]
        for g in range(NG):
            wqkv[j, pl.ds(r, PB), g * 128:(g + 1) * 128] = cols[g]
        return _digest(cols)

    def ln1_piece(i, dst, r, gate=None):
        r0 = _aligned(i * T + r, LB)
        xt = _gated(xv[pl.ds(r0, LB), :].astype(F32), gate)
        hv = _ln_mod(xt, mod_rows(1, LB), mod_rows(0, LB)).astype(BF16)
        dst[pl.ds(r, LB), :] = hv
        return _digest([hv])

    qscale = float(DH ** -0.5 * np.log2(np.e))

    def qkv_dot(h, slot, j, k, g):
        res = jnp.dot(h[:, k * KH:(k + 1) * KH], wqkv[j, k * KH:(k + 1) * KH, g * 128:(g + 1) * 128],
                      preferred_element_type=F32)
        buf, r0 = ((qb, 0), (kb, HALO), (vb, HALO))[j]
        if k > 0:
            res = res + buf[slot, g, r0:r0 + T, :]
        if k == D // KH - 1:
            if j == 0:
                res = res * qscale
            else:
                buf[1 - slot, g, 0:HALO, :] = res[T - HALO:, :]
        buf[slot, g, r0:r0 + T, :] = res
        return res

    def logits_piece(slot, r, gate=None):
        acc = [None] * W
        for g in range(NG):
            qv = qb[slot, g, r:r + RB, :]
            if g == 0:
                qv = _gated(qv, gate)
            for w in range(W):
                o = HALO + r - DIL * w
                p = qv * kb[slot, g, o:o + RB, :]
                acc[w] = p if g == 0 else acc[w] + p
        acc = [a.astype(BF16) for a in acc]
        for w in range(W):
            tb[r * W + w * RB:r * W + (w + 1) * RB, :] = acc[w]
        return _digest(acc)

    def groupsum_piece(r0, r1):
        ri = jax.lax.broadcasted_iota(jnp.int32, (128, 128), 0)
        ci = jax.lax.broadcasted_iota(jnp.int32, (128, 128), 1)
        group_ones = jnp.where((ri >> 2) == (ci >> 2), 1.0, 0.0).astype(BF16)
        lg[r0 * W:r1 * W, :] = jnp.dot(tb[r0 * W:r1 * W, :], group_ones, preferred_element_type=F32)

    def out_piece(i, slot, r, gate=None):
        l = [lg[r * W + w * RB:r * W + (w + 1) * RB, :] for w in range(W)]
        if r < HALO and not (isinstance(i, int) and i > 0):
            pos = i * T + r + jax.lax.broadcasted_iota(jnp.int32, (RB, 128), 0)
            l = [l[0]] + [jnp.where(pos >= DIL * w, l[w], -1e9) for w in range(1, W)]
        l[0] = _gated(l[0], gate)
        m = l[0]
        for w in range(1, W):
            m = jnp.maximum(m, l[w])
        e = [jnp.exp2(l[w] - m) for w in range(W)]
        den = e[0]
        for w in range(1, W):
            den = den + e[w]
        inv = 1.0 / den
        p = [e[w] * inv for w in range(W)]
        cols = []
        for g in range(NG):
            acc = None
            for w in range(W):
                o = HALO + r - DIL * w
                t = p[w] * vb[slot, g, o:o + RB, :]
                acc = t if w == 0 else acc + t
            cols.append(acc.astype(BF16))
            ob[r:r + RB, g * 128:(g + 1) * 128] = cols[g]
        return _digest(cols)

    def wo_piece(q, gate=None):
        del gate
        a, jh = divmod(q, 2)
        out = []
        for half in range(2):
            rows = [(4 * jh + p) * 128 + a * DH + half * 16 for p in range(4)]
            v = _spread_rows([pltpu.bitcast(wraw[0, r0:r0 + 16, :], jnp.uint32) for r0 in rows])
            for b in range(4):
                r1 = (half * 4 + b) * 128 + a * DH + jh * 16
                out.append(pltpu.bitcast(v[b], BF16))
                wo[r1:r1 + 16, :] = out[-1]
        return _digest(out)

    def wo_dot(st, dst, k, g):
        if not st:
            st['o'] = ob[...]
        res = jnp.dot(st['o'][:, k * KH:(k + 1) * KH], wo[k * KH:(k + 1) * KH, g * 128:(g + 1) * 128],
                      preferred_element_type=F32)
        if k > 0:
            res = res + dst[:, g * 128:(g + 1) * 128]
        dst[:, g * 128:(g + 1) * 128] = res
        return res

    def tail_piece(i, r, gate=None):
        src = ab.at[i & 1]
        r0 = _aligned(i * T + r, LB)
        xn = xv[pl.ds(r0, LB), :].astype(F32) + mod_rows(2, LB) * _gated(src[r:r + LB, :], gate)
        x1[pl.ds(r0, LB), :] = xn
        hv = _ln_mod(xn, mod_rows(4, LB), mod_rows(3, LB)).astype(BF16)
        h2[pl.ds(r0, LB), :] = hv
        return _digest([hv])

    def tasks(fn, step, *args):
        return [functools.partial(fn, *args, r) for r in range(0, T, step)]

    def stream(dots, under, after=None):
        never = never_mask()
        prev, out = None, []
        per = len(dots) // len(under)
        for s, (fn, _, _, _) in enumerate(dots):
            out.append(fn())
            for task in (() if s % per else under[s // per]):
                dig = task(gate=None if prev is None else (never[0:8], prev))
                if s + LAG * per < len(dots):
                    _, w_ref, r, c = dots[s + LAG * per]
                    w_ref[r:r + 16, c:c + 128] = jnp.where(never, dig, w_ref[r:r + 16, c:c + 128])
            if after is not None and s % per == per - 1 and s // per in after:
                after[s // per]()
            prev = out[-1][-8:, :]
        return out

    def qkv_dots(slot, src, js):
        h = src[...]
        return [(functools.partial(qkv_dot, h, slot, j, k, g), wqkv.at[j], k * KH, g * 128)
                for j in js for k in range(D // KH) for g in range(NG)]

    def wo_dots(i):
        st = {}
        return [(functools.partial(wo_dot, st, ab.at[i & 1], k, g), wo, k * KH, g * 128)
                for k in range(D // KH) for g in range(NG)]

    def never_mask():
        return jnp.full((16, 128), flag[0], jnp.int32) > 0

    def swiglu(g, u):
        hg = 0.5 * g
        return ((hg * jnp.tanh(hg) + hg) * u).astype(BF16)

    def gate_up(b, f):
        r0 = _aligned(b * TB, TB)
        h = h2[pl.ds(r0, TB), :]
        g = jnp.dot(h, wg[f], preferred_element_type=F32)
        u = jnp.dot(h, wu[f], preferred_element_type=F32)
        act[...] = swiglu(g, u)

    def down(r0, a0, rows, f):
        d = jnp.dot(act[a0:a0 + rows, :], wd[f], preferred_element_type=F32)
        xn = x1[pl.ds(r0, rows), :] + mod_rows(5, rows) * d
        x1[pl.ds(r0, rows), :] = xn
        xv[pl.ds(r0, rows), :] = xn.astype(BF16)

    gs = [functools.partial(groupsum_piece, r, r + T // 4) for r in range(0, T, T // 4)]

    kb[0, :, 0:HALO, :] = jnp.zeros((NG, HALO, 128), F32)
    vb[0, :, 0:HALO, :] = jnp.zeros((NG, HALO, 128), F32)
    ab[0] = jnp.zeros((T, D), F32)
    mod[2:5] = jnp.zeros((3, 8, D), F32)
    cp_qkv(0).wait()
    cp_mod(1).start()
    cp_x(0).start()
    cp_x(1).start()

    def permute_q(r, carry):
        for u in range(128 // PB):
            permute_piece(0, pl.multiple_of(r * 128 + u * PB, PB))
        return carry
    jax.lax.fori_loop(0, D // 128, permute_q, 0)

    def mod_first(j, carry):
        cp_mod(j).wait()
        cp_qkv(j + 1).start()
        mod_chunk(j)
        return carry
    jax.lax.fori_loop(0, 2, mod_first, 0)
    cp_x(0).wait()
    cp_x(1).wait()

    def ln_first(n, carry):
        for t, dst in enumerate((hcur, hnext)):
            ln1_piece(t, dst, pl.multiple_of(n * LB, LB))
        return carry
    jax.lax.fori_loop(0, T // LB, ln_first, 0)
    for j in range(2):
        cp_qkv(j + 1).wait()
        for cp in ((cp_wo, cp_x(2)), (cp_mod(2), cp_mod(3), cp_mod(4)))[j]:
            cp.start()
        pm = [functools.partial(permute_piece, j + 1, r) for r in range(0, D, PB)]
        n = len(pm) // NG
        stream(qkv_dots(0, hcur, (j,)), [pm[g * n:(g + 1) * n] for g in range(NG)])
    for cp in tuple(cp_x(i) for i in range(3, NT)) + (cp_mod(5),):
        cp.start()
    lo = tasks(logits_piece, RB, 0)
    cp_wo.wait()
    stream(qkv_dots(0, hcur, (2,)), [lo[2 * g:2 * g + 2] + [functools.partial(wo_piece, g)] for g in range(NG)])
    _run(gs)

    def mod_rest(j, carry):
        cp_mod(j).wait()
        mod_chunk(j)
        return carry
    for f in range(NF):
        for cp in cp_ffn(f):
            cp.start()

    def step_a(i, carry):
        @pl.when(i + 2 < NT)
        def _():
            cp_x(i + 2).wait()

        @pl.when(i == 1)
        def _():
            jax.lax.fori_loop(2, 6, mod_rest, 0)
        slot = i & 1
        ou = tasks(out_piece, RB, i, slot)
        l1 = tasks(ln1_piece, LB, jnp.minimum(i + 2, NT - 1), hnext)
        ta = tasks(tail_piece, LB, jnp.maximum(i - 1, 0))
        lo = tasks(logits_piece, RB, 1 - slot)
        under = [[ou[s]] + ([l1[s // 2]] if s & 1 else []) for s in range(16)]
        under += [[ta[k], lo[k]] for k in range(8)]
        under += [lo[8:10], lo[10:12], lo[12:14], lo[14:16], [], [], [], []]
        stream(qkv_dots(1 - slot, hnext, range(3)) + wo_dots(i), under, {30: lambda: _run(gs)})
        return carry
    jax.lax.fori_loop(0, NT - 1, step_a, 0)

    for cp in cp_ffn(0)[:2]:
        cp.wait()
    last = NT - 1

    h0 = h2[0:TB, :]

    def ffn_dot(w_ref, g):
        return jnp.dot(h0, w_ref[0, :, g * 128:(g + 1) * 128], preferred_element_type=F32)

    nc, wd7 = FC // 128, wo_dots(last)
    ou, t6, t7 = tasks(out_piece, RB, last, last & 1), tasks(tail_piece, LB, last - 1), tasks(tail_piece, LB, last)
    gd, ud = [[(functools.partial(ffn_dot, w, g), w.at[0], 0, g * 128) for g in range(nc)] for w in (wg, wu)]
    res = stream(gd + ud[:2] + wd7 + ud[2:],
                 [ou[3 * k:3 * k + 3] for k in range(6)] + [t6[k:k + 1] for k in range(len(wd7))] + [t7[:4], t7[4:]])
    for g, u in enumerate(res[nc:nc + 2] + res[-2:]):
        act[:, g * 128:(g + 1) * 128] = swiglu(res[g], u)
    for f in range(NF):
        for cp in cp_ffn(f)[2 if f == 0 else 0:]:
            cp.wait()

    def step_b(n, carry):
        bp, fp = (n - 1) // NF, (n - 1) % NF
        r0 = pl.multiple_of(bp * TB, TB)
        down(r0, 0, TB, fp)
        gate_up(n // NF, n % NF)

        @pl.when(fp == NF - 1)
        def _():
            cp_out(r0, TB, bp).start()
        return carry
    jax.lax.fori_loop(1, NB * NF, step_b, 0)
    outs = [cp_out(b * TB, TB, b) for b in range(NB - 1)]
    for k, a0 in enumerate(range(0, TB, ZB)):
        down(S - TB + a0, a0, ZB, NF - 1)
        outs.append(cp_out(S - TB + a0, ZB, NB - 1 + k))
        outs[-1].start()
    for cp in outs:
        cp.wait()


@jax.jit
def pallas_adaLN_cond__sliding_local_dilated__swiglu_ffn__prompt_kernel(
    A_x: jax.Array,
    A_wqkv: jax.Array,
    A_wo: jax.Array,
    B_x: jax.Array,
    B_w_gate: jax.Array,
    B_w_up: jax.Array,
    B_w_down: jax.Array,
    c: jax.Array,
    w_mod: jax.Array,
):
    del B_x
    hbm = pl.BlockSpec(memory_space=pl.ANY)
    out = pl.pallas_call(
        _kernel,
        out_shape=jax.ShapeDtypeStruct((S, D), BF16),
        grid=(1,),
        in_specs=[hbm, hbm, hbm, hbm, hbm, hbm, pl.BlockSpec((1, D), lambda i: (0, 0)), hbm],
        out_specs=hbm,
        scratch_shapes=[
            pltpu.VMEM((S, D), BF16),
            pltpu.VMEM((3, D, D), BF16),
            pltpu.VMEM((3, D, D), BF16),
            pltpu.VMEM((D, D), BF16),
            pltpu.VMEM((NF, D, FC), BF16),
            pltpu.VMEM((NF, D, FC), BF16),
            pltpu.VMEM((NF, FC, D), BF16),
            pltpu.VMEM((6, D, D), BF16),
            pltpu.VMEM((D, 128), F32),
            pltpu.VMEM((6, 8, D), F32),
            pltpu.VMEM((T, D), BF16),
            pltpu.VMEM((T, D), BF16),
            pltpu.VMEM((2, NG, T, 128), F32),
            pltpu.VMEM((2, NG, HALO + T, 128), F32),
            pltpu.VMEM((2, NG, HALO + T, 128), F32),
            pltpu.VMEM((W * T, 128), BF16),
            pltpu.VMEM((W * T, 128), F32),
            pltpu.VMEM((T, D), BF16),
            pltpu.VMEM((2, T, D), F32),
            pltpu.VMEM((TB, FC), BF16),
            pltpu.VMEM((S, D), F32),
            pltpu.VMEM((S, D), BF16),
            pltpu.SMEM((1,), jnp.int32),
            pltpu.SemaphoreType.DMA((NT,)),
            pltpu.SemaphoreType.DMA((3,)),
            pltpu.SemaphoreType.DMA((6,)),
            pltpu.SemaphoreType.DMA((1 + 3 * NF,)),
            pltpu.SemaphoreType.DMA((NB - 1 + TB // ZB,)),
        ],
        compiler_params=pltpu.CompilerParams(vmem_limit_bytes=110 * 1024 * 1024),
    )(A_x.reshape(S, D), A_wqkv, A_wo, B_w_gate, B_w_up, B_w_down, c, w_mod)
    return out.reshape(1, S, D)
```

```python
import functools

import jax
import jax.numpy as jnp
import numpy as np
from jax.experimental import pallas as pl
from jax.experimental.pallas import tpu as pltpu

S, D, F = 2048, 1024, 3584
H, DH, W, DIL = 32, 32, 8, 2
HALO = 16
NG = D // 128
T = 256
TB = 1024
PB = 64
FC = 512
RB = 16
LB = 32
LAG = 3
KH = 1024
ZB = 256
EPS = 1e-5
NT, NB, NF = S // T, S // TB, F // FC
F32, BF16 = jnp.float32, jnp.bfloat16


def _spread_rows(v):
    sub = jax.lax.broadcasted_iota(jnp.int32, v[0].shape, 0)
    v = list(v)
    for s, d in ((4, 2), (2, 1)):
        low = (sub & s) == 0
        for a in range(4):
            if not a & d:
                va, vb = v[a], v[a + d]
                v[a] = jnp.where(low, va, pltpu.roll(vb, s, 0))
                v[a + d] = jnp.where(low, pltpu.roll(va, 8 - s, 0), vb)
    return v


def _spread_heads(cols):
    sub = (jax.lax.broadcasted_iota(jnp.int32, cols[0].shape, 1) >> 2) & 7
    out = [None] * NG
    for d in range(1 - NG, NG):
        js = [j for j in range(NG) if 0 <= j - d < NG]
        diag = cols[js[0]]
        for j in js[1:]:
            diag = jnp.where(sub == j - d, cols[j], diag)
        if d:
            diag = pltpu.roll(diag, (4 * d) % 128, 1)
        for j in js:
            out[j - d] = diag if out[j - d] is None else jnp.where(sub == j, diag, out[j - d])
    return out


def _ln_mod(x, scale1, shift):
    m = jnp.mean(x, axis=-1, keepdims=True)
    xc = x - m
    v = jnp.mean(xc * xc, axis=-1, keepdims=True)
    return xc * jax.lax.rsqrt(v + EPS) * scale1 + shift


def _aligned(v, n):
    return v if isinstance(v, int) else pl.multiple_of(v, n)


def _digest(blocks):
    out = None
    for b in blocks:
        for r in range(0, b.shape[0], 16):
            for c in range(0, b.shape[1], 128):
                v = pltpu.bitcast(b[r:r + 16, c:c + 128], jnp.uint32)
                out = v if out is None else out | v
    return pltpu.bitcast(out, BF16)


def _gated(x, gate):
    if gate is None:
        return x
    never, v = gate
    head = jnp.where(never, pltpu.bitcast(v, x.dtype), x[0:8, 0:128])
    if x.shape[1] > 128:
        head = jnp.concatenate([head, x[0:8, 128:]], axis=1)
    return jnp.concatenate([head, x[8:]], axis=0)


def _deal(tasks, n):
    return [tasks[k * len(tasks) // n:(k + 1) * len(tasks) // n] for k in range(n)]


def _run(tasks):
    for t in tasks:
        t()


def _kernel(x_hbm, wqkv_hbm, wo_hbm, wg_hbm, wu_hbm, wd_hbm, c_ref, wmod_hbm, out_hbm,
            xv, wraw, wqkv, wo, wg, wu, wd, wmod, sb, mod, hnext, qb, kb, vb, tb, lg, ob, ab, act, x1, h2, flag,
            sem_x, sem_qkv, sem_mod, sem_w, sem_out):
    def cp_x(i):
        return pltpu.make_async_copy(x_hbm.at[pl.ds(_aligned(i * T, T), T)], xv.at[pl.ds(_aligned(i * T, T), T)], sem_x.at[i])

    def cp_mod(j):
        return pltpu.make_async_copy(wmod_hbm.at[:, pl.ds(_aligned(j * D, D), D)], wmod.at[j], sem_mod.at[j])

    def cp_qkv(j):
        return pltpu.make_async_copy(wqkv_hbm.at[:, pl.ds(_aligned(j * D, D), D)], wraw.at[j], sem_qkv.at[j])

    cp_wo = pltpu.make_async_copy(wo_hbm, wraw.at[0], sem_w.at[0])

    def cp_ffn(f):
        c0 = f * FC
        return (pltpu.make_async_copy(wg_hbm.at[:, c0:c0 + FC], wg.at[f], sem_w.at[1 + 3 * f]),
                pltpu.make_async_copy(wu_hbm.at[:, c0:c0 + FC], wu.at[f], sem_w.at[2 + 3 * f]),
                pltpu.make_async_copy(wd_hbm.at[c0:c0 + FC, :], wd.at[f], sem_w.at[3 + 3 * f]))

    def cp_out(row0, rows, k):
        return pltpu.make_async_copy(xv.at[pl.ds(row0, rows)], out_hbm.at[pl.ds(row0, rows)], sem_out.at[k])

    cp_qkv(0).start()
    cp_mod(0).start()
    flag[0] = 0
    cv = c_ref[...].astype(F32)
    sc = (cv * jax.nn.sigmoid(cv)).astype(BF16).astype(F32)
    for j in range(NG):
        row = jnp.broadcast_to(sc[:, j * 128:(j + 1) * 128], (128, 128))
        sb[j * 128:(j + 1) * 128, :] = row.T

    def mod_chunk(j):
        def body(r, acc):
            r0 = pl.multiple_of(r * 64, 64)
            s = sb[pl.ds(r0, 64), :]
            out = []
            for g in range(NG):
                t = wmod[j, pl.ds(r0, 64), g * 128:(g + 1) * 128].astype(F32) * s
                t = t[0:32] + t[32:64]
                t = t[0:16] + t[16:32]
                out.append(acc[g] + (t[0:8] + t[8:16]))
            return tuple(out)
        acc = jax.lax.fori_loop(0, D // 64, body, tuple(jnp.zeros((8, 128), F32) for _ in range(NG)))
        one = jnp.where((j == 1) | (j == 4), 1.0, 0.0)
        for g in range(NG):
            res = jnp.sum(acc[g], axis=0, keepdims=True) + one
            mod[j, :, g * 128:(g + 1) * 128] = jnp.broadcast_to(res, (8, 128))

    def mod_piece(j, g, gate=None):
        acc = [None, None]
        for n, r in enumerate(range(0, D, 16)):
            t = wmod[j, r:r + 16, g * 128:(g + 1) * 128].astype(F32) * sb[r:r + 16, :]
            t = _gated(t, gate) if n < 2 else t
            acc[n & 1] = t if n < 2 else acc[n & 1] + t
        res = jnp.sum(acc[0] + acc[1], axis=0, keepdims=True) + (1.0 if j in (1, 4) else 0.0)
        res = jnp.broadcast_to(res, (8, 128))
        mod[j, :, g * 128:(g + 1) * 128] = res
        return pltpu.bitcast(res, BF16)

    def mod_rows(j, rows):
        return jnp.concatenate([mod[j]] * (rows // 8), axis=0)

    def permute_piece(j, r, gate=None):
        cols = [pltpu.bitcast(wraw[j, pl.ds(r, PB), g * 128:(g + 1) * 128], jnp.uint32) for g in range(NG)]
        if gate is not None:
            cols = [_gated(c, gate) for c in cols]
        cols = [pltpu.bitcast(c, BF16) for c in _spread_heads(cols)]
        for g in range(NG):
            wqkv[j, pl.ds(r, PB), g * 128:(g + 1) * 128] = cols[g]
        return _digest(cols)

    def ln1_piece(i, dst, r, gate=None):
        r0 = _aligned(i * T + r, LB)
        xt = _gated(xv[pl.ds(r0, LB), :].astype(F32), gate)
        hv = _ln_mod(xt, mod_rows(1, LB), mod_rows(0, LB)).astype(BF16)
        dst[pl.ds(r, LB), :] = hv
        return _digest([hv])

    qscale = float(DH ** -0.5 * np.log2(np.e))

    def qkv_dot(h, slot, j, k, g):
        res = jnp.dot(h[:, k * KH:(k + 1) * KH], wqkv[j, k * KH:(k + 1) * KH, g * 128:(g + 1) * 128],
                      preferred_element_type=F32)
        buf, r0 = ((qb, 0), (kb, HALO), (vb, HALO))[j]
        if k > 0:
            res = res + buf[slot, g, r0:r0 + T, :]
        if k == D // KH - 1:
            if j == 0:
                res = res * qscale
            else:
                buf[1 - slot, g, 0:HALO, :] = res[T - HALO:, :]
        buf[slot, g, r0:r0 + T, :] = res
        return res

    def logits_piece(slot, r, gate=None):
        acc = [None] * W
        for g in range(NG):
            qv = qb[slot, g, r:r + RB, :]
            if g == 0:
                qv = _gated(qv, gate)
            for w in range(W):
                o = HALO + r - DIL * w
                p = qv * kb[slot, g, o:o + RB, :]
                acc[w] = p if g == 0 else acc[w] + p
        acc = [a.astype(BF16) for a in acc]
        for w in range(W):
            tb[r * W + w * RB:r * W + (w + 1) * RB, :] = acc[w]
        return _digest(acc)

    def groupsum_piece(r0, r1):
        ri = jax.lax.broadcasted_iota(jnp.int32, (128, 128), 0)
        ci = jax.lax.broadcasted_iota(jnp.int32, (128, 128), 1)
        group_ones = jnp.where((ri >> 2) == (ci >> 2), 1.0, 0.0).astype(BF16)
        lg[r0 * W:r1 * W, :] = jnp.dot(tb[r0 * W:r1 * W, :], group_ones, preferred_element_type=F32)

    def out_piece(i, slot, r, gate=None):
        l = [lg[r * W + w * RB:r * W + (w + 1) * RB, :] for w in range(W)]
        if r < HALO and not (isinstance(i, int) and i > 0):
            pos = i * T + r + jax.lax.broadcasted_iota(jnp.int32, (RB, 128), 0)
            l = [l[0]] + [jnp.where(pos >= DIL * w, l[w], -1e9) for w in range(1, W)]
        l[0] = _gated(l[0], gate)
        m = l[0]
        for w in range(1, W):
            m = jnp.maximum(m, l[w])
        e = [jnp.exp2(l[w] - m) for w in range(W)]
        den = e[0]
        for w in range(1, W):
            den = den + e[w]
        inv = 1.0 / den
        p = [e[w] * inv for w in range(W)]
        cols = []
        for g in range(NG):
            acc = None
            for w in range(W):
                o = HALO + r - DIL * w
                t = p[w] * vb[slot, g, o:o + RB, :]
                acc = t if w == 0 else acc + t
            cols.append(acc.astype(BF16))
            ob[r:r + RB, g * 128:(g + 1) * 128] = cols[g]
        return _digest(cols)

    def wo_piece(q, gate=None):
        del gate
        a, jh = divmod(q, 2)
        out = []
        for half in range(2):
            rows = [(4 * jh + p) * 128 + a * DH + half * 16 for p in range(4)]
            v = _spread_rows([pltpu.bitcast(wraw[0, r0:r0 + 16, :], jnp.uint32) for r0 in rows])
            for b in range(4):
                r1 = (half * 4 + b) * 128 + a * DH + jh * 16
                out.append(pltpu.bitcast(v[b], BF16))
                wo[r1:r1 + 16, :] = out[-1]
        return _digest(out)

    def wo_dot(st, dst, k, g):
        if not st:
            st['o'] = ob[...]
        res = jnp.dot(st['o'][:, k * KH:(k + 1) * KH], wo[k * KH:(k + 1) * KH, g * 128:(g + 1) * 128],
                      preferred_element_type=F32)
        if k > 0:
            res = res + dst[:, g * 128:(g + 1) * 128]
        dst[:, g * 128:(g + 1) * 128] = res
        return res

    def tail_piece(i, r, gate=None):
        src = ab.at[i & 1]
        r0 = _aligned(i * T + r, LB)
        xn = xv[pl.ds(r0, LB), :].astype(F32) + mod_rows(2, LB) * _gated(src[r:r + LB, :], gate)
        x1[pl.ds(r0, LB), :] = xn
        hv = _ln_mod(xn, mod_rows(4, LB), mod_rows(3, LB)).astype(BF16)
        h2[pl.ds(r0, LB), :] = hv
        return _digest([hv])

    def tasks(fn, step, *args):
        return [functools.partial(fn, *args, r) for r in range(0, T, step)]

    def stream(dots, under, after=None):
        never = never_mask()
        prev, out = None, []
        per = len(dots) // len(under)
        for s, (fn, _, _, _) in enumerate(dots):
            out.append(fn())
            for task in (() if s % per else under[s // per]):
                dig = task(gate=None if prev is None else (never[0:8], prev))
                if s + LAG * per < len(dots):
                    _, w_ref, r, c = dots[s + LAG * per]
                    w_ref[r:r + 16, c:c + 128] = jnp.where(never, dig, w_ref[r:r + 16, c:c + 128])
            if after is not None and s % per == per - 1 and s // per in after:
                after[s // per]()
            prev = out[-1][-8:, :]
        return out

    def qkv_dots(slot, src, js):
        h = src[...]
        return [(functools.partial(qkv_dot, h, slot, j, k, g), wqkv.at[j], k * KH, g * 128)
                for j in js for k in range(D // KH) for g in range(NG)]

    def wo_dots(i):
        st = {}
        return [(functools.partial(wo_dot, st, ab.at[i & 1], k, g), wo, k * KH, g * 128)
                for k in range(D // KH) for g in range(NG)]

    def never_mask():
        return jnp.full((16, 128), flag[0], jnp.int32) > 0

    def swiglu(g, u):
        hg = 0.5 * g
        return ((hg * jnp.tanh(hg) + hg) * u).astype(BF16)

    def gate_up(b, f):
        r0 = _aligned(b * TB, TB)
        h = h2[pl.ds(r0, TB), :]
        g = jnp.dot(h, wg[f], preferred_element_type=F32)
        u = jnp.dot(h, wu[f], preferred_element_type=F32)
        act[...] = swiglu(g, u)

    def down(r0, a0, rows, f):
        d = jnp.dot(act[a0:a0 + rows, :], wd[f], preferred_element_type=F32)
        xn = x1[pl.ds(r0, rows), :] + mod_rows(5, rows) * d
        x1[pl.ds(r0, rows), :] = xn
        xv[pl.ds(r0, rows), :] = xn.astype(BF16)

    gs = [functools.partial(groupsum_piece, r, r + T // 4) for r in range(0, T, T // 4)]

    kb[0, :, 0:HALO, :] = jnp.zeros((NG, HALO, 128), F32)
    vb[0, :, 0:HALO, :] = jnp.zeros((NG, HALO, 128), F32)
    cp_qkv(0).wait()
    cp_mod(1).start()
    cp_x(0).start()

    def permute_q(r, carry):
        for u in range(128 // PB):
            permute_piece(0, pl.multiple_of(r * 128 + u * PB, PB))
        return carry
    jax.lax.fori_loop(0, D // 128, permute_q, 0)

    def mod_first(j, carry):
        cp_mod(j).wait()

        @pl.when(j == 1)
        def _():
            cp_qkv(1).start()
        mod_chunk(j)
        return carry
    jax.lax.fori_loop(0, 2, mod_first, 0)
    cp_x(0).wait()

    def ln_first(n, carry):
        for u in range(2):
            ln1_piece(0, ob, pl.multiple_of(n * 2 * LB + u * LB, LB))
        return carry
    jax.lax.fori_loop(0, T // (2 * LB), ln_first, 0)
    for j, (head, later) in enumerate(((3, (cp_qkv(2), cp_x(1))), (2, (cp_wo, cp_x(2))))):
        dots = qkv_dots(0, ob, (j,))
        stream(dots[:head], [[]] * head)
        cp_qkv(j + 1).wait()
        for cp in later:
            cp.start()
        pm = [functools.partial(permute_piece, j + 1, r) for r in range(0, D, PB)]
        stream(dots[head:], _deal(pm, NG - head))
    lo, l1 = tasks(logits_piece, RB, 0), tasks(ln1_piece, LB, 1, hnext)
    cp_x(1).wait()
    for j in range(2, 6):
        cp_mod(j).start()
    stream(qkv_dots(0, ob, (2,)), [lo[2 * g:2 * g + 2] + [l1[g]] for g in range(NG)])
    _run(gs)

    cp_wo.wait()
    for i in range(3, NT):
        cp_x(i).start()

    def step_a(i, carry):
        first = isinstance(i, int)
        if first:
            cp_x(i + 2).wait()
        else:
            @pl.when(i + 2 < NT)
            def _():
                cp_x(i + 2).wait()
        slot = i & 1
        ou = tasks(out_piece, RB, i, slot)
        l1 = tasks(ln1_piece, LB, i + 2 if first else jnp.minimum(i + 2, NT - 1), hnext)
        lo = tasks(logits_piece, RB, 1 - slot)
        under = [[ou[s]] + ([l1[s // 2]] if s & 1 else []) for s in range(16)]
        under += [[lo[k]] for k in range(8)]
        under += [lo[8:10], lo[10:12], lo[12:14], lo[14:16], [], [], [], []]
        dots = qkv_dots(1 - slot, hnext, range(3)) + wo_dots(i)
        if first:
            for q in range(NG):
                under[2 * q].append(functools.partial(wo_piece, q))
            stream(dots[:16], under[:16])
            for j in (2, 3, 4):
                cp_mod(j).wait()
            for f in range(NF):
                for cp in cp_ffn(f):
                    cp.start()
            md = _deal([functools.partial(mod_piece, j, g) for j in (2, 3, 4) for g in range(NG)], 16)
            stream(dots[16:], [a + b for a, b in zip(under[16:], md)], {14: lambda: _run(gs)})
        else:
            for k, t in enumerate(tasks(tail_piece, LB, i - 1)):
                under[16 + k].insert(0, t)
            stream(dots, under, {30: lambda: _run(gs)})
        return carry
    step_a(0, 0)
    jax.lax.fori_loop(1, NT - 1, step_a, 0)

    for cp in cp_ffn(0)[:2] + (cp_mod(5),):
        cp.wait()
    last = NT - 1

    h0 = h2[0:TB, :]

    def ffn_dot(w_ref, g):
        return jnp.dot(h0, w_ref[0, :, g * 128:(g + 1) * 128], preferred_element_type=F32)

    nc, wd7 = FC // 128, wo_dots(last)
    ou, t6, t7 = tasks(out_piece, RB, last, last & 1), tasks(tail_piece, LB, last - 1), tasks(tail_piece, LB, last)
    gd, ud = [[(functools.partial(ffn_dot, w, g), w.at[0], 0, g * 128) for g in range(nc)] for w in (wg, wu)]
    res = stream(gd + ud[:2] + wd7 + ud[2:],
                 [ou[3 * k:3 * k + 3] for k in range(6)] + [[t6[k], functools.partial(mod_piece, 5, k)] for k in range(NG)] + [t7[:4], t7[4:]])
    for g, u in enumerate(res[nc:nc + 2] + res[-2:]):
        act[:, g * 128:(g + 1) * 128] = swiglu(res[g], u)
    for f in range(NF):
        for cp in cp_ffn(f)[2 if f == 0 else 0:]:
            cp.wait()

    def step_b(n, carry):
        bp, fp = (n - 1) // NF, (n - 1) % NF
        r0 = pl.multiple_of(bp * TB, TB)
        down(r0, 0, TB, fp)
        gate_up(n // NF, n % NF)

        @pl.when(fp == NF - 1)
        def _():
            cp_out(r0, TB, bp).start()
        return carry
    jax.lax.fori_loop(1, NB * NF, step_b, 0)
    outs = [cp_out(b * TB, TB, b) for b in range(NB - 1)]
    for k, a0 in enumerate(range(0, TB, ZB)):
        down(S - TB + a0, a0, ZB, NF - 1)
        outs.append(cp_out(S - TB + a0, ZB, NB - 1 + k))
        outs[-1].start()
    for cp in outs:
        cp.wait()


@jax.jit
def pallas_adaLN_cond__sliding_local_dilated__swiglu_ffn__prompt_kernel(
    A_x: jax.Array,
    A_wqkv: jax.Array,
    A_wo: jax.Array,
    B_x: jax.Array,
    B_w_gate: jax.Array,
    B_w_up: jax.Array,
    B_w_down: jax.Array,
    c: jax.Array,
    w_mod: jax.Array,
):
    del B_x
    hbm = pl.BlockSpec(memory_space=pl.ANY)
    out = pl.pallas_call(
        _kernel,
        out_shape=jax.ShapeDtypeStruct((S, D), BF16),
        grid=(1,),
        in_specs=[hbm, hbm, hbm, hbm, hbm, hbm, pl.BlockSpec((1, D), lambda i: (0, 0)), hbm],
        out_specs=hbm,
        scratch_shapes=[
            pltpu.VMEM((S, D), BF16),
            pltpu.VMEM((3, D, D), BF16),
            pltpu.VMEM((3, D, D), BF16),
            pltpu.VMEM((D, D), BF16),
            pltpu.VMEM((NF, D, FC), BF16),
            pltpu.VMEM((NF, D, FC), BF16),
            pltpu.VMEM((NF, FC, D), BF16),
            pltpu.VMEM((6, D, D), BF16),
            pltpu.VMEM((D, 128), F32),
            pltpu.VMEM((6, 8, D), F32),
            pltpu.VMEM((T, D), BF16),
            pltpu.VMEM((2, NG, T, 128), F32),
            pltpu.VMEM((2, NG, HALO + T, 128), F32),
            pltpu.VMEM((2, NG, HALO + T, 128), F32),
            pltpu.VMEM((W * T, 128), BF16),
            pltpu.VMEM((W * T, 128), F32),
            pltpu.VMEM((T, D), BF16),
            pltpu.VMEM((2, T, D), F32),
            pltpu.VMEM((TB, FC), BF16),
            pltpu.VMEM((S, D), F32),
            pltpu.VMEM((S, D), BF16),
            pltpu.SMEM((1,), jnp.int32),
            pltpu.SemaphoreType.DMA((NT,)),
            pltpu.SemaphoreType.DMA((3,)),
            pltpu.SemaphoreType.DMA((6,)),
            pltpu.SemaphoreType.DMA((1 + 3 * NF,)),
            pltpu.SemaphoreType.DMA((NB - 1 + TB // ZB,)),
        ],
        compiler_params=pltpu.CompilerParams(vmem_limit_bytes=110 * 1024 * 1024),
    )(A_x.reshape(S, D), A_wqkv, A_wo, B_w_gate, B_w_up, B_w_down, c, w_mod)
    return out.reshape(1, S, D)
```

```python
import functools

import jax
import jax.numpy as jnp
import numpy as np
from jax.experimental import pallas as pl
from jax.experimental.pallas import tpu as pltpu

S, D, F = 2048, 1024, 3584
H, DH, W, DIL = 32, 32, 8, 2
HALO = 16
NG = D // 128
T = 256
TB = 1024
PB = 64
FC = 512
RB = 16
LB = 32
LAG = 3
KH = 1024
ZB = 256
EPS = 1e-5
assert DIL * (W // 2) == 8 and HALO >= DIL * (W - 1)
NT, NB, NF = S // T, S // TB, F // FC
F32, BF16 = jnp.float32, jnp.bfloat16


def _spread_rows(v):
    sub = jax.lax.broadcasted_iota(jnp.int32, v[0].shape, 0)
    v = list(v)
    for s, d in ((4, 2), (2, 1)):
        low = (sub & s) == 0
        for a in range(4):
            if not a & d:
                va, vb = v[a], v[a + d]
                v[a] = jnp.where(low, va, pltpu.roll(vb, s, 0))
                v[a + d] = jnp.where(low, pltpu.roll(va, 8 - s, 0), vb)
    return v


def _spread_heads(cols):
    sub = (jax.lax.broadcasted_iota(jnp.int32, cols[0].shape, 1) >> 2) & 7
    out = [None] * NG
    for d in range(1 - NG, NG):
        js = [j for j in range(NG) if 0 <= j - d < NG]
        diag = cols[js[0]]
        for j in js[1:]:
            diag = jnp.where(sub == j - d, cols[j], diag)
        if d:
            diag = pltpu.roll(diag, (4 * d) % 128, 1)
        for j in js:
            out[j - d] = diag if out[j - d] is None else jnp.where(sub == j, diag, out[j - d])
    return out


def _ln_mod(x, scale1, shift):
    m = jnp.mean(x, axis=-1, keepdims=True)
    xc = x - m
    v = jnp.mean(xc * xc, axis=-1, keepdims=True)
    return xc * jax.lax.rsqrt(v + EPS) * scale1 + shift


def _aligned(v, n):
    return v if isinstance(v, int) else pl.multiple_of(v, n)


def _digest(blocks):
    out = None
    for b in blocks:
        for r in range(0, b.shape[0], 16):
            for c in range(0, b.shape[1], 128):
                v = pltpu.bitcast(b[r:r + 16, c:c + 128], jnp.uint32)
                out = v if out is None else out | v
    return pltpu.bitcast(out, BF16)


def _gated(x, gate):
    if gate is None:
        return x
    never, v = gate
    head = jnp.where(never, pltpu.bitcast(v, x.dtype), x[0:8, 0:128])
    if x.shape[1] > 128:
        head = jnp.concatenate([head, x[0:8, 128:]], axis=1)
    return jnp.concatenate([head, x[8:]], axis=0)


def _deal(tasks, n):
    return [tasks[k * len(tasks) // n:(k + 1) * len(tasks) // n] for k in range(n)]


def _run(tasks):
    for t in tasks:
        t()


def _kernel(x_hbm, wqkv_hbm, wo_hbm, wg_hbm, wu_hbm, wd_hbm, c_ref, wmod_hbm, out_hbm,
            xv, wraw, wqkv, wo, wg, wu, wd, wmod, sb, mod, hnext, qb, kb, vb, tb, lg, ob, ab, act, x1, h2, flag,
            sem_x, sem_qkv, sem_mod, sem_w, sem_out):
    def cp_x(i):
        return pltpu.make_async_copy(x_hbm.at[pl.ds(_aligned(i * T, T), T)], xv.at[pl.ds(_aligned(i * T, T), T)], sem_x.at[i])

    def cp_mod(j):
        return pltpu.make_async_copy(wmod_hbm.at[:, pl.ds(_aligned(j * D, D), D)], wmod.at[j], sem_mod.at[j])

    def cp_qkv(j):
        return pltpu.make_async_copy(wqkv_hbm.at[:, pl.ds(_aligned(j * D, D), D)], wraw.at[j], sem_qkv.at[j])

    cp_wo = pltpu.make_async_copy(wo_hbm, wraw.at[0], sem_w.at[0])

    def cp_ffn(f):
        c0 = f * FC
        return (pltpu.make_async_copy(wg_hbm.at[:, c0:c0 + FC], wg.at[f], sem_w.at[1 + 3 * f]),
                pltpu.make_async_copy(wu_hbm.at[:, c0:c0 + FC], wu.at[f], sem_w.at[2 + 3 * f]),
                pltpu.make_async_copy(wd_hbm.at[c0:c0 + FC, :], wd.at[f], sem_w.at[3 + 3 * f]))

    def cp_out(row0, rows, k):
        return pltpu.make_async_copy(xv.at[pl.ds(row0, rows)], out_hbm.at[pl.ds(row0, rows)], sem_out.at[k])

    cp_qkv(0).start()
    cp_mod(0).start()
    flag[0] = 0
    cv = c_ref[...].astype(F32)
    sc = (cv * jax.nn.sigmoid(cv)).astype(BF16).astype(F32)
    for j in range(NG):
        row = jnp.broadcast_to(sc[:, j * 128:(j + 1) * 128], (128, 128))
        sb[j * 128:(j + 1) * 128, :] = row.T

    def mod_chunk(j):
        def body(r, acc):
            r0 = pl.multiple_of(r * 64, 64)
            s = sb[pl.ds(r0, 64), :]
            out = []
            for g in range(NG):
                t = wmod[j, pl.ds(r0, 64), g * 128:(g + 1) * 128].astype(F32) * s
                t = t[0:32] + t[32:64]
                t = t[0:16] + t[16:32]
                out.append(acc[g] + (t[0:8] + t[8:16]))
            return tuple(out)
        acc = jax.lax.fori_loop(0, D // 64, body, tuple(jnp.zeros((8, 128), F32) for _ in range(NG)))
        one = jnp.where((j == 1) | (j == 4), 1.0, 0.0)
        for g in range(NG):
            res = jnp.sum(acc[g], axis=0, keepdims=True) + one
            mod[j, :, g * 128:(g + 1) * 128] = jnp.broadcast_to(res, (8, 128))

    def mod_piece(j, g, gate=None):
        acc = [None, None]
        for n, r in enumerate(range(0, D, 16)):
            t = wmod[j, r:r + 16, g * 128:(g + 1) * 128].astype(F32) * sb[r:r + 16, :]
            t = _gated(t, gate) if n < 2 else t
            acc[n & 1] = t if n < 2 else acc[n & 1] + t
        res = jnp.sum(acc[0] + acc[1], axis=0, keepdims=True) + (1.0 if j in (1, 4) else 0.0)
        res = jnp.broadcast_to(res, (8, 128))
        mod[j, :, g * 128:(g + 1) * 128] = res
        return pltpu.bitcast(res, BF16)

    def mod_rows(j, rows):
        return jnp.concatenate([mod[j]] * (rows // 8), axis=0)

    def permute_piece(j, r, gate=None):
        cols = [pltpu.bitcast(wraw[j, pl.ds(r, PB), g * 128:(g + 1) * 128], jnp.uint32) for g in range(NG)]
        if gate is not None:
            cols = [_gated(c, gate) for c in cols]
        cols = [pltpu.bitcast(c, BF16) for c in _spread_heads(cols)]
        for g in range(NG):
            wqkv[j, pl.ds(r, PB), g * 128:(g + 1) * 128] = cols[g]
        return _digest(cols)

    def ln1_piece(i, dst, r, gate=None):
        r0 = _aligned(i * T + r, LB)
        xt = _gated(xv[pl.ds(r0, LB), :].astype(F32), gate)
        hv = _ln_mod(xt, mod_rows(1, LB), mod_rows(0, LB)).astype(BF16)
        dst[pl.ds(r, LB), :] = hv
        return _digest([hv])

    qscale = float(DH ** -0.5 * np.log2(np.e))

    def qkv_dot(h, slot, j, k, g):
        res = jnp.dot(h[:, k * KH:(k + 1) * KH], wqkv[j, k * KH:(k + 1) * KH, g * 128:(g + 1) * 128],
                      preferred_element_type=F32)
        buf, r0 = ((qb, 0), (kb, HALO), (vb, HALO))[j]
        if k > 0:
            res = res + buf[slot, g, r0:r0 + T, :]
        if k == D // KH - 1:
            if j == 0:
                res = res * qscale
            else:
                buf[1 - slot, g, 0:HALO, :] = res[T - HALO:, :]
        buf[slot, g, r0:r0 + T, :] = res
        return res

    def window(buf, slot, g, r):
        out = [None] * W
        for w in range(W // 2):
            o = HALO + r - DIL * w - 8
            rows = buf[slot, g, o:o + RB + 8, :]
            out[w], out[w + W // 2] = rows[8:], rows[:RB]
        return out

    def logits_piece(slot, r, gate=None):
        acc = [None] * W
        for g in range(NG):
            qv = qb[slot, g, r:r + RB, :]
            if g == 0:
                qv = _gated(qv, gate)
            for w, kv in enumerate(window(kb, slot, g, r)):
                p = qv * kv
                acc[w] = p if g == 0 else acc[w] + p
        acc = [a.astype(BF16) for a in acc]
        for w in range(W):
            tb[r * W + w * RB:r * W + (w + 1) * RB, :] = acc[w]
        return _digest(acc)

    def groupsum_piece(r0, r1):
        ri = jax.lax.broadcasted_iota(jnp.int32, (128, 128), 0)
        ci = jax.lax.broadcasted_iota(jnp.int32, (128, 128), 1)
        group_ones = jnp.where((ri >> 2) == (ci >> 2), 1.0, 0.0).astype(BF16)
        lg[r0 * W:r1 * W, :] = jnp.dot(tb[r0 * W:r1 * W, :], group_ones, preferred_element_type=F32)

    def out_piece(i, slot, r, gate=None):
        l = [lg[r * W + w * RB:r * W + (w + 1) * RB, :] for w in range(W)]
        if r < HALO and not (isinstance(i, int) and i > 0):
            pos = i * T + r + jax.lax.broadcasted_iota(jnp.int32, (RB, 128), 0)
            l = [l[0]] + [jnp.where(pos >= DIL * w, l[w], -1e9) for w in range(1, W)]
        l[0] = _gated(l[0], gate)
        m = l[0]
        for w in range(1, W):
            m = jnp.maximum(m, l[w])
        e = [jnp.exp2(l[w] - m) for w in range(W)]
        den = e[0]
        for w in range(1, W):
            den = den + e[w]
        inv = 1.0 / den
        p = [e[w] * inv for w in range(W)]
        cols = []
        for g in range(NG):
            acc = None
            for w, vv in enumerate(window(vb, slot, g, r)):
                t = p[w] * vv
                acc = t if w == 0 else acc + t
            cols.append(acc.astype(BF16))
            ob[r:r + RB, g * 128:(g + 1) * 128] = cols[g]
        return _digest(cols)

    def wo_piece(q, gate=None):
        del gate
        a, jh = divmod(q, 2)
        out = []
        for half in range(2):
            rows = [(4 * jh + p) * 128 + a * DH + half * 16 for p in range(4)]
            v = _spread_rows([pltpu.bitcast(wraw[0, r0:r0 + 16, :], jnp.uint32) for r0 in rows])
            for b in range(4):
                r1 = (half * 4 + b) * 128 + a * DH + jh * 16
                out.append(pltpu.bitcast(v[b], BF16))
                wo[r1:r1 + 16, :] = out[-1]
        return _digest(out)

    def wo_dot(st, dst, k, g):
        if not st:
            st['o'] = ob[...]
        res = jnp.dot(st['o'][:, k * KH:(k + 1) * KH], wo[k * KH:(k + 1) * KH, g * 128:(g + 1) * 128],
                      preferred_element_type=F32)
        if k > 0:
            res = res + dst[:, g * 128:(g + 1) * 128]
        dst[:, g * 128:(g + 1) * 128] = res
        return res

    def tail_piece(i, r, gate=None):
        src = ab.at[i & 1]
        r0 = _aligned(i * T + r, LB)
        xn = xv[pl.ds(r0, LB), :].astype(F32) + mod_rows(2, LB) * _gated(src[r:r + LB, :], gate)
        x1[pl.ds(r0, LB), :] = xn
        hv = _ln_mod(xn, mod_rows(4, LB), mod_rows(3, LB)).astype(BF16)
        h2[pl.ds(r0, LB), :] = hv
        return _digest([hv])

    def tasks(fn, step, *args):
        return [functools.partial(fn, *args, r) for r in range(0, T, step)]

    def stream(dots, under, after=None):
        never = never_mask()
        prev, out = None, []
        per = len(dots) // len(under)
        for s, (fn, _, _, _) in enumerate(dots):
            out.append(fn())
            for task in (() if s % per else under[s // per]):
                dig = task(gate=None if prev is None else (never[0:8], prev))
                if s + LAG * per < len(dots):
                    _, w_ref, r, c = dots[s + LAG * per]
                    w_ref[r:r + 16, c:c + 128] = jnp.where(never, dig, w_ref[r:r + 16, c:c + 128])
            if after is not None and s % per == per - 1 and s // per in after:
                after[s // per]()
            prev = out[-1][-8:, :]
        return out

    def qkv_dots(slot, src, js):
        h = src[...]
        return [(functools.partial(qkv_dot, h, slot, j, k, g), wqkv.at[j], k * KH, g * 128)
                for j in js for k in range(D // KH) for g in range(NG)]

    def wo_dots(i):
        st = {}
        return [(functools.partial(wo_dot, st, ab.at[i & 1], k, g), wo, k * KH, g * 128)
                for k in range(D // KH) for g in range(NG)]

    def never_mask():
        return jnp.full((16, 128), flag[0], jnp.int32) > 0

    def swiglu(g, u):
        hg = 0.5 * g
        return ((hg * jnp.tanh(hg) + hg) * u).astype(BF16)

    def gate_up(b, f):
        r0 = _aligned(b * TB, TB)
        h = h2[pl.ds(r0, TB), :]
        g = jnp.dot(h, wg[f], preferred_element_type=F32)
        u = jnp.dot(h, wu[f], preferred_element_type=F32)
        act[...] = swiglu(g, u)

    def down(r0, a0, rows, f):
        d = jnp.dot(act[a0:a0 + rows, :], wd[f], preferred_element_type=F32)
        xn = x1[pl.ds(r0, rows), :] + mod_rows(5, rows) * d
        x1[pl.ds(r0, rows), :] = xn
        xv[pl.ds(r0, rows), :] = xn.astype(BF16)

    gs = [functools.partial(groupsum_piece, r, r + T // 4) for r in range(0, T, T // 4)]

    kb[0, :, 0:HALO, :] = jnp.zeros((NG, HALO, 128), F32)
    vb[0, :, 0:HALO, :] = jnp.zeros((NG, HALO, 128), F32)
    cp_qkv(0).wait()
    cp_mod(1).start()
    cp_x(0).start()

    def permute_q(r, carry):
        for u in range(128 // PB):
            permute_piece(0, pl.multiple_of(r * 128 + u * PB, PB))
        return carry
    jax.lax.fori_loop(0, D // 128, permute_q, 0)

    def mod_first(j, carry):
        cp_mod(j).wait()

        @pl.when(j == 1)
        def _():
            cp_qkv(1).start()
        mod_chunk(j)
        return carry
    jax.lax.fori_loop(0, 2, mod_first, 0)
    cp_x(0).wait()

    def ln_first(n, carry):
        for u in range(2):
            ln1_piece(0, ob, pl.multiple_of(n * 2 * LB + u * LB, LB))
        return carry
    jax.lax.fori_loop(0, T // (2 * LB), ln_first, 0)
    for j, (head, later) in enumerate(((3, (cp_qkv(2), cp_x(1))), (2, (cp_wo, cp_x(2))))):
        dots = qkv_dots(0, ob, (j,))
        stream(dots[:head], [[]] * head)
        cp_qkv(j + 1).wait()
        for cp in later:
            cp.start()
        pm = [functools.partial(permute_piece, j + 1, r) for r in range(0, D, PB)]
        stream(dots[head:], _deal(pm, NG - head))
    lo, l1 = tasks(logits_piece, RB, 0), tasks(ln1_piece, LB, 1, hnext)
    cp_x(1).wait()
    for j in range(2, 6):
        cp_mod(j).start()
    stream(qkv_dots(0, ob, (2,)), [lo[2 * g:2 * g + 2] + [l1[g]] for g in range(NG)])
    _run(gs)

    cp_wo.wait()
    for i in range(3, NT):
        cp_x(i).start()

    def step_a(i, carry):
        first = isinstance(i, int)
        if first:
            cp_x(i + 2).wait()
        else:
            @pl.when(i + 2 < NT)
            def _():
                cp_x(i + 2).wait()
        slot = i & 1
        ou = tasks(out_piece, RB, i, slot)
        l1 = tasks(ln1_piece, LB, i + 2 if first else jnp.minimum(i + 2, NT - 1), hnext)
        lo = tasks(logits_piece, RB, 1 - slot)
        under = [[ou[s]] + ([l1[s // 2]] if s & 1 else []) for s in range(16)]
        under += [[lo[k]] for k in range(8)]
        under += [lo[8:10], lo[10:12], lo[12:14], lo[14:16], [], [], [], []]
        dots = qkv_dots(1 - slot, hnext, range(3)) + wo_dots(i)
        if first:
            for q in range(NG):
                under[2 * q].append(functools.partial(wo_piece, q))
            stream(dots[:16], under[:16])
            for j in (2, 3, 4):
                cp_mod(j).wait()
            for f in range(NF):
                for cp in cp_ffn(f):
                    cp.start()
            md = _deal([functools.partial(mod_piece, j, g) for j in (2, 3, 4) for g in range(NG)], 16)
            stream(dots[16:], [a + b for a, b in zip(under[16:], md)], {14: lambda: _run(gs)})
        else:
            for k, t in enumerate(tasks(tail_piece, LB, i - 1)):
                under[16 + k].insert(0, t)
            stream(dots, under, {30: lambda: _run(gs)})
        return carry
    step_a(0, 0)
    jax.lax.fori_loop(1, NT - 1, step_a, 0)

    for cp in cp_ffn(0)[:2] + (cp_mod(5),):
        cp.wait()
    last = NT - 1

    h0 = h2[0:TB, :]

    def ffn_dot(w_ref, g):
        return jnp.dot(h0, w_ref[0, :, g * 128:(g + 1) * 128], preferred_element_type=F32)

    nc, wd7 = FC // 128, wo_dots(last)
    ou, t6, t7 = tasks(out_piece, RB, last, last & 1), tasks(tail_piece, LB, last - 1), tasks(tail_piece, LB, last)
    gd, ud = [[(functools.partial(ffn_dot, w, g), w.at[0], 0, g * 128) for g in range(nc)] for w in (wg, wu)]
    res = stream(gd + ud[:2] + wd7 + ud[2:],
                 [ou[3 * k:3 * k + 3] for k in range(6)] + [[t6[k], functools.partial(mod_piece, 5, k)] for k in range(NG)] + [t7[:4], t7[4:]])
    for g, u in enumerate(res[nc:nc + 2] + res[-2:]):
        act[:, g * 128:(g + 1) * 128] = swiglu(res[g], u)
    for f in range(NF):
        for cp in cp_ffn(f)[2 if f == 0 else 0:]:
            cp.wait()

    def step_b(n, carry):
        bp, fp = (n - 1) // NF, (n - 1) % NF
        r0 = pl.multiple_of(bp * TB, TB)
        down(r0, 0, TB, fp)
        gate_up(n // NF, n % NF)

        @pl.when(fp == NF - 1)
        def _():
            cp_out(r0, TB, bp).start()
        return carry
    jax.lax.fori_loop(1, NB * NF, step_b, 0)
    outs = [cp_out(b * TB, TB, b) for b in range(NB - 1)]
    for k, a0 in enumerate(range(0, TB, ZB)):
        down(S - TB + a0, a0, ZB, NF - 1)
        outs.append(cp_out(S - TB + a0, ZB, NB - 1 + k))
        outs[-1].start()
    for cp in outs:
        cp.wait()


@jax.jit
def pallas_adaLN_cond__sliding_local_dilated__swiglu_ffn__prompt_kernel(
    A_x: jax.Array,
    A_wqkv: jax.Array,
    A_wo: jax.Array,
    B_x: jax.Array,
    B_w_gate: jax.Array,
    B_w_up: jax.Array,
    B_w_down: jax.Array,
    c: jax.Array,
    w_mod: jax.Array,
):
    del B_x
    hbm = pl.BlockSpec(memory_space=pl.ANY)
    out = pl.pallas_call(
        _kernel,
        out_shape=jax.ShapeDtypeStruct((S, D), BF16),
        grid=(1,),
        in_specs=[hbm, hbm, hbm, hbm, hbm, hbm, pl.BlockSpec((1, D), lambda i: (0, 0)), hbm],
        out_specs=hbm,
        scratch_shapes=[
            pltpu.VMEM((S, D), BF16),
            pltpu.VMEM((3, D, D), BF16),
            pltpu.VMEM((3, D, D), BF16),
            pltpu.VMEM((D, D), BF16),
            pltpu.VMEM((NF, D, FC), BF16),
            pltpu.VMEM((NF, D, FC), BF16),
            pltpu.VMEM((NF, FC, D), BF16),
            pltpu.VMEM((6, D, D), BF16),
            pltpu.VMEM((D, 128), F32),
            pltpu.VMEM((6, 8, D), F32),
            pltpu.VMEM((T, D), BF16),
            pltpu.VMEM((2, NG, T, 128), F32),
            pltpu.VMEM((2, NG, HALO + T, 128), F32),
            pltpu.VMEM((2, NG, HALO + T, 128), F32),
            pltpu.VMEM((W * T, 128), BF16),
            pltpu.VMEM((W * T, 128), F32),
            pltpu.VMEM((T, D), BF16),
            pltpu.VMEM((2, T, D), F32),
            pltpu.VMEM((TB, FC), BF16),
            pltpu.VMEM((S, D), F32),
            pltpu.VMEM((S, D), BF16),
            pltpu.SMEM((1,), jnp.int32),
            pltpu.SemaphoreType.DMA((NT,)),
            pltpu.SemaphoreType.DMA((3,)),
            pltpu.SemaphoreType.DMA((6,)),
            pltpu.SemaphoreType.DMA((1 + 3 * NF,)),
            pltpu.SemaphoreType.DMA((NB - 1 + TB // ZB,)),
        ],
        compiler_params=pltpu.CompilerParams(vmem_limit_bytes=110 * 1024 * 1024),
    )(A_x.reshape(S, D), A_wqkv, A_wo, B_w_gate, B_w_up, B_w_down, c, w_mod)
    return out.reshape(1, S, D)
```

```python
import functools

import jax
import jax.numpy as jnp
import numpy as np
from jax.experimental import pallas as pl
from jax.experimental.pallas import tpu as pltpu

S, D, F = 2048, 1024, 3584
H, DH, W, DIL = 32, 32, 8, 2
HALO = 16
NG = D // 128
T = 256
TB = 1024
PB = 64
FC = 512
RB = 16
LB = 32
LAG = 3
KH = 1024
ZB = 128
EPS = 1e-5
assert DIL * (W // 2) == 8 and HALO >= DIL * (W - 1)
NT, NB, NF = S // T, S // TB, F // FC
FH = FC // 2
F32, BF16 = jnp.float32, jnp.bfloat16


def _spread_rows(v):
    sub = jax.lax.broadcasted_iota(jnp.int32, v[0].shape, 0)
    v = list(v)
    for s, d in ((4, 2), (2, 1)):
        low = (sub & s) == 0
        for a in range(4):
            if not a & d:
                va, vb = v[a], v[a + d]
                v[a] = jnp.where(low, va, pltpu.roll(vb, s, 0))
                v[a + d] = jnp.where(low, pltpu.roll(va, 8 - s, 0), vb)
    return v


def _spread_heads(cols):
    sub = (jax.lax.broadcasted_iota(jnp.int32, cols[0].shape, 1) >> 2) & 7
    out = [None] * NG
    for d in range(1 - NG, NG):
        js = [j for j in range(NG) if 0 <= j - d < NG]
        diag = cols[js[0]]
        for j in js[1:]:
            diag = jnp.where(sub == j - d, cols[j], diag)
        if d:
            diag = pltpu.roll(diag, (4 * d) % 128, 1)
        for j in js:
            out[j - d] = diag if out[j - d] is None else jnp.where(sub == j, diag, out[j - d])
    return out


def _ln_mod(x, scale1, shift):
    m = jnp.mean(x, axis=-1, keepdims=True)
    xc = x - m
    v = jnp.mean(xc * xc, axis=-1, keepdims=True)
    return xc * jax.lax.rsqrt(v + EPS) * scale1 + shift


def _aligned(v, n):
    return v if isinstance(v, int) else pl.multiple_of(v, n)


def _digest(blocks):
    out = None
    for b in blocks:
        for r in range(0, b.shape[0], 16):
            for c in range(0, b.shape[1], 128):
                v = pltpu.bitcast(b[r:r + 16, c:c + 128], jnp.uint32)
                out = v if out is None else out | v
    return pltpu.bitcast(out, BF16)


def _gated(x, gate):
    if gate is None:
        return x
    never, v = gate
    head = jnp.where(never, pltpu.bitcast(v, x.dtype), x[0:8, 0:128])
    if x.shape[1] > 128:
        head = jnp.concatenate([head, x[0:8, 128:]], axis=1)
    return jnp.concatenate([head, x[8:]], axis=0)


def _deal(tasks, n):
    return [tasks[k * len(tasks) // n:(k + 1) * len(tasks) // n] for k in range(n)]


def _run(tasks):
    for t in tasks:
        t()


def _kernel(x_hbm, wqkv_hbm, wo_hbm, wg_hbm, wu_hbm, wd_hbm, c_ref, wmod_hbm, out_hbm,
            xv, wraw, wqkv, wo, wgu, wd, hs, ws, wmod, sb, mod, hnext, qb, kb, vb, tb, lg, ob, ab, act, x1, h2, flag,
            sem_x, sem_qkv, sem_mod, sem_w, sem_out):
    def cp_x(i):
        return pltpu.make_async_copy(x_hbm.at[pl.ds(_aligned(i * T, T), T)], xv.at[pl.ds(_aligned(i * T, T), T)], sem_x.at[i])

    def cp_mod(j):
        return pltpu.make_async_copy(wmod_hbm.at[:, pl.ds(_aligned(j * D, D), D)], wmod.at[j], sem_mod.at[j])

    def cp_qkv(j):
        return pltpu.make_async_copy(wqkv_hbm.at[:, pl.ds(_aligned(j * D, D), D)], wraw.at[j], sem_qkv.at[j])

    cp_wo = pltpu.make_async_copy(wo_hbm, wraw.at[0], sem_w.at[0])

    def cp_ffn(f):
        c0 = f * FC
        cps = [pltpu.make_async_copy(src.at[:, c0 + p * FH:c0 + (p + 1) * FH],
                                     wgu.at[f, :, (2 * p + q) * FH:(2 * p + q + 1) * FH],
                                     sem_w.at[1 + 5 * f + 2 * p + q])
               for p in range(2) for q, src in enumerate((wg_hbm, wu_hbm))]
        return tuple(cps) + (pltpu.make_async_copy(wd_hbm.at[c0:c0 + FC, :], wd.at[f], sem_w.at[5 + 5 * f]),)

    def cp_out(row0, rows, k):
        return pltpu.make_async_copy(xv.at[pl.ds(row0, rows)], out_hbm.at[pl.ds(row0, rows)], sem_out.at[k])

    cp_qkv(0).start()
    cp_mod(0).start()
    flag[0] = 0
    cv = c_ref[...].astype(F32)
    sc = (cv * jax.nn.sigmoid(cv)).astype(BF16).astype(F32)
    for j in range(NG):
        row = jnp.broadcast_to(sc[:, j * 128:(j + 1) * 128], (128, 128))
        sb[j * 128:(j + 1) * 128, :] = row.T

    def mod_chunk(j):
        def body(r, acc):
            r0 = pl.multiple_of(r * 64, 64)
            s = sb[pl.ds(r0, 64), :]
            out = []
            for g in range(NG):
                t = wmod[j, pl.ds(r0, 64), g * 128:(g + 1) * 128].astype(F32) * s
                t = t[0:32] + t[32:64]
                t = t[0:16] + t[16:32]
                out.append(acc[g] + (t[0:8] + t[8:16]))
            return tuple(out)
        acc = jax.lax.fori_loop(0, D // 64, body, tuple(jnp.zeros((8, 128), F32) for _ in range(NG)))
        one = jnp.where((j == 1) | (j == 4), 1.0, 0.0)
        for g in range(NG):
            res = jnp.sum(acc[g], axis=0, keepdims=True) + one
            mod[j, :, g * 128:(g + 1) * 128] = jnp.broadcast_to(res, (8, 128))

    def mod_piece(j, g, gate=None):
        acc = [None, None]
        for n, r in enumerate(range(0, D, 16)):
            t = wmod[j, r:r + 16, g * 128:(g + 1) * 128].astype(F32) * sb[r:r + 16, :]
            t = _gated(t, gate) if n < 2 else t
            acc[n & 1] = t if n < 2 else acc[n & 1] + t
        res = jnp.sum(acc[0] + acc[1], axis=0, keepdims=True) + (1.0 if j in (1, 4) else 0.0)
        res = jnp.broadcast_to(res, (8, 128))
        mod[j, :, g * 128:(g + 1) * 128] = res
        return pltpu.bitcast(res, BF16)

    def mod_rows(j, rows):
        return jnp.concatenate([mod[j]] * (rows // 8), axis=0)

    def permute_piece(j, r, gate=None):
        cols = [pltpu.bitcast(wraw[j, pl.ds(r, PB), g * 128:(g + 1) * 128], jnp.uint32) for g in range(NG)]
        if gate is not None:
            cols = [_gated(c, gate) for c in cols]
        cols = [pltpu.bitcast(c, BF16) for c in _spread_heads(cols)]
        for g in range(NG):
            wqkv[j, pl.ds(r, PB), g * 128:(g + 1) * 128] = cols[g]
        return _digest(cols)

    def ln1_piece(i, dst, r, gate=None):
        r0 = _aligned(i * T + r, LB)
        xt = _gated(xv[pl.ds(r0, LB), :].astype(F32), gate)
        hv = _ln_mod(xt, mod_rows(1, LB), mod_rows(0, LB)).astype(BF16)
        dst[pl.ds(r, LB), :] = hv
        return _digest([hv])

    qscale = float(DH ** -0.5 * np.log2(np.e))

    def qkv_dot(h, slot, j, k, g):
        res = jnp.dot(h[:, k * KH:(k + 1) * KH], wqkv[j, k * KH:(k + 1) * KH, g * 128:(g + 1) * 128],
                      preferred_element_type=F32)
        buf, r0 = ((qb, 0), (kb, HALO), (vb, HALO))[j]
        if k > 0:
            res = res + buf[slot, g, r0:r0 + T, :]
        if k == D // KH - 1:
            if j == 0:
                res = res * qscale
            else:
                buf[1 - slot, g, 0:HALO, :] = res[T - HALO:, :]
        buf[slot, g, r0:r0 + T, :] = res
        return res

    def window(buf, slot, g, r):
        out = [None] * W
        for w in range(W // 2):
            o = HALO + r - DIL * w - 8
            rows = buf[slot, g, o:o + RB + 8, :]
            out[w], out[w + W // 2] = rows[8:], rows[:RB]
        return out

    def logits_piece(slot, r, gate=None):
        acc = [None] * W
        for g in range(NG):
            qv = qb[slot, g, r:r + RB, :]
            if g == 0:
                qv = _gated(qv, gate)
            for w, kv in enumerate(window(kb, slot, g, r)):
                p = qv * kv
                acc[w] = p if g == 0 else acc[w] + p
        acc = [a.astype(BF16) for a in acc]
        for w in range(W):
            tb[r * W + w * RB:r * W + (w + 1) * RB, :] = acc[w]
        return _digest(acc)

    def groupsum_piece(r0, r1):
        ri = jax.lax.broadcasted_iota(jnp.int32, (128, 128), 0)
        ci = jax.lax.broadcasted_iota(jnp.int32, (128, 128), 1)
        group_ones = jnp.where((ri >> 2) == (ci >> 2), 1.0, 0.0).astype(BF16)
        lg[r0 * W:r1 * W, :] = jnp.dot(tb[r0 * W:r1 * W, :], group_ones, preferred_element_type=F32)

    def out_piece(i, slot, r, gate=None):
        l = [lg[r * W + w * RB:r * W + (w + 1) * RB, :] for w in range(W)]
        if r < HALO and not (isinstance(i, int) and i > 0):
            pos = i * T + r + jax.lax.broadcasted_iota(jnp.int32, (RB, 128), 0)
            l = [l[0]] + [jnp.where(pos >= DIL * w, l[w], -1e9) for w in range(1, W)]
        l[0] = _gated(l[0], gate)
        m = l[0]
        for w in range(1, W):
            m = jnp.maximum(m, l[w])
        e = [jnp.exp2(l[w] - m) for w in range(W)]
        den = e[0]
        for w in range(1, W):
            den = den + e[w]
        inv = 1.0 / den
        p = [e[w] * inv for w in range(W)]
        cols = []
        for g in range(NG):
            acc = None
            for w, vv in enumerate(window(vb, slot, g, r)):
                t = p[w] * vv
                acc = t if w == 0 else acc + t
            cols.append(acc.astype(BF16))
            ob[r:r + RB, g * 128:(g + 1) * 128] = cols[g]
        return _digest(cols)

    def wo_piece(q, gate=None):
        del gate
        a, jh = divmod(q, 2)
        out = []
        for half in range(2):
            rows = [(4 * jh + p) * 128 + a * DH + half * 16 for p in range(4)]
            v = _spread_rows([pltpu.bitcast(wraw[0, r0:r0 + 16, :], jnp.uint32) for r0 in rows])
            for b in range(4):
                r1 = (half * 4 + b) * 128 + a * DH + jh * 16
                out.append(pltpu.bitcast(v[b], BF16))
                wo[r1:r1 + 16, :] = out[-1]
        return _digest(out)

    def wo_dot(st, dst, k, g):
        if not st:
            st['o'] = ob[...]
        res = jnp.dot(st['o'][:, k * KH:(k + 1) * KH], wo[k * KH:(k + 1) * KH, g * 128:(g + 1) * 128],
                      preferred_element_type=F32)
        if k > 0:
            res = res + dst[:, g * 128:(g + 1) * 128]
        dst[:, g * 128:(g + 1) * 128] = res
        return res

    def tail_piece(i, r, gate=None):
        src = ab.at[i & 1]
        r0 = _aligned(i * T + r, LB)
        xn = xv[pl.ds(r0, LB), :].astype(F32) + mod_rows(2, LB) * _gated(src[r:r + LB, :], gate)
        x1[pl.ds(r0, LB), :] = xn
        hv = _ln_mod(xn, mod_rows(4, LB), mod_rows(3, LB)).astype(BF16)
        h2[pl.ds(r0, LB), :] = hv
        return _digest([hv])

    def tasks(fn, step, *args):
        return [functools.partial(fn, *args, r) for r in range(0, T, step)]

    def stream(dots, under, after=None):
        never = never_mask()
        prev, out = None, []
        per = len(dots) // len(under)
        for s, (fn, _, _, _) in enumerate(dots):
            out.append(fn())
            for task in (() if s % per else under[s // per]):
                dig = task(gate=None if prev is None else (never[0:8], prev))
                if s + LAG * per < len(dots):
                    _, w_ref, r, c = dots[s + LAG * per]
                    w_ref[r:r + 16, c:c + 128] = jnp.where(never, dig, w_ref[r:r + 16, c:c + 128])
            if after is not None and s % per == per - 1 and s // per in after:
                after[s // per]()
            prev = out[-1][-8:, :]
        return out

    def qkv_dots(slot, src, js):
        h = src[...]
        return [(functools.partial(qkv_dot, h, slot, j, k, g), wqkv.at[j], k * KH, g * 128)
                for j in js for k in range(D // KH) for g in range(NG)]

    def wo_dots(i):
        st = {}
        return [(functools.partial(wo_dot, st, ab.at[i & 1], k, g), wo, k * KH, g * 128)
                for k in range(D // KH) for g in range(NG)]

    def never_mask():
        return jnp.full((16, 128), flag[0], jnp.int32) > 0

    def swiglu(g, u):
        hg = 0.5 * g
        return ((hg * jnp.tanh(hg) + hg) * u).astype(BF16)

    HM, HK = TB // 2, D // 2

    def combine(x, y, sign):
        x, y = x.astype(F32), y.astype(F32)
        return (x + y if sign > 0 else x - y).astype(BF16)

    def lhs_sums(b):
        def body(n, carry):
            r = pl.multiple_of(n * 64, 64)
            top, bot = pl.ds(_aligned(b * TB, TB) + r, 64), pl.ds(_aligned(b * TB, TB) + HM + r, 64)
            a11, a12, a21, a22 = h2[top, :HK], h2[top, HK:], h2[bot, :HK], h2[bot, HK:]
            for k, (x, y, sign) in enumerate(((a11, a22, 1), (a21, a22, 1), (a11, a12, 1),
                                              (a21, a11, -1), (a12, a22, -1))):
                hs[k, pl.ds(r, 64), :] = combine(x, y, sign)
            return carry
        jax.lax.fori_loop(0, HM // 64, body, 0)

    def rhs_sums(f, r):
        top, bot = slice(r, r + 64), slice(HK + r, HK + r + 64)
        b11, b12, b21, b22 = wgu[f, top, :FC], wgu[f, top, FC:], wgu[f, bot, :FC], wgu[f, bot, FC:]
        out = [combine(x, y, sign) for x, y, sign in ((b11, b22, 1), (b12, b22, -1), (b21, b11, -1),
                                                      (b11, b12, 1), (b21, b22, 1))]
        for k, v in enumerate(out):
            ws[k, r:r + 64, :] = v

    def gate_up(b, f):
        r0 = _aligned(b * TB, TB)
        mm = functools.partial(jnp.dot, preferred_element_type=F32)

        def emit(rows, half, c):
            act[rows, half * FH:(half + 1) * FH] = swiglu(c[:, :FH], c[:, FH:])

        m2 = mm(hs[1], wgu[f, :HK, :FC])
        m4 = mm(h2[pl.ds(r0 + HM, HM), HK:], ws[2])
        emit(slice(HM, TB), 0, m2 + m4)
        m5 = mm(hs[2], wgu[f, HK:, FC:])
        m3 = mm(h2[pl.ds(r0, HM), :HK], ws[1])
        emit(slice(0, HM), 1, m3 + m5)
        c11, c22 = m4 - m5, m3 - m2
        m1 = mm(hs[0], ws[0])
        c11, c22 = c11 + m1, c22 + m1
        emit(slice(0, HM), 0, c11 + mm(hs[4], ws[4]))
        emit(slice(HM, TB), 1, c22 + mm(hs[3], ws[3]))

    def down(r0, a0, rows, f):
        d = jnp.dot(act[a0:a0 + rows, :], wd[f], preferred_element_type=F32)
        xn = x1[pl.ds(r0, rows), :] + mod_rows(5, rows) * d
        x1[pl.ds(r0, rows), :] = xn
        xv[pl.ds(r0, rows), :] = xn.astype(BF16)

    gs = [functools.partial(groupsum_piece, r, r + T // 4) for r in range(0, T, T // 4)]

    kb[0, :, 0:HALO, :] = jnp.zeros((NG, HALO, 128), F32)
    vb[0, :, 0:HALO, :] = jnp.zeros((NG, HALO, 128), F32)
    cp_qkv(0).wait()
    cp_mod(1).start()
    cp_x(0).start()

    def permute_q(r, carry):
        for u in range(128 // PB):
            permute_piece(0, pl.multiple_of(r * 128 + u * PB, PB))
        return carry
    jax.lax.fori_loop(0, D // 128, permute_q, 0)

    def mod_first(j, carry):
        cp_mod(j).wait()

        @pl.when(j == 1)
        def _():
            cp_qkv(1).start()
        mod_chunk(j)
        return carry
    jax.lax.fori_loop(0, 2, mod_first, 0)
    cp_x(0).wait()

    def ln_first(n, carry):
        for u in range(2):
            ln1_piece(0, ob, pl.multiple_of(n * 2 * LB + u * LB, LB))
        return carry
    jax.lax.fori_loop(0, T // (2 * LB), ln_first, 0)
    for j, (head, later) in enumerate(((3, (cp_qkv(2), cp_x(1))), (2, (cp_wo, cp_x(2))))):
        dots = qkv_dots(0, ob, (j,))
        stream(dots[:head], [[]] * head)
        cp_qkv(j + 1).wait()
        for cp in later:
            cp.start()
        pm = [functools.partial(permute_piece, j + 1, r) for r in range(0, D, PB)]
        stream(dots[head:], _deal(pm, NG - head))
    lo, l1 = tasks(logits_piece, RB, 0), tasks(ln1_piece, LB, 1, hnext)
    cp_x(1).wait()
    for j in range(2, 6):
        cp_mod(j).start()
    stream(qkv_dots(0, ob, (2,)), [lo[2 * g:2 * g + 2] + [l1[g]] for g in range(NG)])
    _run(gs)

    cp_wo.wait()
    for i in range(3, NT):
        cp_x(i).start()

    def step_a(i, carry):
        first = isinstance(i, int)
        if first:
            cp_x(i + 2).wait()
        else:
            @pl.when(i + 2 < NT)
            def _():
                cp_x(i + 2).wait()
        slot = i & 1
        ou = tasks(out_piece, RB, i, slot)
        l1 = tasks(ln1_piece, LB, i + 2 if first else jnp.minimum(i + 2, NT - 1), hnext)
        lo = tasks(logits_piece, RB, 1 - slot)
        under = [[ou[s]] + ([l1[s // 2]] if s & 1 else []) for s in range(16)]
        under += [[lo[k]] for k in range(8)]
        under += [lo[8:10], lo[10:12], lo[12:14], lo[14:16], [], [], [], []]
        dots = qkv_dots(1 - slot, hnext, range(3)) + wo_dots(i)
        if first:
            for q in range(NG):
                under[2 * q].append(functools.partial(wo_piece, q))
            stream(dots[:16], under[:16])
            for j in (2, 3, 4):
                cp_mod(j).wait()
            for f in range(NF):
                for cp in cp_ffn(f):
                    cp.start()
            md = _deal([functools.partial(mod_piece, j, g) for j in (2, 3, 4) for g in range(NG)], 16)
            stream(dots[16:], [a + b for a, b in zip(under[16:], md)], {14: lambda: _run(gs)})
        else:
            for k, t in enumerate(tasks(tail_piece, LB, i - 1)):
                under[16 + k].insert(0, t)
            stream(dots, under, {30: lambda: _run(gs)})
        return carry
    step_a(0, 0)
    jax.lax.fori_loop(1, NT - 1, step_a, 0)

    for cp in cp_ffn(0)[:4] + (cp_mod(5),):
        cp.wait()
    last = NT - 1

    h0 = h2[0:TB, :]

    def ffn_dot(c):
        return jnp.dot(h0, wgu[0, :, c:c + 128], preferred_element_type=F32)

    nc, wd7 = FC // 128, wo_dots(last)
    ou, t6, t7 = tasks(out_piece, RB, last, last & 1), tasks(tail_piece, LB, last - 1), tasks(tail_piece, LB, last)
    gcols = [(g * 128 // FH) * 2 * FH + g * 128 % FH for g in range(nc)]
    gd, ud = [[(functools.partial(ffn_dot, c + off), wgu.at[0], 0, c + off) for c in gcols] for off in (0, FH)]
    res = stream(gd + ud[:2] + wd7 + ud[2:],
                 [ou[3 * k:3 * k + 3] for k in range(6)] + [[t6[k], functools.partial(mod_piece, 5, k)] for k in range(NG)] + [t7[:4], t7[4:]])
    for g, u in enumerate(res[nc:nc + 2] + res[-2:]):
        act[:, g * 128:(g + 1) * 128] = swiglu(res[g], u)
    for f in range(NF):
        for cp in cp_ffn(f)[4 if f == 0 else 0:]:
            cp.wait()

    lhs_sums(0)

    def step_b(n, carry):
        bp, fp = (n - 1) // NF, (n - 1) % NF
        r0 = pl.multiple_of(bp * TB, TB)

        @pl.when(n % NF == 0)
        def _():
            lhs_sums(n // NF)
        for r in range(0, HK, 64):
            rhs_sums(n % NF, r)
        down(r0, 0, TB, fp)
        gate_up(n // NF, n % NF)

        @pl.when(fp == NF - 1)
        def _():
            cp_out(r0, TB, bp).start()
        return carry
    jax.lax.fori_loop(1, NB * NF, step_b, 0)
    outs = [cp_out(b * TB, TB, b) for b in range(NB - 1)]
    for k, a0 in enumerate(range(0, TB, ZB)):
        down(S - TB + a0, a0, ZB, NF - 1)
        outs.append(cp_out(S - TB + a0, ZB, NB - 1 + k))
        outs[-1].start()
    for cp in outs:
        cp.wait()


@jax.jit
def pallas_adaLN_cond__sliding_local_dilated__swiglu_ffn__prompt_kernel(
    A_x: jax.Array,
    A_wqkv: jax.Array,
    A_wo: jax.Array,
    B_x: jax.Array,
    B_w_gate: jax.Array,
    B_w_up: jax.Array,
    B_w_down: jax.Array,
    c: jax.Array,
    w_mod: jax.Array,
):
    del B_x
    hbm = pl.BlockSpec(memory_space=pl.ANY)
    out = pl.pallas_call(
        _kernel,
        out_shape=jax.ShapeDtypeStruct((S, D), BF16),
        grid=(1,),
        in_specs=[hbm, hbm, hbm, hbm, hbm, hbm, pl.BlockSpec((1, D), lambda i: (0, 0)), hbm],
        out_specs=hbm,
        scratch_shapes=[
            pltpu.VMEM((S, D), BF16),
            pltpu.VMEM((3, D, D), BF16),
            pltpu.VMEM((3, D, D), BF16),
            pltpu.VMEM((D, D), BF16),
            pltpu.VMEM((NF, D, 2 * FC), BF16),
            pltpu.VMEM((NF, FC, D), BF16),
            pltpu.VMEM((5, TB // 2, D // 2), BF16),
            pltpu.VMEM((5, D // 2, FC), BF16),
            pltpu.VMEM((6, D, D), BF16),
            pltpu.VMEM((D, 128), F32),
            pltpu.VMEM((6, 8, D), F32),
            pltpu.VMEM((T, D), BF16),
            pltpu.VMEM((2, NG, T, 128), F32),
            pltpu.VMEM((2, NG, HALO + T, 128), F32),
            pltpu.VMEM((2, NG, HALO + T, 128), F32),
            pltpu.VMEM((W * T, 128), BF16),
            pltpu.VMEM((W * T, 128), F32),
            pltpu.VMEM((T, D), BF16),
            pltpu.VMEM((2, T, D), F32),
            pltpu.VMEM((TB, FC), BF16),
            pltpu.VMEM((S, D), F32),
            pltpu.VMEM((S, D), BF16),
            pltpu.SMEM((1,), jnp.int32),
            pltpu.SemaphoreType.DMA((NT,)),
            pltpu.SemaphoreType.DMA((3,)),
            pltpu.SemaphoreType.DMA((6,)),
            pltpu.SemaphoreType.DMA((1 + 5 * NF,)),
            pltpu.SemaphoreType.DMA((NB - 1 + TB // ZB,)),
        ],
        compiler_params=pltpu.CompilerParams(vmem_limit_bytes=110 * 1024 * 1024),
    )(A_x.reshape(S, D), A_wqkv, A_wo, B_w_gate, B_w_up, B_w_down, c, w_mod)
    return out.reshape(1, S, D)
```

```python
import functools

import jax
import jax.numpy as jnp
import numpy as np
from jax.experimental import pallas as pl
from jax.experimental.pallas import tpu as pltpu

S, D, F = 2048, 1024, 3584
H, DH, W, DIL = 32, 32, 8, 2
HALO = 16
NG = D // 128
T = 256
TB = 1024
PB = 64
FC = 512
RB = 16
LB = 32
LAG = 3
KH = 1024
ZB = 128
EPS = 1e-5
assert DIL * (W // 2) == 8 and HALO >= DIL * (W - 1)
NT, NB, NF = S // T, S // TB, F // FC
FH = FC // 2
F32, BF16 = jnp.float32, jnp.bfloat16


def _spread_rows(v):
    sub = jax.lax.broadcasted_iota(jnp.int32, v[0].shape, 0)
    v = list(v)
    for s, d in ((4, 2), (2, 1)):
        low = (sub & s) == 0
        for a in range(4):
            if not a & d:
                va, vb = v[a], v[a + d]
                v[a] = jnp.where(low, va, pltpu.roll(vb, s, 0))
                v[a + d] = jnp.where(low, pltpu.roll(va, 8 - s, 0), vb)
    return v


def _spread_heads(cols):
    sub = (jax.lax.broadcasted_iota(jnp.int32, cols[0].shape, 1) >> 2) & 7
    out = [None] * NG
    for d in range(1 - NG, NG):
        js = [j for j in range(NG) if 0 <= j - d < NG]
        diag = cols[js[0]]
        for j in js[1:]:
            diag = jnp.where(sub == j - d, cols[j], diag)
        if d:
            diag = pltpu.roll(diag, (4 * d) % 128, 1)
        for j in js:
            out[j - d] = diag if out[j - d] is None else jnp.where(sub == j, diag, out[j - d])
    return out


def _ln_mod(x, scale1, shift):
    m = jnp.mean(x, axis=-1, keepdims=True)
    xc = x - m
    v = jnp.mean(xc * xc, axis=-1, keepdims=True)
    return xc * jax.lax.rsqrt(v + EPS) * scale1 + shift


def _aligned(v, n):
    return v if isinstance(v, int) else pl.multiple_of(v, n)


def _digest(blocks):
    out = None
    for b in blocks:
        for r in range(0, b.shape[0], 16):
            for c in range(0, b.shape[1], 128):
                v = pltpu.bitcast(b[r:r + 16, c:c + 128], jnp.uint32)
                out = v if out is None else out | v
    return pltpu.bitcast(out, BF16)


def _gated(x, gate):
    if gate is None:
        return x
    never, v = gate
    head = jnp.where(never, pltpu.bitcast(v, x.dtype), x[0:8, 0:128])
    if x.shape[1] > 128:
        head = jnp.concatenate([head, x[0:8, 128:]], axis=1)
    return jnp.concatenate([head, x[8:]], axis=0)


def _deal(tasks, n):
    return [tasks[k * len(tasks) // n:(k + 1) * len(tasks) // n] for k in range(n)]


def _run(tasks):
    for t in tasks:
        t()


def _kernel(x_hbm, wqkv_hbm, wo_hbm, wg_hbm, wu_hbm, wd_hbm, c_ref, wmod_hbm, out_hbm,
            xv, wraw, wqkv, wo, wgu, wd, hs, ws, wds, wmod, sb, mod, hnext, qb, kb, vb, tb, lg, ob, ab, act, x1, h2, flag,
            sem_x, sem_qkv, sem_mod, sem_w, sem_out):
    def cp_x(i):
        return pltpu.make_async_copy(x_hbm.at[pl.ds(_aligned(i * T, T), T)], xv.at[pl.ds(_aligned(i * T, T), T)], sem_x.at[i])

    def cp_mod(j):
        return pltpu.make_async_copy(wmod_hbm.at[:, pl.ds(_aligned(j * D, D), D)], wmod.at[j], sem_mod.at[j])

    def cp_qkv(j):
        return pltpu.make_async_copy(wqkv_hbm.at[:, pl.ds(_aligned(j * D, D), D)], wraw.at[j], sem_qkv.at[j])

    cp_wo = pltpu.make_async_copy(wo_hbm, wraw.at[0], sem_w.at[0])

    def cp_ffn(f):
        c0 = f * FC
        cps = [pltpu.make_async_copy(src.at[:, c0 + p * FH:c0 + (p + 1) * FH],
                                     wgu.at[f, :, (2 * p + q) * FH:(2 * p + q + 1) * FH],
                                     sem_w.at[1 + 5 * f + 2 * p + q])
               for p in range(2) for q, src in enumerate((wg_hbm, wu_hbm))]
        return tuple(cps) + (pltpu.make_async_copy(wd_hbm.at[c0:c0 + FC, :], wd.at[f], sem_w.at[5 + 5 * f]),)

    def cp_out(row0, rows, k):
        return pltpu.make_async_copy(xv.at[pl.ds(row0, rows)], out_hbm.at[pl.ds(row0, rows)], sem_out.at[k])

    cp_qkv(0).start()
    cp_mod(0).start()
    flag[0] = 0
    cv = c_ref[...].astype(F32)
    sc = (cv * jax.nn.sigmoid(cv)).astype(BF16).astype(F32)
    for j in range(NG):
        row = jnp.broadcast_to(sc[:, j * 128:(j + 1) * 128], (128, 128))
        sb[j * 128:(j + 1) * 128, :] = row.T

    def mod_chunk(j):
        def body(r, acc):
            r0 = pl.multiple_of(r * 64, 64)
            s = sb[pl.ds(r0, 64), :]
            out = []
            for g in range(NG):
                t = wmod[j, pl.ds(r0, 64), g * 128:(g + 1) * 128].astype(F32) * s
                t = t[0:32] + t[32:64]
                t = t[0:16] + t[16:32]
                out.append(acc[g] + (t[0:8] + t[8:16]))
            return tuple(out)
        acc = jax.lax.fori_loop(0, D // 64, body, tuple(jnp.zeros((8, 128), F32) for _ in range(NG)))
        one = jnp.where((j == 1) | (j == 4), 1.0, 0.0)
        for g in range(NG):
            res = jnp.sum(acc[g], axis=0, keepdims=True) + one
            mod[j, :, g * 128:(g + 1) * 128] = jnp.broadcast_to(res, (8, 128))

    def mod_piece(j, g, gate=None):
        acc = [None, None]
        for n, r in enumerate(range(0, D, 16)):
            t = wmod[j, r:r + 16, g * 128:(g + 1) * 128].astype(F32) * sb[r:r + 16, :]
            t = _gated(t, gate) if n < 2 else t
            acc[n & 1] = t if n < 2 else acc[n & 1] + t
        res = jnp.sum(acc[0] + acc[1], axis=0, keepdims=True) + (1.0 if j in (1, 4) else 0.0)
        res = jnp.broadcast_to(res, (8, 128))
        mod[j, :, g * 128:(g + 1) * 128] = res
        return pltpu.bitcast(res, BF16)

    def mod_rows(j, rows):
        return jnp.concatenate([mod[j]] * (rows // 8), axis=0)

    def permute_piece(j, r, gate=None):
        cols = [pltpu.bitcast(wraw[j, pl.ds(r, PB), g * 128:(g + 1) * 128], jnp.uint32) for g in range(NG)]
        if gate is not None:
            cols = [_gated(c, gate) for c in cols]
        cols = [pltpu.bitcast(c, BF16) for c in _spread_heads(cols)]
        for g in range(NG):
            wqkv[j, pl.ds(r, PB), g * 128:(g + 1) * 128] = cols[g]
        return _digest(cols)

    def ln1_piece(i, dst, r, gate=None):
        r0 = _aligned(i * T + r, LB)
        xt = _gated(xv[pl.ds(r0, LB), :].astype(F32), gate)
        hv = _ln_mod(xt, mod_rows(1, LB), mod_rows(0, LB)).astype(BF16)
        dst[pl.ds(r, LB), :] = hv
        return _digest([hv])

    qscale = float(DH ** -0.5 * np.log2(np.e))

    def qkv_dot(h, slot, j, k, g):
        res = jnp.dot(h[:, k * KH:(k + 1) * KH], wqkv[j, k * KH:(k + 1) * KH, g * 128:(g + 1) * 128],
                      preferred_element_type=F32)
        buf, r0 = ((qb, 0), (kb, HALO), (vb, HALO))[j]
        if k > 0:
            res = res + buf[slot, g, r0:r0 + T, :]
        if k == D // KH - 1:
            if j == 0:
                res = res * qscale
            else:
                buf[1 - slot, g, 0:HALO, :] = res[T - HALO:, :]
        buf[slot, g, r0:r0 + T, :] = res
        return res

    def window(buf, slot, g, r):
        out = [None] * W
        for w in range(W // 2):
            o = HALO + r - DIL * w - 8
            rows = buf[slot, g, o:o + RB + 8, :]
            out[w], out[w + W // 2] = rows[8:], rows[:RB]
        return out

    def logits_piece(slot, r, gate=None):
        acc = [None] * W
        for g in range(NG):
            qv = qb[slot, g, r:r + RB, :]
            if g == 0:
                qv = _gated(qv, gate)
            for w, kv in enumerate(window(kb, slot, g, r)):
                p = qv * kv
                acc[w] = p if g == 0 else acc[w] + p
        acc = [a.astype(BF16) for a in acc]
        for w in range(W):
            tb[r * W + w * RB:r * W + (w + 1) * RB, :] = acc[w]
        return _digest(acc)

    def groupsum_piece(r0, r1):
        ri = jax.lax.broadcasted_iota(jnp.int32, (128, 128), 0)
        ci = jax.lax.broadcasted_iota(jnp.int32, (128, 128), 1)
        group_ones = jnp.where((ri >> 2) == (ci >> 2), 1.0, 0.0).astype(BF16)
        lg[r0 * W:r1 * W, :] = jnp.dot(tb[r0 * W:r1 * W, :], group_ones, preferred_element_type=F32)

    def out_piece(i, slot, r, gate=None):
        l = [lg[r * W + w * RB:r * W + (w + 1) * RB, :] for w in range(W)]
        if r < HALO and not (isinstance(i, int) and i > 0):
            pos = i * T + r + jax.lax.broadcasted_iota(jnp.int32, (RB, 128), 0)
            l = [l[0]] + [jnp.where(pos >= DIL * w, l[w], -1e9) for w in range(1, W)]
        l[0] = _gated(l[0], gate)
        m = l[0]
        for w in range(1, W):
            m = jnp.maximum(m, l[w])
        e = [jnp.exp2(l[w] - m) for w in range(W)]
        den = e[0]
        for w in range(1, W):
            den = den + e[w]
        inv = 1.0 / den
        p = [e[w] * inv for w in range(W)]
        cols = []
        for g in range(NG):
            acc = None
            for w, vv in enumerate(window(vb, slot, g, r)):
                t = p[w] * vv
                acc = t if w == 0 else acc + t
            cols.append(acc.astype(BF16))
            ob[r:r + RB, g * 128:(g + 1) * 128] = cols[g]
        return _digest(cols)

    def wo_piece(q, gate=None):
        del gate
        a, jh = divmod(q, 2)
        out = []
        for half in range(2):
            rows = [(4 * jh + p) * 128 + a * DH + half * 16 for p in range(4)]
            v = _spread_rows([pltpu.bitcast(wraw[0, r0:r0 + 16, :], jnp.uint32) for r0 in rows])
            for b in range(4):
                r1 = (half * 4 + b) * 128 + a * DH + jh * 16
                out.append(pltpu.bitcast(v[b], BF16))
                wo[r1:r1 + 16, :] = out[-1]
        return _digest(out)

    def wo_dot(st, dst, k, g):
        if not st:
            st['o'] = ob[...]
        res = jnp.dot(st['o'][:, k * KH:(k + 1) * KH], wo[k * KH:(k + 1) * KH, g * 128:(g + 1) * 128],
                      preferred_element_type=F32)
        if k > 0:
            res = res + dst[:, g * 128:(g + 1) * 128]
        dst[:, g * 128:(g + 1) * 128] = res
        return res

    def tail_piece(i, r, gate=None):
        src = ab.at[i & 1]
        r0 = _aligned(i * T + r, LB)
        xn = xv[pl.ds(r0, LB), :].astype(F32) + mod_rows(2, LB) * _gated(src[r:r + LB, :], gate)
        x1[pl.ds(r0, LB), :] = xn
        hv = _ln_mod(xn, mod_rows(4, LB), mod_rows(3, LB)).astype(BF16)
        h2[pl.ds(r0, LB), :] = hv
        return _digest([hv])

    def tasks(fn, step, *args):
        return [functools.partial(fn, *args, r) for r in range(0, T, step)]

    def stream(dots, under, after=None):
        never = never_mask()
        prev, out = None, []
        per = len(dots) // len(under)
        for s, (fn, _, _, _) in enumerate(dots):
            out.append(fn())
            for task in (() if s % per else under[s // per]):
                dig = task(gate=None if prev is None else (never[0:8], prev))
                if s + LAG * per < len(dots):
                    _, w_ref, r, c = dots[s + LAG * per]
                    w_ref[r:r + 16, c:c + 128] = jnp.where(never, dig, w_ref[r:r + 16, c:c + 128])
            if after is not None and s % per == per - 1 and s // per in after:
                after[s // per]()
            prev = out[-1][-8:, :]
        return out

    def qkv_dots(slot, src, js):
        h = src[...]
        return [(functools.partial(qkv_dot, h, slot, j, k, g), wqkv.at[j], k * KH, g * 128)
                for j in js for k in range(D // KH) for g in range(NG)]

    def wo_dots(i):
        st = {}
        return [(functools.partial(wo_dot, st, ab.at[i & 1], k, g), wo, k * KH, g * 128)
                for k in range(D // KH) for g in range(NG)]

    def never_mask():
        return jnp.full((16, 128), flag[0], jnp.int32) > 0

    def swiglu(g, u):
        hg = 0.5 * g
        return ((hg * jnp.tanh(hg) + hg) * u).astype(BF16)

    HM, HK = TB // 2, D // 2

    def combine(x, y, sign):
        x, y = x.astype(F32), y.astype(F32)
        return (x + y if sign > 0 else x - y).astype(BF16)

    def lhs_sums(b):
        def body(n, carry):
            r = pl.multiple_of(n * 64, 64)
            top, bot = pl.ds(_aligned(b * TB, TB) + r, 64), pl.ds(_aligned(b * TB, TB) + HM + r, 64)
            a11, a12, a21, a22 = h2[top, :HK], h2[top, HK:], h2[bot, :HK], h2[bot, HK:]
            for k, (x, y, sign) in enumerate(((a11, a22, 1), (a21, a22, 1), (a11, a12, 1),
                                              (a21, a11, -1), (a12, a22, -1))):
                hs[k, pl.ds(r, 64), :] = combine(x, y, sign)
            return carry
        jax.lax.fori_loop(0, HM // 64, body, 0)

    def rhs_sums(w_ref, dst):
        hk, hn = w_ref.shape[0] // 2, w_ref.shape[1] // 2
        for r in range(0, hk, 64):
            top, bot = slice(r, r + 64), slice(hk + r, hk + r + 64)
            b11, b12, b21, b22 = w_ref[top, :hn], w_ref[top, hn:], w_ref[bot, :hn], w_ref[bot, hn:]
            for k, (x, y, sign) in enumerate(((b11, b22, 1), (b12, b22, -1), (b21, b11, -1),
                                              (b11, b12, 1), (b21, b22, 1))):
                dst[k, top, :] = combine(x, y, sign)

    mm = functools.partial(jnp.dot, preferred_element_type=F32)

    def add_residual(rows, cols, d):
        xn = x1[rows, cols] + mod_rows(5, d.shape[0])[:, cols] * d
        x1[rows, cols] = xn
        xv[rows, cols] = xn.astype(BF16)

    def down_strassen(r0, f):
        top, bot, lo, hi = pl.ds(r0, HM), pl.ds(r0 + HM, HM), slice(0, HK), slice(HK, D)
        a11, a12, a21, a22 = act[:HM, :FH], act[:HM, FH:], act[HM:, :FH], act[HM:, FH:]
        m3, m4 = mm(a11, wds[1]), mm(a22, wds[2])
        m5 = mm(combine(a11, a12, 1), wd[f, FH:, HK:])
        add_residual(top, hi, m3 + m5)
        m2 = mm(combine(a21, a22, 1), wd[f, :FH, :HK])
        add_residual(bot, lo, m2 + m4)
        m1 = mm(combine(a11, a22, 1), wds[0])
        c11, c22 = m4 - m5 + m1, m3 - m2 + m1
        add_residual(top, lo, c11 + mm(combine(a12, a22, -1), wds[4]))
        add_residual(bot, hi, c22 + mm(combine(a21, a11, -1), wds[3]))

    def gate_up(b, f):
        r0 = _aligned(b * TB, TB)

        def emit(rows, half, c):
            act[rows, half * FH:(half + 1) * FH] = swiglu(c[:, :FH], c[:, FH:])

        m2 = mm(hs[1], wgu[f, :HK, :FC])
        m4 = mm(h2[pl.ds(r0 + HM, HM), HK:], ws[2])
        emit(slice(HM, TB), 0, m2 + m4)
        m5 = mm(hs[2], wgu[f, HK:, FC:])
        m3 = mm(h2[pl.ds(r0, HM), :HK], ws[1])
        emit(slice(0, HM), 1, m3 + m5)
        c11, c22 = m4 - m5, m3 - m2
        m1 = mm(hs[0], ws[0])
        c11, c22 = c11 + m1, c22 + m1
        emit(slice(0, HM), 0, c11 + mm(hs[4], ws[4]))
        emit(slice(HM, TB), 1, c22 + mm(hs[3], ws[3]))

    gs = [functools.partial(groupsum_piece, r, r + T // 4) for r in range(0, T, T // 4)]

    kb[0, :, 0:HALO, :] = jnp.zeros((NG, HALO, 128), F32)
    vb[0, :, 0:HALO, :] = jnp.zeros((NG, HALO, 128), F32)
    cp_qkv(0).wait()
    cp_mod(1).start()
    cp_x(0).start()

    def permute_q(r, carry):
        for u in range(128 // PB):
            permute_piece(0, pl.multiple_of(r * 128 + u * PB, PB))
        return carry
    jax.lax.fori_loop(0, D // 128, permute_q, 0)

    def mod_first(j, carry):
        cp_mod(j).wait()

        @pl.when(j == 1)
        def _():
            cp_qkv(1).start()
        mod_chunk(j)
        return carry
    jax.lax.fori_loop(0, 2, mod_first, 0)
    cp_x(0).wait()

    def ln_first(n, carry):
        for u in range(2):
            ln1_piece(0, ob, pl.multiple_of(n * 2 * LB + u * LB, LB))
        return carry
    jax.lax.fori_loop(0, T // (2 * LB), ln_first, 0)
    for j, (head, later) in enumerate(((3, (cp_qkv(2), cp_x(1))), (2, (cp_wo, cp_x(2))))):
        dots = qkv_dots(0, ob, (j,))
        stream(dots[:head], [[]] * head)
        cp_qkv(j + 1).wait()
        for cp in later:
            cp.start()
        pm = [functools.partial(permute_piece, j + 1, r) for r in range(0, D, PB)]
        stream(dots[head:], _deal(pm, NG - head))
    lo, l1 = tasks(logits_piece, RB, 0), tasks(ln1_piece, LB, 1, hnext)
    cp_x(1).wait()
    for j in range(2, 6):
        cp_mod(j).start()
    stream(qkv_dots(0, ob, (2,)), [lo[2 * g:2 * g + 2] + [l1[g]] for g in range(NG)])
    _run(gs)

    cp_wo.wait()
    for i in range(3, NT):
        cp_x(i).start()

    def step_a(i, carry):
        first = isinstance(i, int)
        if first:
            cp_x(i + 2).wait()
        else:
            @pl.when(i + 2 < NT)
            def _():
                cp_x(i + 2).wait()
        slot = i & 1
        ou = tasks(out_piece, RB, i, slot)
        l1 = tasks(ln1_piece, LB, i + 2 if first else jnp.minimum(i + 2, NT - 1), hnext)
        lo = tasks(logits_piece, RB, 1 - slot)
        under = [[ou[s]] + ([l1[s // 2]] if s & 1 else []) for s in range(16)]
        under += [[lo[k]] for k in range(8)]
        under += [lo[8:10], lo[10:12], lo[12:14], lo[14:16], [], [], [], []]
        dots = qkv_dots(1 - slot, hnext, range(3)) + wo_dots(i)
        if first:
            for q in range(NG):
                under[2 * q].append(functools.partial(wo_piece, q))
            stream(dots[:16], under[:16])
            for j in (2, 3, 4):
                cp_mod(j).wait()
            for f in range(NF):
                for cp in cp_ffn(f):
                    cp.start()
            md = _deal([functools.partial(mod_piece, j, g) for j in (2, 3, 4) for g in range(NG)], 16)
            stream(dots[16:], [a + b for a, b in zip(under[16:], md)], {14: lambda: _run(gs)})
        else:
            for k, t in enumerate(tasks(tail_piece, LB, i - 1)):
                under[16 + k].insert(0, t)
            stream(dots, under, {30: lambda: _run(gs)})
        return carry
    step_a(0, 0)
    jax.lax.fori_loop(1, NT - 1, step_a, 0)

    for cp in cp_ffn(0)[:4] + (cp_mod(5),):
        cp.wait()
    last = NT - 1

    h0 = h2[0:TB, :]

    def ffn_dot(c):
        return jnp.dot(h0, wgu[0, :, c:c + 128], preferred_element_type=F32)

    nc, wd7 = FC // 128, wo_dots(last)
    ou, t6, t7 = tasks(out_piece, RB, last, last & 1), tasks(tail_piece, LB, last - 1), tasks(tail_piece, LB, last)
    gcols = [(g * 128 // FH) * 2 * FH + g * 128 % FH for g in range(nc)]
    gd, ud = [[(functools.partial(ffn_dot, c + off), wgu.at[0], 0, c + off) for c in gcols] for off in (0, FH)]
    res = stream(gd + ud[:2] + wd7 + ud[2:],
                 [ou[3 * k:3 * k + 3] for k in range(6)] + [[t6[k], functools.partial(mod_piece, 5, k)] for k in range(NG)] + [t7[:4], t7[4:]])
    for g, u in enumerate(res[nc:nc + 2] + res[-2:]):
        act[:, g * 128:(g + 1) * 128] = swiglu(res[g], u)
    for f in range(NF):
        for cp in cp_ffn(f)[4 if f == 0 else 0:]:
            cp.wait()

    lhs_sums(0)
    rhs_sums(wd.at[0], wds)

    def step_b(n, carry):
        bp, fp = (n - 1) // NF, (n - 1) % NF
        r0 = pl.multiple_of(bp * TB, TB)

        @pl.when(n % NF == 0)
        def _():
            lhs_sums(n // NF)
        rhs_sums(wgu.at[n % NF], ws)
        down_strassen(r0, fp)
        rhs_sums(wd.at[n % NF], wds)
        gate_up(n // NF, n % NF)

        @pl.when(fp == NF - 1)
        def _():
            cp_out(r0, TB, bp).start()
        return carry
    jax.lax.fori_loop(1, NB * NF, step_b, 0)
    outs = [cp_out(b * TB, TB, b) for b in range(NB - 1)]
    for k, a0 in enumerate(range(0, TB, ZB)):
        add_residual(pl.ds(S - TB + a0, ZB), slice(0, D), mm(act[a0:a0 + ZB, :], wd[NF - 1]))
        outs.append(cp_out(S - TB + a0, ZB, NB - 1 + k))
        outs[-1].start()
    for cp in outs:
        cp.wait()


@jax.jit
def pallas_adaLN_cond__sliding_local_dilated__swiglu_ffn__prompt_kernel(
    A_x: jax.Array,
    A_wqkv: jax.Array,
    A_wo: jax.Array,
    B_x: jax.Array,
    B_w_gate: jax.Array,
    B_w_up: jax.Array,
    B_w_down: jax.Array,
    c: jax.Array,
    w_mod: jax.Array,
):
    del B_x
    hbm = pl.BlockSpec(memory_space=pl.ANY)
    out = pl.pallas_call(
        _kernel,
        out_shape=jax.ShapeDtypeStruct((S, D), BF16),
        grid=(1,),
        in_specs=[hbm, hbm, hbm, hbm, hbm, hbm, pl.BlockSpec((1, D), lambda i: (0, 0)), hbm],
        out_specs=hbm,
        scratch_shapes=[
            pltpu.VMEM((S, D), BF16),
            pltpu.VMEM((3, D, D), BF16),
            pltpu.VMEM((3, D, D), BF16),
            pltpu.VMEM((D, D), BF16),
            pltpu.VMEM((NF, D, 2 * FC), BF16),
            pltpu.VMEM((NF, FC, D), BF16),
            pltpu.VMEM((5, TB // 2, D // 2), BF16),
            pltpu.VMEM((5, D // 2, FC), BF16),
            pltpu.VMEM((5, FH, D // 2), BF16),
            pltpu.VMEM((6, D, D), BF16),
            pltpu.VMEM((D, 128), F32),
            pltpu.VMEM((6, 8, D), F32),
            pltpu.VMEM((T, D), BF16),
            pltpu.VMEM((2, NG, T, 128), F32),
            pltpu.VMEM((2, NG, HALO + T, 128), F32),
            pltpu.VMEM((2, NG, HALO + T, 128), F32),
            pltpu.VMEM((W * T, 128), BF16),
            pltpu.VMEM((W * T, 128), F32),
            pltpu.VMEM((T, D), BF16),
            pltpu.VMEM((2, T, D), F32),
            pltpu.VMEM((TB, FC), BF16),
            pltpu.VMEM((S, D), F32),
            pltpu.VMEM((S, D), BF16),
            pltpu.SMEM((1,), jnp.int32),
            pltpu.SemaphoreType.DMA((NT,)),
            pltpu.SemaphoreType.DMA((3,)),
            pltpu.SemaphoreType.DMA((6,)),
            pltpu.SemaphoreType.DMA((1 + 5 * NF,)),
            pltpu.SemaphoreType.DMA((NB - 1 + TB // ZB,)),
        ],
        compiler_params=pltpu.CompilerParams(vmem_limit_bytes=110 * 1024 * 1024),
    )(A_x.reshape(S, D), A_wqkv, A_wo, B_w_gate, B_w_up, B_w_down, c, w_mod)
    return out.reshape(1, S, D)
```

```python
import functools

import jax
import jax.numpy as jnp
import numpy as np
from jax.experimental import pallas as pl
from jax.experimental.pallas import tpu as pltpu

S, D, F = 2048, 1024, 3584
H, DH, W, DIL = 32, 32, 8, 2
HALO = 16
NG = D // 128
T = 256
TB = 1024
PB = 64
FC = 512
RB = 16
LB = 32
LAG = 3
KH = 1024
ZB = 128
EPS = 1e-5
assert DIL * (W // 2) == 8 and HALO >= DIL * (W - 1)
NT, NB, NF = S // T, S // TB, F // FC
FH = FC // 2
F32, BF16 = jnp.float32, jnp.bfloat16


def _spread_rows(v):
    sub = jax.lax.broadcasted_iota(jnp.int32, v[0].shape, 0)
    v = list(v)
    for s, d in ((4, 2), (2, 1)):
        low = (sub & s) == 0
        for a in range(4):
            if not a & d:
                va, vb = v[a], v[a + d]
                v[a] = jnp.where(low, va, pltpu.roll(vb, s, 0))
                v[a + d] = jnp.where(low, pltpu.roll(va, 8 - s, 0), vb)
    return v


def _spread_heads(cols):
    sub = (jax.lax.broadcasted_iota(jnp.int32, cols[0].shape, 1) >> 2) & 7
    out = [None] * NG
    for d in range(1 - NG, NG):
        js = [j for j in range(NG) if 0 <= j - d < NG]
        diag = cols[js[0]]
        for j in js[1:]:
            diag = jnp.where(sub == j - d, cols[j], diag)
        if d:
            diag = pltpu.roll(diag, (4 * d) % 128, 1)
        for j in js:
            out[j - d] = diag if out[j - d] is None else jnp.where(sub == j, diag, out[j - d])
    return out


def _ln_mod(x, scale1, shift):
    m = jnp.mean(x, axis=-1, keepdims=True)
    xc = x - m
    v = jnp.mean(xc * xc, axis=-1, keepdims=True)
    return xc * jax.lax.rsqrt(v + EPS) * scale1 + shift


def _aligned(v, n):
    return v if isinstance(v, int) else pl.multiple_of(v, n)


def _digest(blocks):
    out = None
    for b in blocks:
        for r in range(0, b.shape[0], 16):
            for c in range(0, b.shape[1], 128):
                v = pltpu.bitcast(b[r:r + 16, c:c + 128], jnp.uint32)
                out = v if out is None else out | v
    return pltpu.bitcast(out, BF16)


def _gated(x, gate):
    if gate is None:
        return x
    never, v = gate
    head = jnp.where(never, pltpu.bitcast(v, x.dtype), x[0:8, 0:128])
    if x.shape[1] > 128:
        head = jnp.concatenate([head, x[0:8, 128:]], axis=1)
    return jnp.concatenate([head, x[8:]], axis=0)


def _deal(tasks, n):
    return [tasks[k * len(tasks) // n:(k + 1) * len(tasks) // n] for k in range(n)]


def _run(tasks):
    for t in tasks:
        t()


def _kernel(x_hbm, wqkv_hbm, wo_hbm, wg_hbm, wu_hbm, wd_hbm, c_ref, wmod_hbm, out_hbm,
            xv, wraw, wqkv, wo, wgu, wd, hs, ws, wds, hs2, wmod, sb, mod, hnext, qb, kb, vb, tb, lg, ob, ab, act, x1, h2, flag,
            sem_x, sem_qkv, sem_mod, sem_w, sem_out):
    def cp_x(i):
        return pltpu.make_async_copy(x_hbm.at[pl.ds(_aligned(i * T, T), T)], xv.at[pl.ds(_aligned(i * T, T), T)], sem_x.at[i])

    def cp_mod(j):
        return pltpu.make_async_copy(wmod_hbm.at[:, pl.ds(_aligned(j * D, D), D)], wmod.at[j], sem_mod.at[j])

    def cp_qkv(j):
        return pltpu.make_async_copy(wqkv_hbm.at[:, pl.ds(_aligned(j * D, D), D)], wraw.at[j], sem_qkv.at[j])

    cp_wo = pltpu.make_async_copy(wo_hbm, wraw.at[0], sem_w.at[0])

    def cp_ffn(f):
        c0 = f * FC
        cps = [pltpu.make_async_copy(src.at[:, c0 + p * FH:c0 + (p + 1) * FH],
                                     wgu.at[f, :, (2 * p + q) * FH:(2 * p + q + 1) * FH],
                                     sem_w.at[1 + 5 * f + 2 * p + q])
               for p in range(2) for q, src in enumerate((wg_hbm, wu_hbm))]
        return tuple(cps) + (pltpu.make_async_copy(wd_hbm.at[c0:c0 + FC, :], wd.at[f], sem_w.at[5 + 5 * f]),)

    def cp_out(row0, rows, k):
        return pltpu.make_async_copy(xv.at[pl.ds(row0, rows)], out_hbm.at[pl.ds(row0, rows)], sem_out.at[k])

    cp_qkv(0).start()
    cp_mod(0).start()
    flag[0] = 0
    cv = c_ref[...].astype(F32)
    sc = (cv * jax.nn.sigmoid(cv)).astype(BF16).astype(F32)
    for j in range(NG):
        row = jnp.broadcast_to(sc[:, j * 128:(j + 1) * 128], (128, 128))
        sb[j * 128:(j + 1) * 128, :] = row.T

    def mod_chunk(j):
        def body(r, acc):
            r0 = pl.multiple_of(r * 64, 64)
            s = sb[pl.ds(r0, 64), :]
            out = []
            for g in range(NG):
                t = wmod[j, pl.ds(r0, 64), g * 128:(g + 1) * 128].astype(F32) * s
                t = t[0:32] + t[32:64]
                t = t[0:16] + t[16:32]
                out.append(acc[g] + (t[0:8] + t[8:16]))
            return tuple(out)
        acc = jax.lax.fori_loop(0, D // 64, body, tuple(jnp.zeros((8, 128), F32) for _ in range(NG)))
        one = jnp.where((j == 1) | (j == 4), 1.0, 0.0)
        for g in range(NG):
            res = jnp.sum(acc[g], axis=0, keepdims=True) + one
            mod[j, :, g * 128:(g + 1) * 128] = jnp.broadcast_to(res, (8, 128))

    def mod_piece(j, g, gate=None):
        acc = [None, None]
        for n, r in enumerate(range(0, D, 16)):
            t = wmod[j, r:r + 16, g * 128:(g + 1) * 128].astype(F32) * sb[r:r + 16, :]
            t = _gated(t, gate) if n < 2 else t
            acc[n & 1] = t if n < 2 else acc[n & 1] + t
        res = jnp.sum(acc[0] + acc[1], axis=0, keepdims=True) + (1.0 if j in (1, 4) else 0.0)
        res = jnp.broadcast_to(res, (8, 128))
        mod[j, :, g * 128:(g + 1) * 128] = res
        return pltpu.bitcast(res, BF16)

    def mod_rows(j, rows):
        return jnp.concatenate([mod[j]] * (rows // 8), axis=0)

    def permute_piece(j, r, gate=None):
        cols = [pltpu.bitcast(wraw[j, pl.ds(r, PB), g * 128:(g + 1) * 128], jnp.uint32) for g in range(NG)]
        if gate is not None:
            cols = [_gated(c, gate) for c in cols]
        cols = [pltpu.bitcast(c, BF16) for c in _spread_heads(cols)]
        for g in range(NG):
            wqkv[j, pl.ds(r, PB), g * 128:(g + 1) * 128] = cols[g]
        return _digest(cols)

    def ln1_piece(i, dst, r, gate=None):
        r0 = _aligned(i * T + r, LB)
        xt = _gated(xv[pl.ds(r0, LB), :].astype(F32), gate)
        hv = _ln_mod(xt, mod_rows(1, LB), mod_rows(0, LB)).astype(BF16)
        dst[pl.ds(r, LB), :] = hv
        return _digest([hv])

    qscale = float(DH ** -0.5 * np.log2(np.e))

    def qkv_dot(h, slot, j, k, g):
        res = jnp.dot(h[:, k * KH:(k + 1) * KH], wqkv[j, k * KH:(k + 1) * KH, g * 128:(g + 1) * 128],
                      preferred_element_type=F32)
        buf, r0 = ((qb, 0), (kb, HALO), (vb, HALO))[j]
        if k > 0:
            res = res + buf[slot, g, r0:r0 + T, :]
        if k == D // KH - 1:
            if j == 0:
                res = res * qscale
            else:
                buf[1 - slot, g, 0:HALO, :] = res[T - HALO:, :]
        buf[slot, g, r0:r0 + T, :] = res
        return res

    def window(buf, slot, g, r):
        out = [None] * W
        for w in range(W // 2):
            o = HALO + r - DIL * w - 8
            rows = buf[slot, g, o:o + RB + 8, :]
            out[w], out[w + W // 2] = rows[8:], rows[:RB]
        return out

    def logits_piece(slot, r, gate=None):
        acc = [None] * W
        for g in range(NG):
            qv = qb[slot, g, r:r + RB, :]
            if g == 0:
                qv = _gated(qv, gate)
            for w, kv in enumerate(window(kb, slot, g, r)):
                p = qv * kv
                acc[w] = p if g == 0 else acc[w] + p
        acc = [a.astype(BF16) for a in acc]
        for w in range(W):
            tb[r * W + w * RB:r * W + (w + 1) * RB, :] = acc[w]
        return _digest(acc)

    def groupsum_piece(r0, r1):
        ri = jax.lax.broadcasted_iota(jnp.int32, (128, 128), 0)
        ci = jax.lax.broadcasted_iota(jnp.int32, (128, 128), 1)
        group_ones = jnp.where((ri >> 2) == (ci >> 2), 1.0, 0.0).astype(BF16)
        lg[r0 * W:r1 * W, :] = jnp.dot(tb[r0 * W:r1 * W, :], group_ones, preferred_element_type=F32)

    def out_piece(i, slot, r, gate=None):
        l = [lg[r * W + w * RB:r * W + (w + 1) * RB, :] for w in range(W)]
        if r < HALO and not (isinstance(i, int) and i > 0):
            pos = i * T + r + jax.lax.broadcasted_iota(jnp.int32, (RB, 128), 0)
            l = [l[0]] + [jnp.where(pos >= DIL * w, l[w], -1e9) for w in range(1, W)]
        l[0] = _gated(l[0], gate)
        m = l[0]
        for w in range(1, W):
            m = jnp.maximum(m, l[w])
        e = [jnp.exp2(l[w] - m) for w in range(W)]
        den = e[0]
        for w in range(1, W):
            den = den + e[w]
        inv = 1.0 / den
        p = [e[w] * inv for w in range(W)]
        cols = []
        for g in range(NG):
            acc = None
            for w, vv in enumerate(window(vb, slot, g, r)):
                t = p[w] * vv
                acc = t if w == 0 else acc + t
            cols.append(acc.astype(BF16))
            ob[r:r + RB, g * 128:(g + 1) * 128] = cols[g]
        return _digest(cols)

    def wo_piece(q, gate=None):
        del gate
        a, jh = divmod(q, 2)
        out = []
        for half in range(2):
            rows = [(4 * jh + p) * 128 + a * DH + half * 16 for p in range(4)]
            v = _spread_rows([pltpu.bitcast(wraw[0, r0:r0 + 16, :], jnp.uint32) for r0 in rows])
            for b in range(4):
                r1 = (half * 4 + b) * 128 + a * DH + jh * 16
                out.append(pltpu.bitcast(v[b], BF16))
                wo[r1:r1 + 16, :] = out[-1]
        return _digest(out)

    def wo_dot(st, dst, k, g):
        if not st:
            st['o'] = ob[...]
        res = jnp.dot(st['o'][:, k * KH:(k + 1) * KH], wo[k * KH:(k + 1) * KH, g * 128:(g + 1) * 128],
                      preferred_element_type=F32)
        if k > 0:
            res = res + dst[:, g * 128:(g + 1) * 128]
        dst[:, g * 128:(g + 1) * 128] = res
        return res

    def tail_piece(i, r, gate=None):
        src = ab.at[i & 1]
        r0 = _aligned(i * T + r, LB)
        xn = xv[pl.ds(r0, LB), :].astype(F32) + mod_rows(2, LB) * _gated(src[r:r + LB, :], gate)
        x1[pl.ds(r0, LB), :] = xn
        hv = _ln_mod(xn, mod_rows(4, LB), mod_rows(3, LB)).astype(BF16)
        h2[pl.ds(r0, LB), :] = hv
        return _digest([hv])

    def tasks(fn, step, *args):
        return [functools.partial(fn, *args, r) for r in range(0, T, step)]

    def stream(dots, under, after=None):
        never = never_mask()
        prev, out = None, []
        per = len(dots) // len(under)
        for s, (fn, _, _, _) in enumerate(dots):
            out.append(fn())
            for task in (() if s % per else under[s // per]):
                dig = task(gate=None if prev is None else (never[0:8], prev))
                if s + LAG * per < len(dots):
                    _, w_ref, r, c = dots[s + LAG * per]
                    w_ref[r:r + 16, c:c + 128] = jnp.where(never, dig, w_ref[r:r + 16, c:c + 128])
            if after is not None and s % per == per - 1 and s // per in after:
                after[s // per]()
            prev = out[-1][-8:, :]
        return out

    def qkv_dots(slot, src, js):
        h = src[...]
        return [(functools.partial(qkv_dot, h, slot, j, k, g), wqkv.at[j], k * KH, g * 128)
                for j in js for k in range(D // KH) for g in range(NG)]

    def wo_dots(i):
        st = {}
        return [(functools.partial(wo_dot, st, ab.at[i & 1], k, g), wo, k * KH, g * 128)
                for k in range(D // KH) for g in range(NG)]

    def never_mask():
        return jnp.full((16, 128), flag[0], jnp.int32) > 0

    def swiglu(g, u):
        hg = 0.5 * g
        return ((hg * jnp.tanh(hg) + hg) * u).astype(BF16)

    HM, HK = TB // 2, D // 2

    def combine(x, y, sign):
        x, y = x.astype(F32), y.astype(F32)
        return (x + y if sign > 0 else x - y).astype(BF16)

    QM, QK = HM // 2, HK // 2
    LEFT = ((0, 3, 1), (2, 3, 1), (0, 1, 1), (2, 0, -1), (1, 3, -1))

    def lhs_quarter(b, p, q, r, rows):
        r, c = r + (q // 2) * QM, (q % 2) * QK
        if p < 5:
            return hs[p, pl.ds(r, rows), c:c + QK]
        c += (p - 5) * HK
        return h2[pl.ds(_aligned(b * TB, TB) + (p - 5) * HM + r, rows), c:c + QK]

    def lhs_sums(b):
        def body(n, carry):
            r = pl.multiple_of(n * 64, 64)
            top, bot = pl.ds(_aligned(b * TB, TB) + r, 64), pl.ds(_aligned(b * TB, TB) + HM + r, 64)
            a11, a12, a21, a22 = h2[top, :HK], h2[top, HK:], h2[bot, :HK], h2[bot, HK:]
            for k, (x, y, sign) in enumerate(((a11, a22, 1), (a21, a22, 1), (a11, a12, 1),
                                              (a21, a11, -1), (a12, a22, -1))):
                hs[k, pl.ds(r, 64), :] = combine(x, y, sign)
            return carry
        jax.lax.fori_loop(0, HM // 64, body, 0)

        def second(n, carry):
            r = pl.multiple_of(n * 16, 16)
            for p in range(7):
                q = [lhs_quarter(b, p, k, r, 16) for k in range(4)]
                for k, (x, y, sign) in enumerate(LEFT):
                    hs2[p, k, pl.ds(r, 16), :] = combine(q[x], q[y], sign)
            return carry
        jax.lax.fori_loop(0, QM // 16, second, 0)

    def rhs_sums(w_ref, dst):
        hk, hn = w_ref.shape[0] // 2, w_ref.shape[1] // 2
        for r in range(0, hk, 64):
            top, bot = slice(r, r + 64), slice(hk + r, hk + r + 64)
            b11, b12, b21, b22 = w_ref[top, :hn], w_ref[top, hn:], w_ref[bot, :hn], w_ref[bot, hn:]
            for k, (x, y, sign) in enumerate(((b11, b22, 1), (b12, b22, -1), (b21, b11, -1),
                                              (b11, b12, 1), (b21, b22, 1))):
                dst[k, top, :] = combine(x, y, sign)

    mm = functools.partial(jnp.dot, preferred_element_type=F32)

    def add_residual(rows, cols, d):
        xn = x1[rows, cols] + mod_rows(5, d.shape[0])[:, cols] * d
        x1[rows, cols] = xn
        xv[rows, cols] = xn.astype(BF16)

    def down_strassen(r0, f):
        top, bot, lo, hi = pl.ds(r0, HM), pl.ds(r0 + HM, HM), slice(0, HK), slice(HK, D)
        a11, a12, a21, a22 = act[:HM, :FH], act[:HM, FH:], act[HM:, :FH], act[HM:, FH:]
        m3, m4 = mm(a11, wds[1]), mm(a22, wds[2])
        m5 = mm(combine(a11, a12, 1), wd[f, FH:, HK:])
        add_residual(top, hi, m3 + m5)
        m2 = mm(combine(a21, a22, 1), wd[f, :FH, :HK])
        add_residual(bot, lo, m2 + m4)
        m1 = mm(combine(a11, a22, 1), wds[0])
        c11, c22 = m4 - m5 + m1, m3 - m2 + m1
        add_residual(top, lo, c11 + mm(combine(a12, a22, -1), wds[4]))
        add_residual(bot, hi, c22 + mm(combine(a21, a11, -1), wds[3]))

    def mm2(b, p, y):
        k, n = y.shape[0] // 2, y.shape[1] // 2
        b11, b12, b21, b22 = y[:k, :n], y[:k, n:], y[k:, :n], y[k:, n:]
        m2, m4 = mm(hs2[p, 1], b11), mm(lhs_quarter(b, p, 3, 0, QM), combine(b21, b11, -1))
        m5, m3 = mm(hs2[p, 2], b22), mm(lhs_quarter(b, p, 0, 0, QM), combine(b12, b22, -1))
        m1 = mm(hs2[p, 0], combine(b11, b22, 1))
        c11 = m4 - m5 + m1 + mm(hs2[p, 4], combine(b21, b22, 1))
        c22 = m3 - m2 + m1 + mm(hs2[p, 3], combine(b11, b12, 1))
        return jnp.concatenate([jnp.concatenate([c11, m3 + m5], axis=1),
                                jnp.concatenate([m2 + m4, c22], axis=1)], axis=0)

    def gate_up(b, f):
        def emit(rows, half, c):
            act[rows, half * FH:(half + 1) * FH] = swiglu(c[:, :FH], c[:, FH:])

        m2 = mm2(b, 1, wgu[f, :HK, :FC])
        m4 = mm2(b, 6, ws[2])
        emit(slice(HM, TB), 0, m2 + m4)
        m5 = mm2(b, 2, wgu[f, HK:, FC:])
        m3 = mm2(b, 5, ws[1])
        emit(slice(0, HM), 1, m3 + m5)
        c11, c22 = m4 - m5, m3 - m2
        m1 = mm2(b, 0, ws[0])
        c11, c22 = c11 + m1, c22 + m1
        emit(slice(0, HM), 0, c11 + mm2(b, 4, ws[4]))
        emit(slice(HM, TB), 1, c22 + mm2(b, 3, ws[3]))

    gs = [functools.partial(groupsum_piece, r, r + T // 4) for r in range(0, T, T // 4)]

    kb[0, :, 0:HALO, :] = jnp.zeros((NG, HALO, 128), F32)
    vb[0, :, 0:HALO, :] = jnp.zeros((NG, HALO, 128), F32)
    cp_qkv(0).wait()
    cp_mod(1).start()
    cp_x(0).start()

    def permute_q(r, carry):
        for u in range(128 // PB):
            permute_piece(0, pl.multiple_of(r * 128 + u * PB, PB))
        return carry
    jax.lax.fori_loop(0, D // 128, permute_q, 0)

    def mod_first(j, carry):
        cp_mod(j).wait()

        @pl.when(j == 1)
        def _():
            cp_qkv(1).start()
        mod_chunk(j)
        return carry
    jax.lax.fori_loop(0, 2, mod_first, 0)
    cp_x(0).wait()

    def ln_first(n, carry):
        for u in range(2):
            ln1_piece(0, ob, pl.multiple_of(n * 2 * LB + u * LB, LB))
        return carry
    jax.lax.fori_loop(0, T // (2 * LB), ln_first, 0)
    for j, (head, later) in enumerate(((3, (cp_qkv(2), cp_x(1))), (2, (cp_wo, cp_x(2))))):
        dots = qkv_dots(0, ob, (j,))
        stream(dots[:head], [[]] * head)
        cp_qkv(j + 1).wait()
        for cp in later:
            cp.start()
        pm = [functools.partial(permute_piece, j + 1, r) for r in range(0, D, PB)]
        stream(dots[head:], _deal(pm, NG - head))
    lo, l1 = tasks(logits_piece, RB, 0), tasks(ln1_piece, LB, 1, hnext)
    cp_x(1).wait()
    for j in range(2, 6):
        cp_mod(j).start()
    stream(qkv_dots(0, ob, (2,)), [lo[2 * g:2 * g + 2] + [l1[g]] for g in range(NG)])
    _run(gs)

    cp_wo.wait()
    for i in range(3, NT):
        cp_x(i).start()

    def step_a(i, carry):
        first = isinstance(i, int)
        if first:
            cp_x(i + 2).wait()
        else:
            @pl.when(i + 2 < NT)
            def _():
                cp_x(i + 2).wait()
        slot = i & 1
        ou = tasks(out_piece, RB, i, slot)
        l1 = tasks(ln1_piece, LB, i + 2 if first else jnp.minimum(i + 2, NT - 1), hnext)
        lo = tasks(logits_piece, RB, 1 - slot)
        under = [[ou[s]] + ([l1[s // 2]] if s & 1 else []) for s in range(16)]
        under += [[lo[k]] for k in range(8)]
        under += [lo[8:10], lo[10:12], lo[12:14], lo[14:16], [], [], [], []]
        dots = qkv_dots(1 - slot, hnext, range(3)) + wo_dots(i)
        if first:
            for q in range(NG):
                under[2 * q].append(functools.partial(wo_piece, q))
            stream(dots[:16], under[:16])
            for j in (2, 3, 4):
                cp_mod(j).wait()
            for f in range(NF):
                for cp in cp_ffn(f):
                    cp.start()
            md = _deal([functools.partial(mod_piece, j, g) for j in (2, 3, 4) for g in range(NG)], 16)
            stream(dots[16:], [a + b for a, b in zip(under[16:], md)], {14: lambda: _run(gs)})
        else:
            for k, t in enumerate(tasks(tail_piece, LB, i - 1)):
                under[16 + k].insert(0, t)
            stream(dots, under, {30: lambda: _run(gs)})
        return carry
    step_a(0, 0)
    jax.lax.fori_loop(1, NT - 1, step_a, 0)

    for cp in cp_ffn(0)[:4] + (cp_mod(5),):
        cp.wait()
    last = NT - 1

    h0 = h2[0:TB, :]

    def ffn_dot(c):
        return jnp.dot(h0, wgu[0, :, c:c + 128], preferred_element_type=F32)

    nc, wd7 = FC // 128, wo_dots(last)
    ou, t6, t7 = tasks(out_piece, RB, last, last & 1), tasks(tail_piece, LB, last - 1), tasks(tail_piece, LB, last)
    gcols = [(g * 128 // FH) * 2 * FH + g * 128 % FH for g in range(nc)]
    gd, ud = [[(functools.partial(ffn_dot, c + off), wgu.at[0], 0, c + off) for c in gcols] for off in (0, FH)]
    res = stream(gd + ud[:2] + wd7 + ud[2:],
                 [ou[3 * k:3 * k + 3] for k in range(6)] + [[t6[k], functools.partial(mod_piece, 5, k)] for k in range(NG)] + [t7[:4], t7[4:]])
    for g, u in enumerate(res[nc:nc + 2] + res[-2:]):
        act[:, g * 128:(g + 1) * 128] = swiglu(res[g], u)
    for f in range(NF):
        for cp in cp_ffn(f)[4 if f == 0 else 0:]:
            cp.wait()

    lhs_sums(0)
    rhs_sums(wd.at[0], wds)

    def step_b(n, carry):
        bp, fp = (n - 1) // NF, (n - 1) % NF
        r0 = pl.multiple_of(bp * TB, TB)

        @pl.when(n % NF == 0)
        def _():
            lhs_sums(n // NF)
        rhs_sums(wgu.at[n % NF], ws)
        down_strassen(r0, fp)
        rhs_sums(wd.at[n % NF], wds)
        gate_up(n // NF, n % NF)

        @pl.when(fp == NF - 1)
        def _():
            cp_out(r0, TB, bp).start()
        return carry
    jax.lax.fori_loop(1, NB * NF, step_b, 0)
    outs = [cp_out(b * TB, TB, b) for b in range(NB - 1)]
    for k, a0 in enumerate(range(0, TB, ZB)):
        add_residual(pl.ds(S - TB + a0, ZB), slice(0, D), mm(act[a0:a0 + ZB, :], wd[NF - 1]))
        outs.append(cp_out(S - TB + a0, ZB, NB - 1 + k))
        outs[-1].start()
    for cp in outs:
        cp.wait()


@jax.jit
def pallas_adaLN_cond__sliding_local_dilated__swiglu_ffn__prompt_kernel(
    A_x: jax.Array,
    A_wqkv: jax.Array,
    A_wo: jax.Array,
    B_x: jax.Array,
    B_w_gate: jax.Array,
    B_w_up: jax.Array,
    B_w_down: jax.Array,
    c: jax.Array,
    w_mod: jax.Array,
):
    del B_x
    hbm = pl.BlockSpec(memory_space=pl.ANY)
    out = pl.pallas_call(
        _kernel,
        out_shape=jax.ShapeDtypeStruct((S, D), BF16),
        grid=(1,),
        in_specs=[hbm, hbm, hbm, hbm, hbm, hbm, pl.BlockSpec((1, D), lambda i: (0, 0)), hbm],
        out_specs=hbm,
        scratch_shapes=[
            pltpu.VMEM((S, D), BF16),
            pltpu.VMEM((3, D, D), BF16),
            pltpu.VMEM((3, D, D), BF16),
            pltpu.VMEM((D, D), BF16),
            pltpu.VMEM((NF, D, 2 * FC), BF16),
            pltpu.VMEM((NF, FC, D), BF16),
            pltpu.VMEM((5, TB // 2, D // 2), BF16),
            pltpu.VMEM((5, D // 2, FC), BF16),
            pltpu.VMEM((5, FH, D // 2), BF16),
            pltpu.VMEM((7, 5, TB // 4, D // 4), BF16),
            pltpu.VMEM((6, D, D), BF16),
            pltpu.VMEM((D, 128), F32),
            pltpu.VMEM((6, 8, D), F32),
            pltpu.VMEM((T, D), BF16),
            pltpu.VMEM((2, NG, T, 128), F32),
            pltpu.VMEM((2, NG, HALO + T, 128), F32),
            pltpu.VMEM((2, NG, HALO + T, 128), F32),
            pltpu.VMEM((W * T, 128), BF16),
            pltpu.VMEM((W * T, 128), F32),
            pltpu.VMEM((T, D), BF16),
            pltpu.VMEM((2, T, D), F32),
            pltpu.VMEM((TB, FC), BF16),
            pltpu.VMEM((S, D), F32),
            pltpu.VMEM((S, D), BF16),
            pltpu.SMEM((1,), jnp.int32),
            pltpu.SemaphoreType.DMA((NT,)),
            pltpu.SemaphoreType.DMA((3,)),
            pltpu.SemaphoreType.DMA((6,)),
            pltpu.SemaphoreType.DMA((1 + 5 * NF,)),
            pltpu.SemaphoreType.DMA((NB - 1 + TB // ZB,)),
        ],
        compiler_params=pltpu.CompilerParams(vmem_limit_bytes=110 * 1024 * 1024),
    )(A_x.reshape(S, D), A_wqkv, A_wo, B_w_gate, B_w_up, B_w_down, c, w_mod)
    return out.reshape(1, S, D)
```

```python
import functools

import jax
import jax.numpy as jnp
import numpy as np
from jax.experimental import pallas as pl
from jax.experimental.pallas import tpu as pltpu

S, D, F = 2048, 1024, 3584
H, DH, W, DIL = 32, 32, 8, 2
HALO = 16
NG = D // 128
T = 256
TB = 1024
PB = 64
FC = 512
RB = 16
LB = 32
LAG = 3
KH = 1024
ZB = 128
EPS = 1e-5
assert DIL * (W // 2) == 8 and HALO >= DIL * (W - 1)
NT, NB, NF = S // T, S // TB, F // FC
FH = FC // 2
F32, BF16 = jnp.float32, jnp.bfloat16


def _spread_rows(v):
    sub = jax.lax.broadcasted_iota(jnp.int32, v[0].shape, 0)
    v = list(v)
    for s, d in ((4, 2), (2, 1)):
        low = (sub & s) == 0
        for a in range(4):
            if not a & d:
                va, vb = v[a], v[a + d]
                v[a] = jnp.where(low, va, pltpu.roll(vb, s, 0))
                v[a + d] = jnp.where(low, pltpu.roll(va, 8 - s, 0), vb)
    return v


def _spread_heads(cols):
    sub = (jax.lax.broadcasted_iota(jnp.int32, cols[0].shape, 1) >> 2) & 7
    out = [None] * NG
    for d in range(1 - NG, NG):
        js = [j for j in range(NG) if 0 <= j - d < NG]
        diag = cols[js[0]]
        for j in js[1:]:
            diag = jnp.where(sub == j - d, cols[j], diag)
        if d:
            diag = pltpu.roll(diag, (4 * d) % 128, 1)
        for j in js:
            out[j - d] = diag if out[j - d] is None else jnp.where(sub == j, diag, out[j - d])
    return out


def _ln_mod(x, scale1, shift):
    m = jnp.mean(x, axis=-1, keepdims=True)
    xc = x - m
    v = jnp.mean(xc * xc, axis=-1, keepdims=True)
    return xc * jax.lax.rsqrt(v + EPS) * scale1 + shift


def _aligned(v, n):
    return v if isinstance(v, int) else pl.multiple_of(v, n)


def _digest(blocks):
    out = None
    for b in blocks:
        for r in range(0, b.shape[0], 16):
            for c in range(0, b.shape[1], 128):
                v = pltpu.bitcast(b[r:r + 16, c:c + 128], jnp.uint32)
                out = v if out is None else out | v
    return pltpu.bitcast(out, BF16)


def _gated(x, gate):
    if gate is None:
        return x
    never, v = gate
    head = jnp.where(never, pltpu.bitcast(v, x.dtype), x[0:8, 0:128])
    if x.shape[1] > 128:
        head = jnp.concatenate([head, x[0:8, 128:]], axis=1)
    return jnp.concatenate([head, x[8:]], axis=0)


def _deal(tasks, n):
    return [tasks[k * len(tasks) // n:(k + 1) * len(tasks) // n] for k in range(n)]


def _run(tasks):
    for t in tasks:
        t()


def _kernel(x_hbm, wqkv_hbm, wo_hbm, wg_hbm, wu_hbm, wd_hbm, c_ref, wmod_hbm, out_hbm,
            xv, wraw, wqkv, wo, wgu, wd, hs, ws, wds, hs2, wmod, sb, mod, hnext, qb, kb, vb, tb, lg, ob, ab, act, x1, h2, flag,
            sem_x, sem_qkv, sem_mod, sem_w, sem_out):
    def cp_x(i):
        return pltpu.make_async_copy(x_hbm.at[pl.ds(_aligned(i * T, T), T)], xv.at[pl.ds(_aligned(i * T, T), T)], sem_x.at[i])

    def cp_mod(j):
        return pltpu.make_async_copy(wmod_hbm.at[:, pl.ds(_aligned(j * D, D), D)], wmod.at[j], sem_mod.at[j])

    def cp_qkv(j):
        return pltpu.make_async_copy(wqkv_hbm.at[:, pl.ds(_aligned(j * D, D), D)], wraw.at[j], sem_qkv.at[j])

    cp_wo = pltpu.make_async_copy(wo_hbm, wraw.at[0], sem_w.at[0])

    def cp_ffn(f, gate_up_part=True, down_part=True):
        c0 = f * FC
        cps = []
        if gate_up_part:
            cps += [pltpu.make_async_copy(src.at[:, c0 + p * FH:c0 + (p + 1) * FH],
                                          wgu.at[f, :, (2 * p + q) * FH:(2 * p + q + 1) * FH],
                                          sem_w.at[1 + 5 * f + 2 * p + q])
                    for p in range(2) for q, src in enumerate((wg_hbm, wu_hbm))]
        if down_part:
            cps.append(pltpu.make_async_copy(wd_hbm.at[c0:c0 + FC, :], wd.at[f], sem_w.at[5 + 5 * f]))
        return tuple(cps)

    def cp_out(row0, rows, k):
        return pltpu.make_async_copy(xv.at[pl.ds(row0, rows)], out_hbm.at[pl.ds(row0, rows)], sem_out.at[k])

    cp_qkv(0).start()
    cp_mod(0).start()
    flag[0] = 0
    cv = c_ref[...].astype(F32)
    sc = (cv * jax.nn.sigmoid(cv)).astype(BF16).astype(F32)
    for j in range(NG):
        row = jnp.broadcast_to(sc[:, j * 128:(j + 1) * 128], (128, 128))
        sb[j * 128:(j + 1) * 128, :] = row.T

    def mod_chunk(j):
        def body(r, acc):
            r0 = pl.multiple_of(r * 64, 64)
            s = sb[pl.ds(r0, 64), :]
            out = []
            for g in range(NG):
                t = wmod[j, pl.ds(r0, 64), g * 128:(g + 1) * 128].astype(F32) * s
                t = t[0:32] + t[32:64]
                t = t[0:16] + t[16:32]
                out.append(acc[g] + (t[0:8] + t[8:16]))
            return tuple(out)
        acc = jax.lax.fori_loop(0, D // 64, body, tuple(jnp.zeros((8, 128), F32) for _ in range(NG)))
        one = jnp.where((j == 1) | (j == 4), 1.0, 0.0)
        for g in range(NG):
            res = jnp.sum(acc[g], axis=0, keepdims=True) + one
            mod[j, :, g * 128:(g + 1) * 128] = jnp.broadcast_to(res, (8, 128))

    def mod_piece(j, g, gate=None):
        acc = [None, None]
        for n, r in enumerate(range(0, D, 16)):
            t = wmod[j, r:r + 16, g * 128:(g + 1) * 128].astype(F32) * sb[r:r + 16, :]
            t = _gated(t, gate) if n < 2 else t
            acc[n & 1] = t if n < 2 else acc[n & 1] + t
        res = jnp.sum(acc[0] + acc[1], axis=0, keepdims=True) + (1.0 if j in (1, 4) else 0.0)
        res = jnp.broadcast_to(res, (8, 128))
        mod[j, :, g * 128:(g + 1) * 128] = res
        return pltpu.bitcast(res, BF16)

    def mod_rows(j, rows):
        return jnp.concatenate([mod[j]] * (rows // 8), axis=0)

    def permute_piece(j, r, gate=None):
        cols = [pltpu.bitcast(wraw[j, pl.ds(r, PB), g * 128:(g + 1) * 128], jnp.uint32) for g in range(NG)]
        if gate is not None:
            cols = [_gated(c, gate) for c in cols]
        cols = [pltpu.bitcast(c, BF16) for c in _spread_heads(cols)]
        for g in range(NG):
            wqkv[j, pl.ds(r, PB), g * 128:(g + 1) * 128] = cols[g]
        return _digest(cols)

    def ln1_piece(i, dst, r, gate=None):
        r0 = _aligned(i * T + r, LB)
        xt = _gated(xv[pl.ds(r0, LB), :].astype(F32), gate)
        hv = _ln_mod(xt, mod_rows(1, LB), mod_rows(0, LB)).astype(BF16)
        dst[pl.ds(r, LB), :] = hv
        return _digest([hv])

    qscale = float(DH ** -0.5 * np.log2(np.e))

    def qkv_dot(h, slot, j, k, g):
        res = jnp.dot(h[:, k * KH:(k + 1) * KH], wqkv[j, k * KH:(k + 1) * KH, g * 128:(g + 1) * 128],
                      preferred_element_type=F32)
        buf, r0 = ((qb, 0), (kb, HALO), (vb, HALO))[j]
        if k > 0:
            res = res + buf[slot, g, r0:r0 + T, :]
        if k == D // KH - 1:
            if j == 0:
                res = res * qscale
            else:
                buf[1 - slot, g, 0:HALO, :] = res[T - HALO:, :]
        buf[slot, g, r0:r0 + T, :] = res
        return res

    def window(buf, slot, g, r):
        out = [None] * W
        for w in range(W // 2):
            o = HALO + r - DIL * w - 8
            rows = buf[slot, g, o:o + RB + 8, :]
            out[w], out[w + W // 2] = rows[8:], rows[:RB]
        return out

    def logits_piece(slot, r, gate=None):
        acc = [None] * W
        for g in range(NG):
            qv = qb[slot, g, r:r + RB, :]
            if g == 0:
                qv = _gated(qv, gate)
            for w, kv in enumerate(window(kb, slot, g, r)):
                p = qv * kv
                acc[w] = p if g == 0 else acc[w] + p
        acc = [a.astype(BF16) for a in acc]
        for w in range(W):
            tb[r * W + w * RB:r * W + (w + 1) * RB, :] = acc[w]
        return _digest(acc)

    def groupsum_piece(r0, r1):
        ri = jax.lax.broadcasted_iota(jnp.int32, (128, 128), 0)
        ci = jax.lax.broadcasted_iota(jnp.int32, (128, 128), 1)
        group_ones = jnp.where((ri >> 2) == (ci >> 2), 1.0, 0.0).astype(BF16)
        lg[r0 * W:r1 * W, :] = jnp.dot(tb[r0 * W:r1 * W, :], group_ones, preferred_element_type=F32)

    def out_piece(i, slot, r, gate=None):
        l = [lg[r * W + w * RB:r * W + (w + 1) * RB, :] for w in range(W)]
        if r < HALO and not (isinstance(i, int) and i > 0):
            pos = i * T + r + jax.lax.broadcasted_iota(jnp.int32, (RB, 128), 0)
            l = [l[0]] + [jnp.where(pos >= DIL * w, l[w], -1e9) for w in range(1, W)]
        l[0] = _gated(l[0], gate)
        m = l[0]
        for w in range(1, W):
            m = jnp.maximum(m, l[w])
        e = [jnp.exp2(l[w] - m) for w in range(W)]
        den = e[0]
        for w in range(1, W):
            den = den + e[w]
        inv = 1.0 / den
        p = [e[w] * inv for w in range(W)]
        cols = []
        for g in range(NG):
            acc = None
            for w, vv in enumerate(window(vb, slot, g, r)):
                t = p[w] * vv
                acc = t if w == 0 else acc + t
            cols.append(acc.astype(BF16))
            ob[r:r + RB, g * 128:(g + 1) * 128] = cols[g]
        return _digest(cols)

    def wo_piece(q, gate=None):
        del gate
        a, jh = divmod(q, 2)
        out = []
        for half in range(2):
            rows = [(4 * jh + p) * 128 + a * DH + half * 16 for p in range(4)]
            v = _spread_rows([pltpu.bitcast(wraw[0, r0:r0 + 16, :], jnp.uint32) for r0 in rows])
            for b in range(4):
                r1 = (half * 4 + b) * 128 + a * DH + jh * 16
                out.append(pltpu.bitcast(v[b], BF16))
                wo[r1:r1 + 16, :] = out[-1]
        return _digest(out)

    def wo_dot(st, dst, k, g):
        if not st:
            st['o'] = ob[...]
        res = jnp.dot(st['o'][:, k * KH:(k + 1) * KH], wo[k * KH:(k + 1) * KH, g * 128:(g + 1) * 128],
                      preferred_element_type=F32)
        if k > 0:
            res = res + dst[:, g * 128:(g + 1) * 128]
        dst[:, g * 128:(g + 1) * 128] = res
        return res

    def tail_piece(i, r, gate=None):
        src = ab.at[i & 1]
        r0 = _aligned(i * T + r, LB)
        xn = xv[pl.ds(r0, LB), :].astype(F32) + mod_rows(2, LB) * _gated(src[r:r + LB, :], gate)
        x1[pl.ds(r0, LB), :] = xn
        hv = _ln_mod(xn, mod_rows(4, LB), mod_rows(3, LB)).astype(BF16)
        h2[pl.ds(r0, LB), :] = hv
        return _digest([hv])

    def tasks(fn, step, *args):
        return [functools.partial(fn, *args, r) for r in range(0, T, step)]

    def stream(dots, under, after=None):
        never = never_mask()
        prev, out = None, []
        per = len(dots) // len(under)
        for s, (fn, _, _, _) in enumerate(dots):
            out.append(fn())
            for task in (() if s % per else under[s // per]):
                dig = task(gate=None if prev is None else (never[0:8], prev))
                if s + LAG * per < len(dots):
                    _, w_ref, r, c = dots[s + LAG * per]
                    w_ref[r:r + 16, c:c + 128] = jnp.where(never, dig, w_ref[r:r + 16, c:c + 128])
            if after is not None and s % per == per - 1 and s // per in after:
                after[s // per]()
            prev = out[-1][-8:, :]
        return out

    def qkv_dots(slot, src, js):
        h = src[...]
        return [(functools.partial(qkv_dot, h, slot, j, k, g), wqkv.at[j], k * KH, g * 128)
                for j in js for k in range(D // KH) for g in range(NG)]

    def wo_dots(i):
        st = {}
        return [(functools.partial(wo_dot, st, ab.at[i & 1], k, g), wo, k * KH, g * 128)
                for k in range(D // KH) for g in range(NG)]

    def never_mask():
        return jnp.full((16, 128), flag[0], jnp.int32) > 0

    def swiglu(g, u):
        hg = 0.5 * g
        return ((hg * jnp.tanh(hg) + hg) * u).astype(BF16)

    HM, HK = TB // 2, D // 2

    def combine(x, y, sign):
        x, y = x.astype(F32), y.astype(F32)
        return (x + y if sign > 0 else x - y).astype(BF16)

    QM, QK = HM // 2, HK // 2
    LEFT = ((0, 3, 1), (2, 3, 1), (0, 1, 1), (2, 0, -1), (1, 3, -1))

    def lhs_quarter(b, p, q, r, rows):
        r, c = r + (q // 2) * QM, (q % 2) * QK
        if p < 5:
            return hs[p, pl.ds(r, rows), c:c + QK]
        c += (p - 5) * HK
        return h2[pl.ds(_aligned(b * TB, TB) + (p - 5) * HM + r, rows), c:c + QK]

    def lhs_sums(b):
        def body(n, carry):
            r = pl.multiple_of(n * 64, 64)
            top, bot = pl.ds(_aligned(b * TB, TB) + r, 64), pl.ds(_aligned(b * TB, TB) + HM + r, 64)
            a11, a12, a21, a22 = h2[top, :HK], h2[top, HK:], h2[bot, :HK], h2[bot, HK:]
            for k, (x, y, sign) in enumerate(((a11, a22, 1), (a21, a22, 1), (a11, a12, 1),
                                              (a21, a11, -1), (a12, a22, -1))):
                hs[k, pl.ds(r, 64), :] = combine(x, y, sign)
            return carry
        jax.lax.fori_loop(0, HM // 64, body, 0)

        def second(n, carry):
            r = pl.multiple_of(n * 16, 16)
            for p in range(7):
                q = [lhs_quarter(b, p, k, r, 16) for k in range(4)]
                for k, (x, y, sign) in enumerate(LEFT):
                    hs2[p, k, pl.ds(r, 16), :] = combine(q[x], q[y], sign)
            return carry
        jax.lax.fori_loop(0, QM // 16, second, 0)

    def rhs_sums(w_ref, dst):
        hk, hn = w_ref.shape[0] // 2, w_ref.shape[1] // 2
        for r in range(0, hk, 64):
            top, bot = slice(r, r + 64), slice(hk + r, hk + r + 64)
            b11, b12, b21, b22 = w_ref[top, :hn], w_ref[top, hn:], w_ref[bot, :hn], w_ref[bot, hn:]
            for k, (x, y, sign) in enumerate(((b11, b22, 1), (b12, b22, -1), (b21, b11, -1),
                                              (b11, b12, 1), (b21, b22, 1))):
                dst[k, top, :] = combine(x, y, sign)

    mm = functools.partial(jnp.dot, preferred_element_type=F32)

    def add_residual(rows, cols, d):
        xn = x1[rows, cols] + mod_rows(5, d.shape[0])[:, cols] * d
        x1[rows, cols] = xn
        xv[rows, cols] = xn.astype(BF16)

    def down_strassen(r0, f):
        top, bot, lo, hi = pl.ds(r0, HM), pl.ds(r0 + HM, HM), slice(0, HK), slice(HK, D)
        a11, a12, a21, a22 = act[:HM, :FH], act[:HM, FH:], act[HM:, :FH], act[HM:, FH:]
        m3, m4 = mm(a11, wds[1]), mm(a22, wds[2])
        m5 = mm(combine(a11, a12, 1), wd[f, FH:, HK:])
        add_residual(top, hi, m3 + m5)
        m2 = mm(combine(a21, a22, 1), wd[f, :FH, :HK])
        add_residual(bot, lo, m2 + m4)
        m1 = mm(combine(a11, a22, 1), wds[0])
        c11, c22 = m4 - m5 + m1, m3 - m2 + m1
        add_residual(top, lo, c11 + mm(combine(a12, a22, -1), wds[4]))
        add_residual(bot, hi, c22 + mm(combine(a21, a11, -1), wds[3]))

    def mm2(b, p, y):
        k, n = y.shape[0] // 2, y.shape[1] // 2
        b11, b12, b21, b22 = y[:k, :n], y[:k, n:], y[k:, :n], y[k:, n:]
        m2, m4 = mm(hs2[p, 1], b11), mm(lhs_quarter(b, p, 3, 0, QM), combine(b21, b11, -1))
        m5, m3 = mm(hs2[p, 2], b22), mm(lhs_quarter(b, p, 0, 0, QM), combine(b12, b22, -1))
        m1 = mm(hs2[p, 0], combine(b11, b22, 1))
        c11 = m4 - m5 + m1 + mm(hs2[p, 4], combine(b21, b22, 1))
        c22 = m3 - m2 + m1 + mm(hs2[p, 3], combine(b11, b12, 1))
        return jnp.concatenate([jnp.concatenate([c11, m3 + m5], axis=1),
                                jnp.concatenate([m2 + m4, c22], axis=1)], axis=0)

    def gate_up(b, f):
        def emit(rows, half, c):
            act[rows, half * FH:(half + 1) * FH] = swiglu(c[:, :FH], c[:, FH:])

        m2 = mm2(b, 1, wgu[f, :HK, :FC])
        m4 = mm2(b, 6, ws[2])
        emit(slice(HM, TB), 0, m2 + m4)
        m5 = mm2(b, 2, wgu[f, HK:, FC:])
        m3 = mm2(b, 5, ws[1])
        emit(slice(0, HM), 1, m3 + m5)
        c11, c22 = m4 - m5, m3 - m2
        m1 = mm2(b, 0, ws[0])
        c11, c22 = c11 + m1, c22 + m1
        emit(slice(0, HM), 0, c11 + mm2(b, 4, ws[4]))
        emit(slice(HM, TB), 1, c22 + mm2(b, 3, ws[3]))

    gs = [functools.partial(groupsum_piece, r, r + T // 4) for r in range(0, T, T // 4)]

    kb[0, :, 0:HALO, :] = jnp.zeros((NG, HALO, 128), F32)
    vb[0, :, 0:HALO, :] = jnp.zeros((NG, HALO, 128), F32)
    cp_qkv(0).wait()
    cp_mod(1).start()
    cp_x(0).start()

    def permute_q(r, carry):
        for u in range(128 // PB):
            permute_piece(0, pl.multiple_of(r * 128 + u * PB, PB))
        return carry
    jax.lax.fori_loop(0, D // 128, permute_q, 0)

    def mod_first(j, carry):
        cp_mod(j).wait()

        @pl.when(j == 1)
        def _():
            cp_qkv(1).start()
        mod_chunk(j)
        return carry
    jax.lax.fori_loop(0, 2, mod_first, 0)
    cp_x(0).wait()

    def ln_first(n, carry):
        for u in range(2):
            ln1_piece(0, ob, pl.multiple_of(n * 2 * LB + u * LB, LB))
        return carry
    jax.lax.fori_loop(0, T // (2 * LB), ln_first, 0)
    for j, (head, later) in enumerate(((3, (cp_qkv(2), cp_x(1))), (2, (cp_wo, cp_x(2))))):
        dots = qkv_dots(0, ob, (j,))
        stream(dots[:head], [[]] * head)
        cp_qkv(j + 1).wait()
        for cp in later:
            cp.start()
        pm = [functools.partial(permute_piece, j + 1, r) for r in range(0, D, PB)]
        stream(dots[head:], _deal(pm, NG - head))
    lo, l1 = tasks(logits_piece, RB, 0), tasks(ln1_piece, LB, 1, hnext)
    cp_x(1).wait()
    for j in range(2, 6):
        cp_mod(j).start()
    stream(qkv_dots(0, ob, (2,)), [lo[2 * g:2 * g + 2] + [l1[g]] for g in range(NG)])
    _run(gs)

    cp_wo.wait()
    for i in range(3, NT):
        cp_x(i).start()

    def step_a(i, carry):
        first = isinstance(i, int)
        if first:
            cp_x(i + 2).wait()
        else:
            @pl.when(i + 2 < NT)
            def _():
                cp_x(i + 2).wait()
        slot = i & 1
        ou = tasks(out_piece, RB, i, slot)
        l1 = tasks(ln1_piece, LB, i + 2 if first else jnp.minimum(i + 2, NT - 1), hnext)
        lo = tasks(logits_piece, RB, 1 - slot)
        under = [[ou[s]] + ([l1[s // 2]] if s & 1 else []) for s in range(16)]
        under += [[lo[k]] for k in range(8)]
        under += [lo[8:10], lo[10:12], lo[12:14], lo[14:16], [], [], [], []]
        dots = qkv_dots(1 - slot, hnext, range(3)) + wo_dots(i)
        if first:
            for q in range(NG):
                under[2 * q].append(functools.partial(wo_piece, q))
            stream(dots[:16], under[:16])
            for j in (2, 3, 4):
                cp_mod(j).wait()
            for f in range(NF):
                for cp in cp_ffn(f):
                    cp.start()
            md = _deal([functools.partial(mod_piece, j, g) for j in (2, 3, 4) for g in range(NG)], 16)
            stream(dots[16:], [a + b for a, b in zip(under[16:], md)], {14: lambda: _run(gs)})
        else:
            for k, t in enumerate(tasks(tail_piece, LB, i - 1)):
                under[16 + k].insert(0, t)
            stream(dots, under, {30: lambda: _run(gs)})
        return carry
    step_a(0, 0)
    jax.lax.fori_loop(1, NT - 1, step_a, 0)

    for cp in cp_ffn(0, down_part=False) + (cp_mod(5),):
        cp.wait()
    last = NT - 1

    h0 = h2[0:TB, :]

    def ffn_dot(c):
        return jnp.dot(h0, wgu[0, :, c:c + 128], preferred_element_type=F32)

    nc, wd7 = FC // 128, wo_dots(last)
    ou, t6, t7 = tasks(out_piece, RB, last, last & 1), tasks(tail_piece, LB, last - 1), tasks(tail_piece, LB, last)
    gcols = [(g * 128 // FH) * 2 * FH + g * 128 % FH for g in range(nc)]
    gd, ud = [[(functools.partial(ffn_dot, c + off), wgu.at[0], 0, c + off) for c in gcols] for off in (0, FH)]
    res = stream(gd + ud[:2] + wd7 + ud[2:],
                 [ou[3 * k:3 * k + 3] for k in range(6)] + [[t6[k], functools.partial(mod_piece, 5, k)] for k in range(NG)] + [t7[:4], t7[4:]])
    for g, u in enumerate(res[nc:nc + 2] + res[-2:]):
        act[:, g * 128:(g + 1) * 128] = swiglu(res[g], u)
    for f in range(NF):
        for cp in cp_ffn(f, gate_up_part=f > 0):
            cp.wait()

    lhs_sums(0)
    rhs_sums(wd.at[0], wds)

    def step_b(n, carry):
        bp, fp = (n - 1) // NF, (n - 1) % NF
        r0 = pl.multiple_of(bp * TB, TB)

        @pl.when(n % NF == 0)
        def _():
            lhs_sums(n // NF)
        rhs_sums(wgu.at[n % NF], ws)
        down_strassen(r0, fp)
        rhs_sums(wd.at[n % NF], wds)
        gate_up(n // NF, n % NF)

        @pl.when(fp == NF - 1)
        def _():
            cp_out(r0, TB, bp).start()
        return carry
    jax.lax.fori_loop(1, NB * NF, step_b, 0)
    outs = [cp_out(b * TB, TB, b) for b in range(NB - 1)]
    for k, a0 in enumerate(range(0, TB, ZB)):
        add_residual(pl.ds(S - TB + a0, ZB), slice(0, D), mm(act[a0:a0 + ZB, :], wd[NF - 1]))
        outs.append(cp_out(S - TB + a0, ZB, NB - 1 + k))
        outs[-1].start()
    for cp in outs:
        cp.wait()


@jax.jit
def pallas_adaLN_cond__sliding_local_dilated__swiglu_ffn__prompt_kernel(
    A_x: jax.Array,
    A_wqkv: jax.Array,
    A_wo: jax.Array,
    B_x: jax.Array,
    B_w_gate: jax.Array,
    B_w_up: jax.Array,
    B_w_down: jax.Array,
    c: jax.Array,
    w_mod: jax.Array,
):
    del B_x
    hbm = pl.BlockSpec(memory_space=pl.ANY)
    out = pl.pallas_call(
        _kernel,
        out_shape=jax.ShapeDtypeStruct((S, D), BF16),
        grid=(1,),
        in_specs=[hbm, hbm, hbm, hbm, hbm, hbm, pl.BlockSpec((1, D), lambda i: (0, 0)), hbm],
        out_specs=hbm,
        scratch_shapes=[
            pltpu.VMEM((S, D), BF16),
            pltpu.VMEM((3, D, D), BF16),
            pltpu.VMEM((3, D, D), BF16),
            pltpu.VMEM((D, D), BF16),
            pltpu.VMEM((NF, D, 2 * FC), BF16),
            pltpu.VMEM((NF, FC, D), BF16),
            pltpu.VMEM((5, TB // 2, D // 2), BF16),
            pltpu.VMEM((5, D // 2, FC), BF16),
            pltpu.VMEM((5, FH, D // 2), BF16),
            pltpu.VMEM((7, 5, TB // 4, D // 4), BF16),
            pltpu.VMEM((6, D, D), BF16),
            pltpu.VMEM((D, 128), F32),
            pltpu.VMEM((6, 8, D), F32),
            pltpu.VMEM((T, D), BF16),
            pltpu.VMEM((2, NG, T, 128), F32),
            pltpu.VMEM((2, NG, HALO + T, 128), F32),
            pltpu.VMEM((2, NG, HALO + T, 128), F32),
            pltpu.VMEM((W * T, 128), BF16),
            pltpu.VMEM((W * T, 128), F32),
            pltpu.VMEM((T, D), BF16),
            pltpu.VMEM((2, T, D), F32),
            pltpu.VMEM((TB, FC), BF16),
            pltpu.VMEM((S, D), F32),
            pltpu.VMEM((S, D), BF16),
            pltpu.SMEM((1,), jnp.int32),
            pltpu.SemaphoreType.DMA((NT,)),
            pltpu.SemaphoreType.DMA((3,)),
            pltpu.SemaphoreType.DMA((6,)),
            pltpu.SemaphoreType.DMA((1 + 5 * NF,)),
            pltpu.SemaphoreType.DMA((NB - 1 + TB // ZB,)),
        ],
        compiler_params=pltpu.CompilerParams(vmem_limit_bytes=110 * 1024 * 1024),
    )(A_x.reshape(S, D), A_wqkv, A_wo, B_w_gate, B_w_up, B_w_down, c, w_mod)
    return out.reshape(1, S, D)
```

```python
import functools

import jax
import jax.numpy as jnp
import numpy as np
from jax.experimental import pallas as pl
from jax.experimental.pallas import tpu as pltpu

S, D, F = 2048, 1024, 3584
H, DH, W, DIL = 32, 32, 8, 2
HALO = 16
NG = D // 128
T = 256
TB = 1024
PB = 64
FC = 512
RB = 16
LB = 32
LAG = 3
KH = 1024
ZB = 128
EPS = 1e-5
assert DIL * (W // 2) == 8 and HALO >= DIL * (W - 1)
NT, NB, NF = S // T, S // TB, F // FC
FH = FC // 2
F32, BF16 = jnp.float32, jnp.bfloat16


def _spread_rows(v):
    sub = jax.lax.broadcasted_iota(jnp.int32, v[0].shape, 0)
    v = list(v)
    for s, d in ((4, 2), (2, 1)):
        low = (sub & s) == 0
        for a in range(4):
            if not a & d:
                va, vb = v[a], v[a + d]
                v[a] = jnp.where(low, va, pltpu.roll(vb, s, 0))
                v[a + d] = jnp.where(low, pltpu.roll(va, 8 - s, 0), vb)
    return v


def _spread_heads(cols):
    sub = (jax.lax.broadcasted_iota(jnp.int32, cols[0].shape, 1) >> 2) & 7
    out = [None] * NG
    for d in range(1 - NG, NG):
        js = [j for j in range(NG) if 0 <= j - d < NG]
        diag = cols[js[0]]
        for j in js[1:]:
            diag = jnp.where(sub == j - d, cols[j], diag)
        if d:
            diag = pltpu.roll(diag, (4 * d) % 128, 1)
        for j in js:
            out[j - d] = diag if out[j - d] is None else jnp.where(sub == j, diag, out[j - d])
    return out


def _ln_mod(x, scale1, shift):
    m = jnp.mean(x, axis=-1, keepdims=True)
    xc = x - m
    v = jnp.mean(xc * xc, axis=-1, keepdims=True)
    return xc * jax.lax.rsqrt(v + EPS) * scale1 + shift


def _aligned(v, n):
    return v if isinstance(v, int) else pl.multiple_of(v, n)


def _digest(blocks):
    out = None
    for b in blocks:
        for r in range(0, b.shape[0], 16):
            for c in range(0, b.shape[1], 128):
                v = pltpu.bitcast(b[r:r + 16, c:c + 128], jnp.uint32)
                out = v if out is None else out | v
    return pltpu.bitcast(out, BF16)


def _gated(x, gate):
    if gate is None:
        return x
    never, v = gate
    head = jnp.where(never, pltpu.bitcast(v, x.dtype), x[0:8, 0:128])
    if x.shape[1] > 128:
        head = jnp.concatenate([head, x[0:8, 128:]], axis=1)
    return jnp.concatenate([head, x[8:]], axis=0)


def _deal(tasks, n):
    return [tasks[k * len(tasks) // n:(k + 1) * len(tasks) // n] for k in range(n)]


def _run(tasks):
    for t in tasks:
        t()


def _kernel(x_hbm, wqkv_hbm, wo_hbm, wg_hbm, wu_hbm, wd_hbm, c_ref, wmod_hbm, out_hbm,
            xv, wraw, wqkv, wo, wgu, wd, hs, ws, wds, hs2, wmod, sb, mod, hnext, qb, kb, vb, tb, lg, ob, ab, act, x1, h2, flag,
            sem_x, sem_qkv, sem_mod, sem_w, sem_out):
    def cp_x(i):
        return pltpu.make_async_copy(x_hbm.at[pl.ds(_aligned(i * T, T), T)], xv.at[pl.ds(_aligned(i * T, T), T)], sem_x.at[i])

    def cp_mod(j):
        return pltpu.make_async_copy(wmod_hbm.at[:, pl.ds(_aligned(j * D, D), D)], wmod.at[j], sem_mod.at[j])

    def cp_qkv(j):
        return pltpu.make_async_copy(wqkv_hbm.at[:, pl.ds(_aligned(j * D, D), D)], wraw.at[j], sem_qkv.at[j])

    cp_wo = pltpu.make_async_copy(wo_hbm, wraw.at[0], sem_w.at[0])

    def cp_ffn(f, gate_up_part=True, down_part=True):
        c0 = f * FC
        cps = []
        if gate_up_part:
            cps += [pltpu.make_async_copy(src.at[:, c0 + p * FH:c0 + (p + 1) * FH],
                                          wgu.at[f, :, (2 * p + q) * FH:(2 * p + q + 1) * FH],
                                          sem_w.at[1 + 5 * f + 2 * p + q])
                    for p in range(2) for q, src in enumerate((wg_hbm, wu_hbm))]
        if down_part:
            cps.append(pltpu.make_async_copy(wd_hbm.at[c0:c0 + FC, :], wd.at[f], sem_w.at[5 + 5 * f]))
        return tuple(cps)

    def cp_out(row0, rows, k):
        return pltpu.make_async_copy(xv.at[pl.ds(row0, rows)], out_hbm.at[pl.ds(row0, rows)], sem_out.at[k])

    cp_qkv(0).start()
    cp_mod(0).start()
    flag[0] = 0
    cv = c_ref[...].astype(F32)
    sc = (cv * jax.nn.sigmoid(cv)).astype(BF16).astype(F32)
    for j in range(NG):
        row = jnp.broadcast_to(sc[:, j * 128:(j + 1) * 128], (128, 128))
        sb[j * 128:(j + 1) * 128, :] = row.T

    def mod_chunk(j):
        def body(r, acc):
            r0 = pl.multiple_of(r * 64, 64)
            s = sb[pl.ds(r0, 64), :]
            out = []
            for g in range(NG):
                t = wmod[j, pl.ds(r0, 64), g * 128:(g + 1) * 128].astype(F32) * s
                t = t[0:32] + t[32:64]
                t = t[0:16] + t[16:32]
                out.append(acc[g] + (t[0:8] + t[8:16]))
            return tuple(out)
        acc = jax.lax.fori_loop(0, D // 64, body, tuple(jnp.zeros((8, 128), F32) for _ in range(NG)))
        one = jnp.where((j == 1) | (j == 4), 1.0, 0.0)
        for g in range(NG):
            res = jnp.sum(acc[g], axis=0, keepdims=True) + one
            mod[j, :, g * 128:(g + 1) * 128] = jnp.broadcast_to(res, (8, 128))

    def mod_piece(j, g, gate=None):
        acc = [None, None]
        for n, r in enumerate(range(0, D, 16)):
            t = wmod[j, r:r + 16, g * 128:(g + 1) * 128].astype(F32) * sb[r:r + 16, :]
            t = _gated(t, gate) if n < 2 else t
            acc[n & 1] = t if n < 2 else acc[n & 1] + t
        res = jnp.sum(acc[0] + acc[1], axis=0, keepdims=True) + (1.0 if j in (1, 4) else 0.0)
        res = jnp.broadcast_to(res, (8, 128))
        mod[j, :, g * 128:(g + 1) * 128] = res
        return pltpu.bitcast(res, BF16)

    def mod_rows(j, rows):
        return jnp.concatenate([mod[j]] * (rows // 8), axis=0)

    def permute_piece(j, r, gate=None):
        cols = [pltpu.bitcast(wraw[j, pl.ds(r, PB), g * 128:(g + 1) * 128], jnp.uint32) for g in range(NG)]
        if gate is not None:
            cols = [_gated(c, gate) for c in cols]
        cols = [pltpu.bitcast(c, BF16) for c in _spread_heads(cols)]
        for g in range(NG):
            wqkv[j, pl.ds(r, PB), g * 128:(g + 1) * 128] = cols[g]
        return _digest(cols)

    def ln1_piece(i, dst, r, gate=None):
        r0 = _aligned(i * T + r, LB)
        xt = _gated(xv[pl.ds(r0, LB), :].astype(F32), gate)
        hv = _ln_mod(xt, mod_rows(1, LB), mod_rows(0, LB)).astype(BF16)
        dst[pl.ds(r, LB), :] = hv
        return _digest([hv])

    qscale = float(DH ** -0.5 * np.log2(np.e))

    def qkv_dot(h, slot, j, k, g):
        res = jnp.dot(h[:, k * KH:(k + 1) * KH], wqkv[j, k * KH:(k + 1) * KH, g * 128:(g + 1) * 128],
                      preferred_element_type=F32)
        buf, r0 = ((qb, 0), (kb, HALO), (vb, HALO))[j]
        if k > 0:
            res = res + buf[slot, g, r0:r0 + T, :]
        if k == D // KH - 1:
            if j == 0:
                res = res * qscale
            else:
                buf[1 - slot, g, 0:HALO, :] = res[T - HALO:, :]
        buf[slot, g, r0:r0 + T, :] = res
        return res

    def window(buf, slot, g, r):
        out = [None] * W
        for w in range(W // 2):
            o = HALO + r - DIL * w - 8
            rows = buf[slot, g, o:o + RB + 8, :]
            out[w], out[w + W // 2] = rows[8:], rows[:RB]
        return out

    def logits_piece(slot, r, gate=None):
        acc = [None] * W
        for g in range(NG):
            qv = qb[slot, g, r:r + RB, :]
            if g == 0:
                qv = _gated(qv, gate)
            for w, kv in enumerate(window(kb, slot, g, r)):
                p = qv * kv
                acc[w] = p if g == 0 else acc[w] + p
        acc = [a.astype(BF16) for a in acc]
        for w in range(W):
            tb[r * W + w * RB:r * W + (w + 1) * RB, :] = acc[w]
        return _digest(acc)

    def groupsum_piece(r0, r1):
        ri = jax.lax.broadcasted_iota(jnp.int32, (128, 128), 0)
        ci = jax.lax.broadcasted_iota(jnp.int32, (128, 128), 1)
        group_ones = jnp.where((ri >> 2) == (ci >> 2), 1.0, 0.0).astype(BF16)
        lg[r0 * W:r1 * W, :] = jnp.dot(tb[r0 * W:r1 * W, :], group_ones, preferred_element_type=F32)

    def out_piece(i, slot, r, gate=None):
        l = [lg[r * W + w * RB:r * W + (w + 1) * RB, :] for w in range(W)]
        if r < HALO and not (isinstance(i, int) and i > 0):
            pos = i * T + r + jax.lax.broadcasted_iota(jnp.int32, (RB, 128), 0)
            l = [l[0]] + [jnp.where(pos >= DIL * w, l[w], -1e9) for w in range(1, W)]
        l[0] = _gated(l[0], gate)
        m = l[0]
        for w in range(1, W):
            m = jnp.maximum(m, l[w])
        e = [jnp.exp2(l[w] - m) for w in range(W)]
        den = e[0]
        for w in range(1, W):
            den = den + e[w]
        inv = 1.0 / den
        p = [e[w] * inv for w in range(W)]
        cols = []
        for g in range(NG):
            acc = None
            for w, vv in enumerate(window(vb, slot, g, r)):
                t = p[w] * vv
                acc = t if w == 0 else acc + t
            cols.append(acc.astype(BF16))
            ob[r:r + RB, g * 128:(g + 1) * 128] = cols[g]
        return _digest(cols)

    def wo_piece(q, gate=None):
        del gate
        a, jh = divmod(q, 2)
        out = []
        for half in range(2):
            rows = [(4 * jh + p) * 128 + a * DH + half * 16 for p in range(4)]
            v = _spread_rows([pltpu.bitcast(wraw[0, r0:r0 + 16, :], jnp.uint32) for r0 in rows])
            for b in range(4):
                r1 = (half * 4 + b) * 128 + a * DH + jh * 16
                out.append(pltpu.bitcast(v[b], BF16))
                wo[r1:r1 + 16, :] = out[-1]
        return _digest(out)

    def wo_dot(st, dst, k, g):
        if not st:
            st['o'] = ob[...]
        res = jnp.dot(st['o'][:, k * KH:(k + 1) * KH], wo[k * KH:(k + 1) * KH, g * 128:(g + 1) * 128],
                      preferred_element_type=F32)
        if k > 0:
            res = res + dst[:, g * 128:(g + 1) * 128]
        dst[:, g * 128:(g + 1) * 128] = res
        return res

    def tail_piece(i, r, gate=None):
        src = ab.at[i & 1]
        r0 = _aligned(i * T + r, LB)
        xn = xv[pl.ds(r0, LB), :].astype(F32) + mod_rows(2, LB) * _gated(src[r:r + LB, :], gate)
        x1[pl.ds(r0, LB), :] = xn
        hv = _ln_mod(xn, mod_rows(4, LB), mod_rows(3, LB)).astype(BF16)
        h2[pl.ds(r0, LB), :] = hv
        return _digest([hv])

    def tasks(fn, step, *args):
        return [functools.partial(fn, *args, r) for r in range(0, T, step)]

    def stream(dots, under, after=None):
        never = never_mask()
        prev, out = None, []
        per = len(dots) // len(under)
        for s, (fn, _, _, _) in enumerate(dots):
            out.append(fn())
            for task in (() if s % per else under[s // per]):
                dig = task(gate=None if prev is None else (never[0:8], prev))
                if s + LAG * per < len(dots):
                    _, w_ref, r, c = dots[s + LAG * per]
                    w_ref[r:r + 16, c:c + 128] = jnp.where(never, dig, w_ref[r:r + 16, c:c + 128])
            if after is not None and s % per == per - 1 and s // per in after:
                after[s // per]()
            prev = out[-1][-8:, :]
        return out

    def qkv_dots(slot, src, js):
        h = src[...]
        return [(functools.partial(qkv_dot, h, slot, j, k, g), wqkv.at[j], k * KH, g * 128)
                for j in js for k in range(D // KH) for g in range(NG)]

    def wo_dots(i):
        st = {}
        return [(functools.partial(wo_dot, st, ab.at[i & 1], k, g), wo, k * KH, g * 128)
                for k in range(D // KH) for g in range(NG)]

    def never_mask():
        return jnp.full((16, 128), flag[0], jnp.int32) > 0

    def swiglu(g, u):
        hg = 0.5 * g
        return ((hg * jnp.tanh(hg) + hg) * u).astype(BF16)

    HM, HK = TB // 2, D // 2

    def combine(x, y, sign):
        x, y = x.astype(F32), y.astype(F32)
        return (x + y if sign > 0 else x - y).astype(BF16)

    QM, QK = HM // 2, HK // 2
    LEFT = ((0, 3, 1), (2, 3, 1), (0, 1, 1), (2, 0, -1), (1, 3, -1))

    def lhs_quarter(b, p, q, r, rows):
        r, c = r + (q // 2) * QM, (q % 2) * QK
        if p < 5:
            return hs[p, pl.ds(r, rows), c:c + QK]
        c += (p - 5) * HK
        return h2[pl.ds(_aligned(b * TB, TB) + (p - 5) * HM + r, rows), c:c + QK]

    def lhs_first(b, r, gate=None):
        top, bot = pl.ds(_aligned(b * TB, TB) + r, 64), pl.ds(_aligned(b * TB, TB) + HM + r, 64)
        q = (h2[top, :HK], h2[top, HK:], h2[bot, :HK], h2[bot, HK:])
        out = [combine(q[x], q[y], sign) for x, y, sign in LEFT]
        for k, v in enumerate(out):
            hs[k, pl.ds(r, 64), :] = v
        return _digest([v[-16:, -128:] for v in out])

    def lhs_second(b, r, gate=None):
        out = []
        for p in range(7):
            q = [lhs_quarter(b, p, k, r, 16) for k in range(4)]
            for k, (x, y, sign) in enumerate(LEFT):
                out.append(combine(q[x], q[y], sign))
                hs2[p, k, pl.ds(r, 16), :] = out[-1]
        return _digest([v[:, -128:] for v in out])

    def lhs_sums(b):
        for fn, rows, step in ((lhs_first, HM, 64), (lhs_second, QM, 16)):
            def body(n, carry, fn=fn, step=step):
                fn(b, pl.multiple_of(n * step, step))
                return carry
            jax.lax.fori_loop(0, rows // step, body, 0)

    def rhs_sums(w_ref, dst):
        hk, hn = w_ref.shape[0] // 2, w_ref.shape[1] // 2
        for r in range(0, hk, 64):
            top, bot = slice(r, r + 64), slice(hk + r, hk + r + 64)
            b11, b12, b21, b22 = w_ref[top, :hn], w_ref[top, hn:], w_ref[bot, :hn], w_ref[bot, hn:]
            for k, (x, y, sign) in enumerate(((b11, b22, 1), (b12, b22, -1), (b21, b11, -1),
                                              (b11, b12, 1), (b21, b22, 1))):
                dst[k, top, :] = combine(x, y, sign)

    mm = functools.partial(jnp.dot, preferred_element_type=F32)

    def add_residual(rows, cols, d):
        xn = x1[rows, cols] + mod_rows(5, d.shape[0])[:, cols] * d
        x1[rows, cols] = xn
        xv[rows, cols] = xn.astype(BF16)

    def down_strassen(r0, f):
        top, bot, lo, hi = pl.ds(r0, HM), pl.ds(r0 + HM, HM), slice(0, HK), slice(HK, D)
        a11, a12, a21, a22 = act[:HM, :FH], act[:HM, FH:], act[HM:, :FH], act[HM:, FH:]
        m3, m4 = mm(a11, wds[1]), mm(a22, wds[2])
        m5 = mm(combine(a11, a12, 1), wd[f, FH:, HK:])
        add_residual(top, hi, m3 + m5)
        m2 = mm(combine(a21, a22, 1), wd[f, :FH, :HK])
        add_residual(bot, lo, m2 + m4)
        m1 = mm(combine(a11, a22, 1), wds[0])
        c11, c22 = m4 - m5 + m1, m3 - m2 + m1
        add_residual(top, lo, c11 + mm(combine(a12, a22, -1), wds[4]))
        add_residual(bot, hi, c22 + mm(combine(a21, a11, -1), wds[3]))

    def mm2(b, p, y):
        k, n = y.shape[0] // 2, y.shape[1] // 2
        b11, b12, b21, b22 = y[:k, :n], y[:k, n:], y[k:, :n], y[k:, n:]
        m2, m4 = mm(hs2[p, 1], b11), mm(lhs_quarter(b, p, 3, 0, QM), combine(b21, b11, -1))
        m5, m3 = mm(hs2[p, 2], b22), mm(lhs_quarter(b, p, 0, 0, QM), combine(b12, b22, -1))
        m1 = mm(hs2[p, 0], combine(b11, b22, 1))
        c11 = m4 - m5 + m1 + mm(hs2[p, 4], combine(b21, b22, 1))
        c22 = m3 - m2 + m1 + mm(hs2[p, 3], combine(b11, b12, 1))
        return jnp.concatenate([jnp.concatenate([c11, m3 + m5], axis=1),
                                jnp.concatenate([m2 + m4, c22], axis=1)], axis=0)

    def gate_up(b, f):
        def emit(rows, half, c):
            act[rows, half * FH:(half + 1) * FH] = swiglu(c[:, :FH], c[:, FH:])

        m2 = mm2(b, 1, wgu[f, :HK, :FC])
        m4 = mm2(b, 6, ws[2])
        emit(slice(HM, TB), 0, m2 + m4)
        m5 = mm2(b, 2, wgu[f, HK:, FC:])
        m3 = mm2(b, 5, ws[1])
        emit(slice(0, HM), 1, m3 + m5)
        c11, c22 = m4 - m5, m3 - m2
        m1 = mm2(b, 0, ws[0])
        c11, c22 = c11 + m1, c22 + m1
        emit(slice(0, HM), 0, c11 + mm2(b, 4, ws[4]))
        emit(slice(HM, TB), 1, c22 + mm2(b, 3, ws[3]))

    gs = [functools.partial(groupsum_piece, r, r + T // 4) for r in range(0, T, T // 4)]

    kb[0, :, 0:HALO, :] = jnp.zeros((NG, HALO, 128), F32)
    vb[0, :, 0:HALO, :] = jnp.zeros((NG, HALO, 128), F32)
    cp_qkv(0).wait()
    cp_mod(1).start()
    cp_x(0).start()

    def permute_q(r, carry):
        for u in range(128 // PB):
            permute_piece(0, pl.multiple_of(r * 128 + u * PB, PB))
        return carry
    jax.lax.fori_loop(0, D // 128, permute_q, 0)

    def mod_first(j, carry):
        cp_mod(j).wait()

        @pl.when(j == 1)
        def _():
            cp_qkv(1).start()
        mod_chunk(j)
        return carry
    jax.lax.fori_loop(0, 2, mod_first, 0)
    cp_x(0).wait()

    def ln_first(n, carry):
        for u in range(2):
            ln1_piece(0, ob, pl.multiple_of(n * 2 * LB + u * LB, LB))
        return carry
    jax.lax.fori_loop(0, T // (2 * LB), ln_first, 0)
    for j, (head, later) in enumerate(((3, (cp_qkv(2), cp_x(1))), (2, (cp_wo, cp_x(2))))):
        dots = qkv_dots(0, ob, (j,))
        stream(dots[:head], [[]] * head)
        cp_qkv(j + 1).wait()
        for cp in later:
            cp.start()
        pm = [functools.partial(permute_piece, j + 1, r) for r in range(0, D, PB)]
        stream(dots[head:], _deal(pm, NG - head))
    lo, l1 = tasks(logits_piece, RB, 0), tasks(ln1_piece, LB, 1, hnext)
    cp_x(1).wait()
    for j in range(2, 6):
        cp_mod(j).start()
    stream(qkv_dots(0, ob, (2,)), [lo[2 * g:2 * g + 2] + [l1[g]] for g in range(NG)])
    _run(gs)

    cp_wo.wait()
    for i in range(3, NT):
        cp_x(i).start()

    def step_a(i, carry):
        first = isinstance(i, int)
        if first:
            cp_x(i + 2).wait()
        else:
            @pl.when(i + 2 < NT)
            def _():
                cp_x(i + 2).wait()
        slot = i & 1
        ou = tasks(out_piece, RB, i, slot)
        l1 = tasks(ln1_piece, LB, i + 2 if first else jnp.minimum(i + 2, NT - 1), hnext)
        lo = tasks(logits_piece, RB, 1 - slot)
        under = [[ou[s]] + ([l1[s // 2]] if s & 1 else []) for s in range(16)]
        under += [[lo[k]] for k in range(8)]
        under += [lo[8:10], lo[10:12], lo[12:14], lo[14:16], [], [], [], []]
        dots = qkv_dots(1 - slot, hnext, range(3)) + wo_dots(i)
        if first:
            for q in range(NG):
                under[2 * q].append(functools.partial(wo_piece, q))
            stream(dots[:16], under[:16])
            for j in (2, 3, 4):
                cp_mod(j).wait()
            for f in range(NF):
                for cp in cp_ffn(f):
                    cp.start()
            md = _deal([functools.partial(mod_piece, j, g) for j in (2, 3, 4) for g in range(NG)], 16)
            stream(dots[16:], [a + b for a, b in zip(under[16:], md)], {14: lambda: _run(gs)})
        else:
            for k, t in enumerate(tasks(tail_piece, LB, i - 1)):
                under[16 + k].insert(0, t)
            stream(dots, under, {30: lambda: _run(gs)})
        return carry
    step_a(0, 0)
    jax.lax.fori_loop(1, NT - 1, step_a, 0)

    for cp in cp_ffn(0, down_part=False) + (cp_mod(5),):
        cp.wait()
    last = NT - 1

    h0 = h2[0:TB, :]

    def ffn_dot(c):
        return jnp.dot(h0, wgu[0, :, c:c + 128], preferred_element_type=F32)

    nc, wd7 = FC // 128, wo_dots(last)
    ou, t6, t7 = tasks(out_piece, RB, last, last & 1), tasks(tail_piece, LB, last - 1), tasks(tail_piece, LB, last)
    gcols = [(g * 128 // FH) * 2 * FH + g * 128 % FH for g in range(nc)]
    gd, ud = [[(functools.partial(ffn_dot, c + off), wgu.at[0], 0, c + off) for c in gcols] for off in (0, FH)]
    s1 = _deal([functools.partial(lhs_first, 0, r) for r in range(0, HM, 64)], 4)
    s2 = _deal([functools.partial(lhs_second, 0, r) for r in range(0, QM, 16)], 4)
    res = stream(gd + ud[:2] + wd7 + ud[2:],
                 [ou[3 * k:3 * k + 3] + (s1 + s2)[k] for k in range(6)]
                 + [[t6[k], functools.partial(mod_piece, 5, k)] for k in range(NG)] + [t7[:4] + s2[2], t7[4:] + s2[3]])
    for g, u in enumerate(res[nc:nc + 2] + res[-2:]):
        act[:, g * 128:(g + 1) * 128] = swiglu(res[g], u)
    for f in range(NF):
        for cp in cp_ffn(f, gate_up_part=f > 0):
            cp.wait()

    rhs_sums(wd.at[0], wds)

    def step_b(n, carry):
        bp, fp = (n - 1) // NF, (n - 1) % NF
        r0 = pl.multiple_of(bp * TB, TB)

        @pl.when(n % NF == 0)
        def _():
            lhs_sums(n // NF)
        rhs_sums(wgu.at[n % NF], ws)
        down_strassen(r0, fp)
        rhs_sums(wd.at[n % NF], wds)
        gate_up(n // NF, n % NF)

        @pl.when(fp == NF - 1)
        def _():
            cp_out(r0, TB, bp).start()
        return carry
    jax.lax.fori_loop(1, NB * NF, step_b, 0)
    outs = [cp_out(b * TB, TB, b) for b in range(NB - 1)]
    for k, a0 in enumerate(range(0, TB, ZB)):
        add_residual(pl.ds(S - TB + a0, ZB), slice(0, D), mm(act[a0:a0 + ZB, :], wd[NF - 1]))
        outs.append(cp_out(S - TB + a0, ZB, NB - 1 + k))
        outs[-1].start()
    for cp in outs:
        cp.wait()


@jax.jit
def pallas_adaLN_cond__sliding_local_dilated__swiglu_ffn__prompt_kernel(
    A_x: jax.Array,
    A_wqkv: jax.Array,
    A_wo: jax.Array,
    B_x: jax.Array,
    B_w_gate: jax.Array,
    B_w_up: jax.Array,
    B_w_down: jax.Array,
    c: jax.Array,
    w_mod: jax.Array,
):
    del B_x
    hbm = pl.BlockSpec(memory_space=pl.ANY)
    out = pl.pallas_call(
        _kernel,
        out_shape=jax.ShapeDtypeStruct((S, D), BF16),
        grid=(1,),
        in_specs=[hbm, hbm, hbm, hbm, hbm, hbm, pl.BlockSpec((1, D), lambda i: (0, 0)), hbm],
        out_specs=hbm,
        scratch_shapes=[
            pltpu.VMEM((S, D), BF16),
            pltpu.VMEM((3, D, D), BF16),
            pltpu.VMEM((3, D, D), BF16),
            pltpu.VMEM((D, D), BF16),
            pltpu.VMEM((NF, D, 2 * FC), BF16),
            pltpu.VMEM((NF, FC, D), BF16),
            pltpu.VMEM((5, TB // 2, D // 2), BF16),
            pltpu.VMEM((5, D // 2, FC), BF16),
            pltpu.VMEM((5, FH, D // 2), BF16),
            pltpu.VMEM((7, 5, TB // 4, D // 4), BF16),
            pltpu.VMEM((6, D, D), BF16),
            pltpu.VMEM((D, 128), F32),
            pltpu.VMEM((6, 8, D), F32),
            pltpu.VMEM((T, D), BF16),
            pltpu.VMEM((2, NG, T, 128), F32),
            pltpu.VMEM((2, NG, HALO + T, 128), F32),
            pltpu.VMEM((2, NG, HALO + T, 128), F32),
            pltpu.VMEM((W * T, 128), BF16),
            pltpu.VMEM((W * T, 128), F32),
            pltpu.VMEM((T, D), BF16),
            pltpu.VMEM((2, T, D), F32),
            pltpu.VMEM((TB, FC), BF16),
            pltpu.VMEM((S, D), F32),
            pltpu.VMEM((S, D), BF16),
            pltpu.SMEM((1,), jnp.int32),
            pltpu.SemaphoreType.DMA((NT,)),
            pltpu.SemaphoreType.DMA((3,)),
            pltpu.SemaphoreType.DMA((6,)),
            pltpu.SemaphoreType.DMA((1 + 5 * NF,)),
            pltpu.SemaphoreType.DMA((NB - 1 + TB // ZB,)),
        ],
        compiler_params=pltpu.CompilerParams(vmem_limit_bytes=110 * 1024 * 1024),
    )(A_x.reshape(S, D), A_wqkv, A_wo, B_w_gate, B_w_up, B_w_down, c, w_mod)
    return out.reshape(1, S, D)
```
